```python
import jax
import jax.numpy as jnp

def _softmax(x, axis=-1):
    return jax.nn.softmax(x, axis=axis)
def _gelu(x):
    return jax.nn.gelu(x, approximate=True)
def _silu(x):
    return jax.nn.silu(x)
def _sigmoid(x):
    return jax.nn.sigmoid(x)
def _layernorm(x, axis=-1, eps=1e-5):
    m = jnp.mean(x, axis=axis, keepdims=True)
    v = jnp.var(x, axis=axis, keepdims=True)
    return (x - m) / jnp.sqrt(v + eps)
def _scatter_add(tgt, idx, src, axis=0):
    return tgt.at[idx].add(src)
def _segment_sum(src, seg, n):
    return jax.ops.segment_sum(src, seg, n)
class _Rng:
    def __init__(self, key):
        self._k = key
    def _next(self):
        self._k, sub = jax.random.split(self._k)
        return sub
    def normal(self, shape):
        return jax.random.normal(self._next(), shape, dtype=jnp.bfloat16)
    def randint(self, lo, hi, shape):
        return jax.random.randint(self._next(), shape, lo, hi, dtype=jnp.int32)
    def uniform(self, shape, lo=0.0, hi=1.0):
        return jax.random.uniform(self._next(), shape, jnp.bfloat16, lo, hi)
    def permutation(self, n):
        return jax.random.permutation(self._next(), n)


kernel_name = 'gated_mix__compressed_kv_cla__moe_arch_mod__prompt'

def setup_inputs():
    _rng = _Rng(jax.random.key(int.from_bytes(__import__("os").urandom(4), "little")))
    _w = (lambda a: (lambda t: t.astype(jnp.bfloat16) if jnp.issubdtype(t.dtype, jnp.floating) else t)(jnp.asarray(a)))
    def _A_setup():
        B, H, Sq, Sk, D, M = 1, 16, 2048, 2048, 256, 448
        Dc = 4 * D
        return {
            "x": _w((lambda *s: _rng.normal(s) * 0.05)(B, Sq, M)),
            "c_kv": _w((lambda *s: _rng.normal(s) * 0.05)(B, Sk, Dc)),
            "w_q": _w((lambda *s: _rng.normal(s) * 0.05)(M, H, D) * (M ** -0.5)),
            "w_uk": _w((lambda *s: _rng.normal(s) * 0.05)(Dc, H, D) * (Dc ** -0.5)),
            "w_uv": _w((lambda *s: _rng.normal(s) * 0.05)(Dc, H, D) * (Dc ** -0.5)),
            "w_o": _w((lambda *s: _rng.normal(s) * 0.05)(H, D, M) * ((H * D) ** -0.5)),
        }
    _A_in = _A_setup()

    def _B_setup():
        B, S, D, F, C = 1, 2048, 448, 1792, 2
        return {
            "x": _w((lambda *s: _rng.normal(s) * 0.05)(B, S, D)),
            "w_r": _w((lambda *s: _rng.normal(s) * 0.05)(D)),
            "w_gate": _w((lambda *s: _rng.normal(s) * 0.05)(D, F)),
            "w_up": _w((lambda *s: _rng.normal(s) * 0.05)(D, F)),
            "w_down": _w((lambda *s: _rng.normal(s) * 0.05)(F, D)),
        }
    _B_in = _B_setup()

    return {
        "A_x": _A_in["x"],
        "A_c_kv": _A_in["c_kv"],
        "A_w_q": _A_in["w_q"],
        "A_w_uk": _A_in["w_uk"],
        "A_w_uv": _A_in["w_uv"],
        "A_w_o": _A_in["w_o"],
        "B_x": _B_in["x"],
        "B_w_r": _B_in["w_r"],
        "B_w_gate": _B_in["w_gate"],
        "B_w_up": _B_in["w_up"],
        "B_w_down": _B_in["w_down"],
        "gate_w": _w((lambda *s: _rng.normal(s) * 0.05)(448)),
    }

def reference(A_x, A_c_kv, A_w_q, A_w_uk, A_w_uv, A_w_o, B_x, B_w_r, B_w_gate, B_w_up, B_w_down, gate_w):
    def _A_ref(x, c_kv, w_q, w_uk, w_uv, w_o):
        B, Sq, M = x.shape[0], x.shape[1], x.shape[2]
        Sk = c_kv.shape[1]
        H, D = w_q.shape[1], w_q.shape[2]
        q = jnp.einsum("bqm,mhd->bhqd", x, w_q)
        k = jnp.einsum("bkc,chd->bhkd", c_kv, w_uk)
        v = jnp.einsum("bkc,chd->bhkd", c_kv, w_uv)
        scores = jnp.einsum("bhqd,bhkd->bhqk", q, k) * (D ** -0.5)
        off = Sk - Sq
        qi = jnp.arange(Sq)[:, None]
        kj = jnp.arange(Sk)[None, :]
        cmask = kj <= (qi + off)
        scores = jnp.where(cmask[None, None], scores, -1e9)
        p = _softmax(scores, axis=-1)
        ctx = jnp.einsum("bhqk,bhkd->bhqd", p, v)
        return jnp.einsum("bhqd,hdm->bqm", ctx, w_o)

    def _B_ref(x, w_r, w_gate, w_up, w_down):
        B, S, D = x.shape
        C = 2
        r = x @ w_r
        idx = jnp.argsort(-r, axis=-1)[:, :C]
        idx_e = jnp.repeat(idx.reshape(B, C, 1), D, axis=2)
        x_sel = jnp.take_along_axis(x, idx_e, axis=1)
        g = _silu(x_sel @ w_gate)
        u = x_sel @ w_up
        y = (g * u) @ w_down
        r_sel = _sigmoid(jnp.take_along_axis(r, idx, axis=1))
        y = y * r_sel.reshape(B, C, 1)
        b_off = (jnp.arange(B) * S).reshape(B, 1)
        flat_idx = (idx + b_off).reshape(B * C)
        zero = (x * 0.0).reshape(B * S, D)
        upd = _scatter_add(zero, flat_idx, y.reshape(B * C, D), axis=0)
        return x + upd.reshape(B, S, D)

    x = A_x
    g = _sigmoid((x * gate_w).sum(-1, keepdims=True))
    a = _A_ref(x, A_c_kv, A_w_q, A_w_uk, A_w_uv, A_w_o)
    b = _B_ref(x, B_w_r, B_w_gate, B_w_up, B_w_down)
    return g * a + (1 - g) * b
```

```python
import functools
import math

import jax
import jax.numpy as jnp
from jax import lax
import jax.experimental.pallas as pl
import jax.experimental.pallas.tpu as pltpu

BF = jnp.bfloat16
F32 = jnp.float32
NT = (((1,), (1,)), ((), ()))


def _dot(a, b):
    return jnp.dot(a, b, preferred_element_type=F32)


def _dot_nt(a, b):
    return lax.dot_general(a, b, NT, preferred_element_type=F32)


def _lo(w32):
    return pltpu.bitcast(w32 << 16, F32).astype(BF)


def _hi(w32):
    return pltpu.bitcast(w32 & jnp.uint32(0xFFFF0000), F32).astype(BF)


def _sigmoid(z):
    return 1.0 / (1.0 + jnp.exp(-z))


def make(tq=128, out_chunk=256, interleave=True, name="k1"):
    def kernel(xT_hbm, c_hbm, wq_hbm, wuk_hbm, wuv_hbm, woT_hbm, wr_ref, wg_hbm, wu_hbm, wdT_hbm, gw_ref,
               outT_hbm,
               xT, xn, c, wq, wuk, wuv, woT, wg, wu, wdT, qc, kb, vb, wk16, wv16, outT,
               sem, sem_q, sem_k, sem_v, sem_o):
        M, S = xT.shape
        H, _, D = qc.shape
        P = H // 2
        qscale = (D ** -0.5) * math.log2(math.e)

        wq32 = wq_hbm.bitcast(jnp.uint32)
        wuk32 = wuk_hbm.bitcast(jnp.uint32)
        wuv32 = wuv_hbm.bitcast(jnp.uint32)

        cp_x = pltpu.make_async_copy(xT_hbm, xT, sem.at[0])
        cp_c = pltpu.make_async_copy(c_hbm, c, sem.at[1])
        cp_wo = pltpu.make_async_copy(woT_hbm, woT, sem.at[2])
        cp_wg = pltpu.make_async_copy(wg_hbm, wg, sem.at[3])
        cp_wu = pltpu.make_async_copy(wu_hbm, wu, sem.at[4])
        cp_wd = pltpu.make_async_copy(wdT_hbm, wdT, sem.at[5])

        def cp_q(j):
            return pltpu.make_async_copy(wq32.at[:, j, :], wq.at[j], sem_q.at[j])

        def cp_k(j):
            return pltpu.make_async_copy(wuk32.at[:, j, :], wuk.at[j], sem_k.at[j])

        def cp_v(j):
            return pltpu.make_async_copy(wuv32.at[:, j, :], wuv.at[j], sem_v.at[j])

        cp_x.start()
        for j in range(P):
            cp_q(j).start()
        cp_c.start()
        for j in range(P):
            cp_k(j).start()
            cp_v(j).start()
        cp_wo.start()
        cp_wg.start()
        cp_wu.start()
        cp_wd.start()

        cp_x.wait()
        for t in range(S // 256):
            sl = slice(t * 256, (t + 1) * 256)
            xn[sl, :] = xT[:, sl].T

        def q_body(j, _):
            cp_q(j).wait()
            w = wq[j]
            w2 = jnp.concatenate([_lo(w), _hi(w)], axis=1)
            q = (_dot(xn[...], w2) * qscale).astype(BF)
            qc[2 * j] = q[:, :D]
            qc[2 * j + 1] = q[:, D:]
            return 0

        lax.fori_loop(0, P, q_body, 0)

        cp_c.wait()

        def unpack_w(h):
            j = h // 2
            sh = ((1 - h % 2) * 16).astype(jnp.uint32) if not isinstance(h, int) else (1 - h % 2) * 16
            wk16[...] = pltpu.bitcast((wuk[j] << sh) & jnp.uint32(0xFFFF0000), F32).astype(BF)
            wv16[...] = pltpu.bitcast((wuv[j] << sh) & jnp.uint32(0xFFFF0000), F32).astype(BF)

        def kv_rows(slot, r0, r1):
            kb[slot, r0:r1, :] = _dot(c[r0:r1, :], wk16[...]).astype(BF)
            vb[slot, r0:r1, :] = _dot(c[r0:r1, :], wv16[...]).astype(BF)

        def scores(h, slot, i):
            q0 = i * tq
            q = qc[h, q0:q0 + tq, :]
            parts = [_dot_nt(q, kb[slot, 0:q0 + 128, :])]
            for a in range(1, tq // 128):
                parts.append(_dot_nt(q[a * 128:], kb[slot, q0 + a * 128:q0 + (a + 1) * 128, :]))
            return parts

        def softmax(parts, i):
            q0 = i * tq
            tri = (lax.broadcasted_iota(jnp.int32, (128, 128), 1)
                   <= lax.broadcasted_iota(jnp.int32, (128, 128), 0))
            rows_p, rows_l = [], []
            for a in range(tq // 128):
                tiles = [parts[0][a * 128:(a + 1) * 128, t * 128:(t + 1) * 128] for t in range(q0 // 128 + 1)]
                for b in range(1, a + 1):
                    tiles.append(parts[b][(a - b) * 128:(a - b + 1) * 128, :])
                tiles[-1] = jnp.where(tri, tiles[-1], -1e9)
                m = functools.reduce(jnp.maximum, tiles)
                m = jnp.max(m, axis=1, keepdims=True)
                e = [jnp.exp2(t - m) for t in tiles]
                l = jnp.sum(functools.reduce(jnp.add, e), axis=1, keepdims=True)
                rows_p.append([t.astype(BF) for t in e])
                rows_l.append(l)
            return rows_p, rows_l

        def pv(h, slot, i, rows_p, rows_l):
            q0 = i * tq
            na = tq // 128
            nt = q0 // 128 + 1
            p0 = jnp.concatenate([jnp.concatenate(rows_p[a][:nt], axis=1) for a in range(na)], axis=0)
            acc = _dot(p0, vb[slot, 0:q0 + 128, :])
            accs = [acc[a * 128:(a + 1) * 128] for a in range(na)]
            for b in range(1, na):
                pb = jnp.concatenate([rows_p[a][nt - 1 + b] for a in range(b, na)], axis=0)
                ab = _dot(pb, vb[slot, q0 + b * 128:q0 + (b + 1) * 128, :])
                for a in range(b, na):
                    accs[a] = accs[a] + ab[(a - b) * 128:(a - b + 1) * 128]
            for a in range(na):
                qc[h, q0 + a * 128:q0 + (a + 1) * 128, :] = (accs[a] * (1.0 / rows_l[a])).astype(BF)

        nq = S // tq

        def attn(h, slot, filler):
            s = scores(h, slot, 0)
            for i in range(nq):
                s_next = scores(h, slot, i + 1) if i + 1 < nq else None
                if filler is not None:
                    filler(i)
                p, l = softmax(s, i)
                pv(h, slot, i, p, l)
                s = s_next

        if interleave:
            cp_k(0).wait()
            cp_v(0).wait()
            unpack_w(0)
            kv_rows(0, 0, S)

            def head_body(h, _):
                slot = h % 2

                @pl.when(slot == 1)
                def _():
                    cp_k((h + 1) // 2).wait()
                    cp_v((h + 1) // 2).wait()

                unpack_w(h + 1)
                attn(h, slot, lambda i: kv_rows(1 - slot, i * tq, (i + 1) * tq))
                return 0

            lax.fori_loop(0, H - 1, head_body, 0)
            attn(H - 1, (H - 1) % 2, None)
        else:
            def head_body(h, _):
                @pl.when(h % 2 == 0)
                def _():
                    cp_k(h // 2).wait()
                    cp_v(h // 2).wait()

                unpack_w(h)
                kv_rows(0, 0, S)
                attn(h, 0, None)
                return 0

            lax.fori_loop(0, H, head_body, 0)

        cp_wo.wait()
        cp_wg.wait()
        cp_wu.wait()
        cp_wd.wait()

        def col(ref):
            row = ref[...].astype(F32).reshape(1, M)
            return jnp.broadcast_to(row, (128, M)).T

        wr_c = col(wr_ref)
        gw_c = col(gw_ref)
        r_parts, g_parts = [], []
        for t in range(S // 128):
            xt = xT[:, t * 128:(t + 1) * 128].astype(F32)
            r_parts.append(jnp.sum(xt * wr_c, axis=0, keepdims=True))
            g_parts.append(jnp.sum(xt * gw_c, axis=0, keepdims=True))
        r = jnp.concatenate(r_parts, axis=1).astype(BF).astype(F32)
        gate = _sigmoid(jnp.concatenate(g_parts, axis=1))
        tok = lax.broadcasted_iota(jnp.int32, (1, S), 1)
        neg = jnp.float32(-jnp.inf)
        rs = jnp.where(r != r, neg, r)
        m0 = jnp.max(rs, axis=1, keepdims=True)
        i0 = jnp.min(jnp.where(rs == m0, tok, S), axis=1, keepdims=True)
        hot0 = tok == i0
        rs1 = jnp.where(hot0, neg, rs)
        m1 = jnp.max(rs1, axis=1, keepdims=True)
        i1 = jnp.min(jnp.where((rs1 == m1) & (tok != i0), tok, S), axis=1, keepdims=True)
        hot1 = tok == i1
        r0 = jnp.sum(jnp.where(hot0, r, 0.0), axis=1, keepdims=True)
        r1 = jnp.sum(jnp.where(hot1, r, 0.0), axis=1, keepdims=True)
        row = lax.broadcasted_iota(jnp.int32, (16, S), 0)
        sel = jnp.where(((row == 0) & hot0) | ((row == 1) & hot1), 1.0, 0.0).astype(BF)
        xs = _dot(sel, xn[...]).astype(BF)
        gg = _dot(xs, wg[...])
        uu = _dot(xs, wu[...])
        hh = (gg * _sigmoid(gg) * uu).astype(BF)
        hh = jnp.concatenate([hh, jnp.zeros((112, hh.shape[1]), BF)], axis=0)
        yT = _dot_nt(wdT[...], hh)
        y0 = yT[:, 0:1] * _sigmoid(r0)
        y1 = yT[:, 1:2] * _sigmoid(r1)

        nchunk = S // out_chunk
        for t in range(nchunk):
            sl = slice(t * out_chunk, (t + 1) * out_chunk)
            a = _dot_nt(woT[0], qc[0, sl, :])
            for h in range(1, H):
                a = a + _dot_nt(woT[h], qc[h, sl, :])
            upd = jnp.where(hot0[:, sl], y0, 0.0) + jnp.where(hot1[:, sl], y1, 0.0)
            b = xT[:, sl].astype(F32) + upd
            g = gate[:, sl]
            outT[:, sl] = (g * a + (1.0 - g) * b).astype(BF)
            pltpu.make_async_copy(outT.at[:, sl], outT_hbm.at[:, sl], sem_o.at[t]).start()
        for t in range(nchunk):
            sl = slice(t * out_chunk, (t + 1) * out_chunk)
            pltpu.make_async_copy(outT.at[:, sl], outT_hbm.at[:, sl], sem_o.at[t]).wait()

    def fn(A_x, A_c_kv, A_w_q, A_w_uk, A_w_uv, A_w_o, B_x, B_w_r, B_w_gate, B_w_up, B_w_down, gate_w):
        del B_x
        _, S, M = A_x.shape
        Dc = A_c_kv.shape[2]
        _, H, D = A_w_q.shape
        F = B_w_gate.shape[1]
        any_spec = pl.BlockSpec(memory_space=pl.ANY)
        vmem_spec = pl.BlockSpec(memory_space=pltpu.VMEM)
        outT = pl.pallas_call(
            kernel,
            name=name,
            in_specs=[any_spec] * 6 + [vmem_spec] + [any_spec] * 3 + [vmem_spec],
            out_specs=any_spec,
            out_shape=jax.ShapeDtypeStruct((M, S), BF),
            scratch_shapes=[
                pltpu.VMEM((M, S), BF),
                pltpu.VMEM((S, M), BF),
                pltpu.VMEM((S, Dc), BF),
                pltpu.VMEM((H // 2, M, D), jnp.uint32),
                pltpu.VMEM((H // 2, Dc, D), jnp.uint32),
                pltpu.VMEM((H // 2, Dc, D), jnp.uint32),
                pltpu.VMEM((H, M, D), BF),
                pltpu.VMEM((M, F), BF),
                pltpu.VMEM((M, F), BF),
                pltpu.VMEM((M, F), BF),
                pltpu.VMEM((H, S, D), BF),
                pltpu.VMEM((2, S, D), BF),
                pltpu.VMEM((2, S, D), BF),
                pltpu.VMEM((Dc, D), BF),
                pltpu.VMEM((Dc, D), BF),
                pltpu.VMEM((M, S), BF),
                pltpu.SemaphoreType.DMA((6,)),
                pltpu.SemaphoreType.DMA((H // 2,)),
                pltpu.SemaphoreType.DMA((H // 2,)),
                pltpu.SemaphoreType.DMA((H // 2,)),
                pltpu.SemaphoreType.DMA((S // out_chunk,)),
            ],
            compiler_params=pltpu.CompilerParams(vmem_limit_bytes=120 * 2**20),
        )(A_x[0].T, A_c_kv[0], A_w_q, A_w_uk, A_w_uv, jnp.swapaxes(A_w_o, 1, 2), B_w_r,
          B_w_gate, B_w_up, B_w_down.T, gate_w)
        return outT.T[None]

    return fn


_impl = make(tq=128, interleave=True)


@jax.jit
def pallas_gated_mix__compressed_kv_cla__moe_arch_mod__prompt_kernel(
    A_x, A_c_kv, A_w_q, A_w_uk, A_w_uv, A_w_o, B_x, B_w_r, B_w_gate, B_w_up, B_w_down, gate_w,
):
    return _impl(A_x, A_c_kv, A_w_q, A_w_uk, A_w_uv, A_w_o, B_x, B_w_r, B_w_gate, B_w_up, B_w_down, gate_w)
```

```python
import contextlib
import functools
import math

import jax
import jax.numpy as jnp
from jax import lax
import jax.experimental.pallas as pl
import jax.experimental.pallas.tpu as pltpu

BF = jnp.bfloat16
F32 = jnp.float32
T = 128
_NT = (((1,), (1,)), ((), ()))
_cat = jnp.concatenate

PROG = "K0-1 K2-3 K4-5 K6-7 S7 V0-1 V2-3 S6 V4-5 V6-7 P7 S5 P6 S4 P5 S3 P4 S2 P3 S1 P2 S0 P1 P0"


def _dot(a, b):
    return jnp.dot(a, b, preferred_element_type=F32)


def _dot_nt(a, b):
    return lax.dot_general(a, b, _NT, preferred_element_type=F32)


def _sigmoid(z):
    return 1.0 / (1.0 + jnp.exp(-z))


def _lhs7(a11, a12, a21, a22):
    return (a11 + a22, a21 + a22, a11, a22, a11 + a12, a21 - a11, a12 - a22)


def _rhs7(b11, b12, b21, b22):
    return (b11 + b22, b11, b12 - b22, b21 - b11, b22, b11 + b12, b21 + b22)


def _combine(m):
    return m[0] + m[3] - m[4] + m[6], m[2] + m[4], m[1] + m[3], m[0] - m[1] + m[2] + m[5]


def make(prog=PROG, xchunks=((0, 1), (1, 3), (3, 8)), q_unroll=1, o_unroll=1, scopes=False, flags=None, name="k3"):
    scope = jax.named_scope if scopes else (lambda n: contextlib.nullcontext())

    def kernel(xT_hbm, c_hbm, wq_hbm, wuk_hbm, wuv_hbm, woT_hbm, wr_ref, wg_hbm, wu_hbm, wdT_hbm, gw_ref,
               outT_hbm,
               xT, xa, c, ca, wq, wuk, wuv, woT, wa, wg, wu, wdT, qo, ko, vo, gate_s, hot_s, y_s, outT,
               sem, sem_x, sem_c, sem_q, sem_k, sem_v, sem_o):
        nb, M, _ = xT.shape
        S = nb * 2 * T
        H = qo.shape[0]
        D = 2 * T
        P = H // 2
        Mh = M // 2
        Ch = c.shape[1] // 2
        qscale = (D ** -0.5) * math.log2(math.e)

        wq32 = wq_hbm.bitcast(jnp.uint32)
        wuk32 = wuk_hbm.bitcast(jnp.uint32)
        wuv32 = wuv_hbm.bitcast(jnp.uint32)

        def blk(i):
            return pl.ds(i * D if isinstance(i, int) else pl.multiple_of(i * D, D), D)

        def half(i):
            return pl.ds(i * T if isinstance(i, int) else pl.multiple_of(i * T, T), T)

        cp_wo = pltpu.make_async_copy(woT_hbm, woT, sem.at[0])
        cp_wg = pltpu.make_async_copy(wg_hbm, wg, sem.at[1])
        cp_wu = pltpu.make_async_copy(wu_hbm, wu, sem.at[2])
        cp_wd = pltpu.make_async_copy(wdT_hbm, wdT, sem.at[3])

        def cp_x(i):
            return pltpu.make_async_copy(xT_hbm.at[:, blk(i)], xT.at[i], sem_x.at[i])

        def cp_c(i):
            return pltpu.make_async_copy(c_hbm.at[blk(i), :], c.at[blk(i), :], sem_c.at[i])

        def cp_q(j):
            return pltpu.make_async_copy(wq32.at[:, j, :], wq.at[j], sem_q.at[j])

        def cp_k(j):
            return pltpu.make_async_copy(wuk32.at[:, j, :], wuk.at[j % 2], sem_k.at[j % 2])

        def cp_v(j):
            return pltpu.make_async_copy(wuv32.at[:, j, :], wuv.at[j % 2], sem_v.at[j % 2])

        def cp_out(i):
            return pltpu.make_async_copy(outT.at[i], outT_hbm.at[:, blk(i)], sem_o.at[i])

        def x_ops(i):
            xt = xT[i].astype(F32)
            ops = _lhs7(xt[:Mh, :T], xt[Mh:, :T], xt[:Mh, T:], xt[Mh:, T:])
            for n, t in enumerate(ops):
                xa[n, half(i), :] = t.astype(BF).T

        def c_ops(i):
            cb = c[blk(i), :].astype(F32)
            ops = _lhs7(cb[:T, :Ch], cb[:T, Ch:], cb[T:, :Ch], cb[T:, Ch:])
            for n, t in enumerate(ops):
                for u in range(Ch // T):
                    ca[n, u, half(i), :] = t[:, u * T:(u + 1) * T].astype(BF)

        def wo_ops(h):
            w = woT[h].astype(F32)
            for n, t in enumerate(_lhs7(w[:Mh, :T], w[:Mh, T:], w[Mh:, :T], w[Mh:, T:])):
                wa[n, h] = t.astype(BF)

        def w_ops(w32, shift):
            w = pltpu.bitcast((w32 << shift) & jnp.uint32(0xFFFF0000), F32)
            k = w.shape[0] // 2
            return [t.astype(BF) for t in _rhs7(w[:k, :T], w[:k, T:], w[k:, :T], w[k:, T:])]

        def router():
            def col(ref):
                row = ref[...].astype(F32).reshape(1, M)
                return jnp.broadcast_to(row, (T, M)).T

            wr_c = col(wr_ref)
            gw_c = col(gw_ref)
            r_parts, g_parts = [], []
            for t in range(S // T):
                xt = xT[t // 2, :, (t % 2) * T:(t % 2 + 1) * T].astype(F32)
                r_parts.append(jnp.sum(xt * wr_c, axis=0, keepdims=True))
                g_parts.append(jnp.sum(xt * gw_c, axis=0, keepdims=True))
            r = _cat(r_parts, axis=1).astype(BF).astype(F32)
            gate = _sigmoid(_cat(g_parts, axis=1))
            tok = lax.broadcasted_iota(jnp.int32, (1, S), 1)
            rs = jnp.where(r != r, -jnp.inf, r)
            m0 = jnp.max(rs, axis=1, keepdims=True)
            i0 = jnp.min(jnp.where(rs == m0, tok, S), axis=1, keepdims=True)
            hot0 = tok == i0
            rs1 = jnp.where(hot0, -jnp.inf, rs)
            m1 = jnp.max(rs1, axis=1, keepdims=True)
            i1 = jnp.min(jnp.where((rs1 == m1) & (tok != i0), tok, S), axis=1, keepdims=True)
            hot1 = tok == i1
            r0 = jnp.sum(jnp.where(hot0, r, 0.0), axis=1, keepdims=True)
            r1 = jnp.sum(jnp.where(hot1, r, 0.0), axis=1, keepdims=True)
            hot = jnp.where(hot0, 1, jnp.where(hot1, 2, 0))
            for i in range(nb):
                hot_s[i] = hot[:, i * D:(i + 1) * D]
                gate_s[i] = gate[:, i * D:(i + 1) * D]
            row = lax.broadcasted_iota(jnp.int32, (16, S), 0)
            sel = jnp.where(hot == row + 1, 1.0, 0.0).astype(BF)
            return sel, _sigmoid(r0), _sigmoid(r1)

        def ffn(sel, s0, s1):
            xs = _dot_nt(sel, _cat([xT[i] for i in range(nb)], axis=1)).astype(BF)
            gg = _dot(xs, wg[...])
            uu = _dot(xs, wu[...])
            hh = (gg * _sigmoid(gg) * uu).astype(BF)
            hh = _cat([hh, jnp.zeros((T - 16, hh.shape[1]), BF)], axis=0)
            yT = _dot_nt(wdT[...], hh)
            y_s[0] = jnp.broadcast_to(yT[:, 0:1] * s0, (M, T))
            y_s[1] = jnp.broadcast_to(yT[:, 1:2] * s1, (M, T))

        def q_weights(j):
            w = wq[j]
            return w_ops(w, 16), w_ops(w, 0)

        def q_proj(j, b, lo, hi):
            r = slice(lo * T, hi * T)
            for e in range(2):
                q11, q12, q21, q22 = (t * qscale for t in _combine([_dot(xa[n, r, :], b[e][n]) for n in range(7)]))
                for n, t in enumerate(_lhs7(q11, q12, q21, q22) + (q12, q21)):
                    qo[2 * j + e, n, r, :] = t.astype(BF)

        def kv_proj(kind, b, lo, hi):
            r = slice(lo * T, hi * T)
            c11, c12, c21, c22 = _combine(
                [_dot(_cat([ca[n, u, r, :] for u in range(Ch // T)], axis=1), b[n]) for n in range(7)])
            ops = _rhs7(c11, c21, c12, c22) if kind == "K" else _rhs7(c11, c12, c21, c22)
            dst = ko if kind == "K" else vo
            for n, t in enumerate(ops + (c12, c21)):
                dst[n, r, :] = t.astype(BF)

        def scores(h, i):
            r = slice(i * T, (i + 1) * T)
            q = [qo[h, n, r, :] for n in range(9)]
            quad = [[], [], [], []]
            if i:
                full = _combine([_dot_nt(q[n], ko[n, 0:i * T, :]) for n in range(7)])
                quad = [[s[:, t * T:(t + 1) * T] for t in range(i)] for s in full]
            q_bot = _cat([q[8], q[3]], axis=1)
            d1 = _dot_nt(_cat([_cat([q[2], q[7]], axis=1), q_bot], axis=0), _cat([ko[1, r, :], ko[7, r, :]], axis=1))
            d22 = _dot_nt(q_bot, _cat([ko[8, r, :], ko[4, r, :]], axis=1))
            return quad, d1[:T], d1[T:], d22

        def softmax(s, i):
            (s11, s12, s21, s22), d11, d21, d22 = s
            tri = lax.broadcasted_iota(jnp.int32, (T, T), 1) <= lax.broadcasted_iota(jnp.int32, (T, T), 0)

            def rows(tiles):
                m = jnp.max(functools.reduce(jnp.maximum, tiles), axis=1, keepdims=True)
                e = [jnp.exp2(t - m) for t in tiles]
                l = jnp.sum(functools.reduce(jnp.add, e), axis=1, keepdims=True)
                r = pl.reciprocal(l, approx=True)
                return e, r * (2.0 - l * r)

            et, rt = rows(s11 + s12 + [jnp.where(tri, d11, -1e9)])
            eb, rb = rows(s21 + s22 + [d21, jnp.where(tri, d22, -1e9)])
            ops = [_lhs7(et[t], et[i + t], eb[t], eb[i + t]) for t in range(i)]
            return ops, _cat([et[-1], eb[-2]], axis=0).astype(BF), eb[-1].astype(BF), rt, rb

        def pv(h, i, p):
            ops, p1, p22, rt, rb = p
            r = slice(i * T, (i + 1) * T)
            if i:
                c11, c12, c21, c22 = _combine(
                    [_dot(_cat([o[n] for o in ops], axis=1).astype(BF), vo[n, 0:i * T, :]) for n in range(7)])
            a1 = _dot(p1, _cat([vo[1, r, :], vo[7, r, :]], axis=1))
            a2 = _dot(p22, _cat([vo[8, r, :], vo[4, r, :]], axis=1))
            o11, o12, o21, o22 = a1[:T, :T], a1[:T, T:], a1[T:, :T] + a2[:, :T], a1[T:, T:] + a2[:, T:]
            if i:
                o11, o12, o21, o22 = o11 + c11, o12 + c12, o21 + c21, o22 + c22
            for n, t in enumerate(_rhs7(o11 * rt, o21 * rb, o12 * rt, o22 * rb)):
                qo[h, n, r, :] = t.astype(BF)

        def head_body(h, _):
            j = h // 2

            @pl.when(h % 2 == 0)
            def _():
                cp_k(j).wait()
                cp_v(j).wait()

                @pl.when(j + 1 < P)
                def _():
                    cp_k(j + 1).start()
                    cp_v(j + 1).start()

            with scope("head"):
                shift = ((1 - h % 2) * 16).astype(jnp.uint32)
                b = {"K": w_ops(wuk[j % 2], shift), "V": w_ops(wuv[j % 2], shift)}
                wo_ops(h)
                live = {}
                for op in prog.split():
                    kind, (lo, _, hi) = op[0], op[1:].partition("-")
                    lo = int(lo)
                    if kind in "KV":
                        kv_proj(kind, b[kind], lo, int(hi or lo) + 1)
                    elif kind == "S":
                        live[lo] = softmax(scores(h, lo), lo)
                    else:
                        pv(h, lo, live.pop(lo))
            return 0

        def out_block(i):
            a11, a12, a21, a22 = _combine([
                _dot_nt(_cat([wa[n, h] for h in range(H)], axis=1),
                        _cat([qo[h, n, half(i), :] for h in range(H)], axis=1)) for n in range(7)])
            hot = hot_s[i]
            gate = gate_s[i]
            for (rs, t), a in zip(((0, 0), (0, 1), (1, 0), (1, 1)), (a11, a12, a21, a22)):
                rows, cols = slice(rs * Mh, (rs + 1) * Mh), slice(t * T, (t + 1) * T)
                upd = (jnp.where(hot[:, cols] == 1, y_s[0, rows, :], 0.0)
                       + jnp.where(hot[:, cols] == 2, y_s[1, rows, :], 0.0))
                b = xT[i, rows, cols].astype(F32) + upd
                g = gate[:, cols]
                outT[i, rows, cols] = (g * a + (1.0 - g) * b).astype(BF)
            cp_out(i).start()

        for i in range(*xchunks[0]):
            cp_x(i).start()
        cp_q(0).start()
        for i in range(xchunks[0][1], nb):
            cp_x(i).start()
        for j in range(1, P):
            cp_q(j).start()
            cp_c(j - 1).start()
        cp_c(nb - 1).start()
        cp_wg.start()
        cp_wu.start()
        cp_wd.start()
        cp_k(0).start()
        cp_v(0).start()
        cp_wo.start()

        with scope("q0"):
            cp_q(0).wait()
            for lo, hi in xchunks:
                for i in range(lo, hi):
                    cp_x(i).wait()
                if lo == 0:
                    b = q_weights(0)
                for i in range(lo, hi):
                    x_ops(i)
                    q_proj(0, b, i, i + 1)
            sel, s0, s1 = router()

        def q_body(j, _):
            cp_q(j).wait()
            cp_c(j - 1).wait()
            with scope("q"):
                b = q_weights(j)
                c_ops(j - 1)
                for lo in range(0, nb, 2):
                    q_proj(j, b, lo, lo + 2)
            return 0

        with scope("qloop"):
            lax.fori_loop(1, P, q_body, 0)

        with scope("ffn"):
            cp_c(nb - 1).wait()
            cp_wg.wait()
            cp_wu.wait()
            cp_wd.wait()
            cp_wo.wait()
            c_ops(nb - 1)
            ffn(sel, s0, s1)

        lax.fori_loop(0, H, head_body, 0)

        def out_body(i, _):
            with scope("out"):
                for u in range(o_unroll):
                    out_block(i * o_unroll + u)
            return 0

        lax.fori_loop(0, nb // o_unroll, out_body, 0)
        for i in range(nb):
            cp_out(i).wait()

    def fn(A_x, A_c_kv, A_w_q, A_w_uk, A_w_uv, A_w_o, B_x, B_w_r, B_w_gate, B_w_up, B_w_down, gate_w):
        del B_x
        _, S, M = A_x.shape
        Dc = A_c_kv.shape[2]
        _, H, D = A_w_q.shape
        F = B_w_gate.shape[1]
        nb = S // D
        any_spec = pl.BlockSpec(memory_space=pl.ANY)
        vmem_spec = pl.BlockSpec(memory_space=pltpu.VMEM)
        cp = dict(vmem_limit_bytes=124 * 2**20)
        if flags:
            cp["flags"] = flags
        outT = pl.pallas_call(
            kernel,
            name=name,
            in_specs=[any_spec] * 6 + [vmem_spec] + [any_spec] * 3 + [vmem_spec],
            out_specs=any_spec,
            out_shape=jax.ShapeDtypeStruct((M, S), BF),
            scratch_shapes=[
                pltpu.VMEM((nb, M, D), BF),
                pltpu.VMEM((7, S // 2, M // 2), BF),
                pltpu.VMEM((S, Dc), BF),
                pltpu.VMEM((7, Dc // D, S // 2, T), BF),
                pltpu.VMEM((H // 2, M, D), jnp.uint32),
                pltpu.VMEM((2, Dc, D), jnp.uint32),
                pltpu.VMEM((2, Dc, D), jnp.uint32),
                pltpu.VMEM((H, M, D), BF),
                pltpu.VMEM((7, H, M // 2, T), BF),
                pltpu.VMEM((M, F), BF),
                pltpu.VMEM((M, F), BF),
                pltpu.VMEM((M, F), BF),
                pltpu.VMEM((H, 9, S // 2, T), BF),
                pltpu.VMEM((9, S // 2, T), BF),
                pltpu.VMEM((9, S // 2, T), BF),
                pltpu.VMEM((nb, 1, D), F32),
                pltpu.VMEM((nb, 1, D), jnp.int32),
                pltpu.VMEM((2, M, T), F32),
                pltpu.VMEM((nb, M, D), BF),
                pltpu.SemaphoreType.DMA((4,)),
                pltpu.SemaphoreType.DMA((nb,)),
                pltpu.SemaphoreType.DMA((nb,)),
                pltpu.SemaphoreType.DMA((H // 2,)),
                pltpu.SemaphoreType.DMA((2,)),
                pltpu.SemaphoreType.DMA((2,)),
                pltpu.SemaphoreType.DMA((nb,)),
            ],
            compiler_params=pltpu.CompilerParams(**cp),
        )(A_x[0].T, A_c_kv[0], A_w_q, A_w_uk, A_w_uv, jnp.swapaxes(A_w_o, 1, 2), B_w_r,
          B_w_gate, B_w_up, B_w_down.T, gate_w)
        return outT.T[None]

    return fn


_impl = make()


@jax.jit
def pallas_gated_mix__compressed_kv_cla__moe_arch_mod__prompt_kernel(
    A_x, A_c_kv, A_w_q, A_w_uk, A_w_uv, A_w_o, B_x, B_w_r, B_w_gate, B_w_up, B_w_down, gate_w,
):
    return _impl(A_x, A_c_kv, A_w_q, A_w_uk, A_w_uv, A_w_o, B_x, B_w_r, B_w_gate, B_w_up, B_w_down, gate_w)
```

```python
import contextlib
import functools
import math

import jax
import jax.numpy as jnp
from jax import lax
import jax.experimental.pallas as pl
import jax.experimental.pallas.tpu as pltpu

BF = jnp.bfloat16
F32 = jnp.float32
T = 128
_NT = (((1,), (1,)), ((), ()))
_cat = jnp.concatenate

PROG = "K0-1 K2-3 K4-5 K6-7 S7 V0-1 V2-3 S6 V4-5 V6-7 P7 S5 P6 O7 S4 P5 O6 S3 P4 O5 S2 P3 O4 S1 P2 O3 S0 P1 P0 O2 O0-1"
COEF = ({0: 1, 3: 1, 4: -1, 6: 1}, {2: 1, 4: 1}, {1: 1, 3: 1}, {0: 1, 1: -1, 2: 1, 5: 1})


def _dot(a, b):
    return jnp.dot(a, b, preferred_element_type=F32)


def _dot_nt(a, b):
    return lax.dot_general(a, b, _NT, preferred_element_type=F32)


def _sigmoid(z):
    return 1.0 / (1.0 + jnp.exp(-z))


def _lhs7(a11, a12, a21, a22):
    return (a11 + a22, a21 + a22, a11, a22, a11 + a12, a21 - a11, a12 - a22)


def _rhs7(b11, b12, b21, b22):
    return (b11 + b22, b11, b12 - b22, b21 - b11, b22, b11 + b12, b21 + b22)


def _combine(m, order, defer):
    out = []
    for k, cf in enumerate(COEF):
        ns = [n for n in order if n in cf]
        if defer and len(ns) == 4:
            ns = ns[::-1] if k == 3 else [ns[2], ns[1], ns[0], ns[3]]
        acc, sign = None, 1
        for n in ns:
            if acc is None:
                acc, sign = m[n], cf[n]
            elif sign > 0:
                acc = acc + m[n] if cf[n] > 0 else acc - m[n]
            elif cf[n] > 0:
                acc, sign = m[n] - acc, 1
            else:
                acc = acc + m[n]
        out.append(acc)
    return out


def make(prog=PROG, xchunks=((0, 1), (1, 3), (3, 8)), sord=(0, 1, 2, 5, 3, 4, 6), pord=(2, 4, 5, 1, 3, 0, 6),
         kord=(0, 1, 2, 5, 3, 4, 6), oord=(0, 1, 2, 5, 3, 4, 6), qord=(0, 1, 2, 5, 3, 4, 6), schunk=8, pchunk=8,
         defer="SPKOQ", dep=range(8), lsum=False, mxord=False, wmem="K", wamem=False, early_out=True, qstep=2,
         qcat=False, head_only=False, nocheck=True, scopes=False, flags=None, name="k4"):
    scope = jax.named_scope if scopes else (lambda n: contextlib.nullcontext())

    def kernel(xT_hbm, c_hbm, wq_hbm, wuk_hbm, wuv_hbm, woT_hbm, wr_ref, gw_ref, wg_hbm, wu_hbm, wdT_hbm,
               outT_hbm,
               xT, xa, c, ca, wq, wqb, wuk, wuv, wb, woT, wa, wg, wu, wdT, qo, ko, vo, co, vec_s, r_s, g_s, acc, outT,
               sem, sem_x, sem_c, sem_q, sem_k, sem_v):
        nb, M, _ = xT.shape
        S = nb * 2 * T
        H = qo.shape[0]
        D = 2 * T
        P = H // 2
        Mh = M // 2
        Ch = c.shape[1] // 2
        qscale = (D ** -0.5) * math.log2(math.e)

        wq32 = wq_hbm.bitcast(jnp.uint32)
        wuk32 = wuk_hbm.bitcast(jnp.uint32)
        wuv32 = wuv_hbm.bitcast(jnp.uint32)

        def blk(i):
            return pl.ds(i * D if isinstance(i, int) else pl.multiple_of(i * D, D), D)

        def half(i):
            return pl.ds(i * T if isinstance(i, int) else pl.multiple_of(i * T, T), T)

        def cp_misc(n):
            src, dst = ((woT_hbm, woT), (wg_hbm, wg), (wu_hbm, wu), (wdT_hbm, wdT))[n]
            return pltpu.make_async_copy(src, dst, sem.at[n])

        def cp_x(i):
            return pltpu.make_async_copy(xT_hbm.at[:, blk(i)], xT.at[i], sem_x.at[i])

        def cp_c(i):
            return pltpu.make_async_copy(c_hbm.at[blk(i), :], c.at[blk(i), :], sem_c.at[i])

        def cp_q(j):
            return pltpu.make_async_copy(wq32.at[:, j, :], wq.at[j], sem_q.at[j])

        def cp_k(j):
            return pltpu.make_async_copy(wuk32.at[:, j, :], wuk.at[j % 2], sem_k.at[j % 2])

        def cp_v(j):
            return pltpu.make_async_copy(wuv32.at[:, j, :], wuv.at[j % 2], sem_v.at[j % 2])

        def cp_out(i):
            return pltpu.make_async_copy(outT.at[i], outT_hbm.at[:, blk(i)], sem.at[4])

        def x_ops(i):
            xt = xT[i].astype(F32)
            ops = _lhs7(xt[:Mh, :T], xt[Mh:, :T], xt[:Mh, T:], xt[Mh:, T:])
            for n, t in enumerate(ops):
                xa[n, half(i), :] = t.astype(BF).T

        def c_ops(i):
            cb = c[blk(i), :].astype(F32)
            ops = _lhs7(cb[:T, :Ch], cb[:T, Ch:], cb[T:, :Ch], cb[T:, Ch:])
            for n, t in enumerate(ops):
                for u in range(Ch // T):
                    ca[n, u, half(i), :] = t[:, u * T:(u + 1) * T].astype(BF)

        def wo_ops(h):
            w = woT[h].astype(F32)
            return [t.astype(BF) for t in _lhs7(w[:Mh, :T], w[:Mh, T:], w[Mh:, :T], w[Mh:, T:])]

        def w_ops(w32, shift):
            w = pltpu.bitcast((w32 << shift) & jnp.uint32(0xFFFF0000), F32)
            k = w.shape[0] // 2
            return [t.astype(BF) for t in _rhs7(w[:k, :T], w[:k, T:], w[k:, :T], w[k:, T:])]

        def kv_weights(kind, h):
            shift = (1 - h % 2) * 16
            if not isinstance(h, int):
                shift = shift.astype(jnp.uint32)
            return w_ops((wuk if kind == "K" else wuv)[(h // 2) % 2], shift)

        def stage_kv_weights(h):
            for kind in wmem:
                for n, t in enumerate(kv_weights(kind, h)):
                    wb["KV".index(kind), n] = t

        def stage_q_weights(j):
            w = wq[j]
            for e in range(2):
                for n, t in enumerate(w_ops(w, 16 * (1 - e))):
                    wqb[j % 2, n, :, e * T:(e + 1) * T] = t

        def gate_block(i):
            gs, rs = [], []
            for t in range(2):
                xt = xT[i, :, t * T:(t + 1) * T].astype(F32)
                rs.append(jnp.sum(xt * vec_s[0], axis=0, keepdims=True))
                g = _sigmoid(jnp.sum(xt * vec_s[1], axis=0, keepdims=True))
                gs.append(g)
                acc[i, :, t * T:(t + 1) * T] = (1.0 - g) * xt
            r_s[i] = _cat(rs, axis=1)
            g_s[i] = _cat(gs, axis=1)

        def routed_ffn():
            r = _cat([r_s[i] for i in range(nb)], axis=1).astype(BF).astype(F32)
            tok = lax.broadcasted_iota(jnp.int32, (1, S), 1)
            rs = jnp.where(r != r, -jnp.inf, r)
            i0 = jnp.min(jnp.where(rs == jnp.max(rs, axis=1, keepdims=True), tok, S), axis=1, keepdims=True)
            rs = jnp.where(tok == i0, -jnp.inf, rs)
            i1 = jnp.min(jnp.where((rs == jnp.max(rs, axis=1, keepdims=True)) & (tok != i0), tok, S),
                         axis=1, keepdims=True)
            lane = lax.broadcasted_iota(jnp.int32, (1, D), 1)
            picks = []
            xsT = jnp.zeros((M, T), F32)
            for u, iv in enumerate((i0, i1)):
                idx = iv[0, 0]
                b = idx // D
                hot = lane == idx % D
                w = _sigmoid(jnp.sum(jnp.where(tok == iv, r, 0.0), axis=1, keepdims=True))
                col = jnp.sum(jnp.where(hot, xT[b].astype(F32), 0.0), axis=1, keepdims=True)
                xsT = jnp.where(lane[:, :T] == u, col, xsT)
                picks.append((b, hot, w))
            xs = xsT.T[:16].astype(BF)
            gg = _dot(xs, wg[...])
            uu = _dot(xs, wu[...])
            hh = (gg * _sigmoid(gg) * uu).astype(BF)
            hh = _cat([hh, jnp.zeros((T - 16, hh.shape[1]), BF)], axis=0)
            yT = _dot_nt(wdT[...], hh)
            for u, (b, hot, w) in enumerate(picks):
                acc[b] += jnp.where(hot, (1.0 - g_s[b]) * (yT[:, u:u + 1] * w), 0.0)

        def q_proj(j, weights, lo, hi):
            r = slice(lo * T, hi * T)
            if qcat:
                m = [None] * 7
                for n in qord:
                    m[n] = _dot(xa[n, r, :], weights(n))
                ms = [[t[:, e * T:(e + 1) * T] for t in m] for e in range(2)]
            else:
                ms = [[None] * 7, [None] * 7]
                for e in range(2):
                    for n in qord:
                        ms[e][n] = _dot(xa[n, r, :], weights(n)[:, e * T:(e + 1) * T])
            for e in range(2):
                q11, q12, q21, q22 = (t * qscale for t in _combine(ms[e], qord, "Q" in defer))
                for n, t in enumerate(_lhs7(q11, q12, q21, q22) + (q12, q21)):
                    qo[2 * j + e, n, r, :] = t.astype(BF)

        def head_body(h, _):
            @pl.when((h % 2 == 1) & (h + 1 < H))
            def _():
                cp_k((h + 1) // 2).wait()
                cp_v((h + 1) // 2).wait()

            @pl.when((h % 2 == 0) & (h + 2 < H))
            def _():
                cp_k(h // 2 + 1).start()
                cp_v(h // 2 + 1).start()

            with scope("head"):
                one_head(h)
            return 0

        def one_head(h):
            never = h >= H
            bw = {kind: kv_weights(kind, h) for kind in "KV" if kind not in wmem}
            wo = None if wamem else wo_ops(h)
            live = {}

            def kv_proj(kind, lo, hi):
                r = slice(lo * T, hi * T)
                m = [None] * 7
                for n in kord:
                    b = wb["KV".index(kind), n] if kind in wmem else bw[kind][n]
                    m[n] = _dot(_cat([ca[n, u, r, :] for u in range(Ch // T)], axis=1), b)
                    yield 4 * (hi - lo)
                c11, c12, c21, c22 = _combine(m, kord, "K" in defer)
                ops = _rhs7(c11, c21, c12, c22) if kind == "K" else _rhs7(c11, c12, c21, c22)
                dst = ko if kind == "K" else vo
                for n, t in enumerate(ops + (c12, c21)):
                    dst[n, r, :] = t.astype(BF)

            def scores(i):
                r = slice(i * T, (i + 1) * T)
                quad = [[], [], [], []]
                for t0 in range(0, i, schunk):
                    t1 = min(i, t0 + schunk)
                    m = [None] * 7
                    for n in sord:
                        m[n] = _dot_nt(qo[h, n, r, :], ko[n, t0 * T:t1 * T, :])
                        yield t1 - t0
                    for lst, s in zip(quad, _combine(m, sord, "S" in defer)):
                        lst += [s[:, t * T:(t + 1) * T] for t in range(t1 - t0)]
                q_top = _cat([qo[h, 2, r, :], qo[h, 7, r, :]], axis=1)
                q_bot = _cat([qo[h, 8, r, :], qo[h, 3, r, :]], axis=1)
                d1 = _dot_nt(_cat([q_top, q_bot], axis=0), _cat([ko[1, r, :], ko[7, r, :]], axis=1))
                d22 = _dot_nt(q_bot, _cat([ko[8, r, :], ko[4, r, :]], axis=1))
                yield 6
                tri = lax.broadcasted_iota(jnp.int32, (T, T), 1) <= lax.broadcasted_iota(jnp.int32, (T, T), 0)
                dt, db = [jnp.where(tri, d1[:T], -1e9)], [d1[T:], jnp.where(tri, d22, -1e9)]

                def expd(ks, d):
                    tiles = quad[ks[0]] + quad[ks[1]] + d
                    seq = tiles
                    if mxord:
                        ko_ = sorted(ks, key=lambda k: max(sord.index(n) for n in COEF[k]))
                        seq = [quad[k][t] for t0 in range(0, i, schunk) for k in ko_
                               for t in range(t0, min(i, t0 + schunk))] + d
                    mx = jnp.max(functools.reduce(jnp.maximum, seq), axis=1, keepdims=True)
                    return [jnp.exp2(t - mx) for t in tiles]

                live[i] = expd((0, 1), dt), expd((2, 3), db)

            def pv(i):
                et, eb = live.pop(i)
                r = slice(i * T, (i + 1) * T)
                ops = [_lhs7(et[t], et[i + t], eb[t], eb[i + t]) for t in range(i)]
                m = [None] * 7
                for t0 in range(0, i, pchunk):
                    t1 = min(i, t0 + pchunk)
                    for n in pord:
                        x = _dot(_cat([o[n] for o in ops[t0:t1]], axis=1).astype(BF), vo[n, t0 * T:t1 * T, :])
                        m[n] = x if m[n] is None else m[n] + x
                        yield t1 - t0
                a1 = _dot(_cat([et[-1], eb[-2]], axis=0).astype(BF), _cat([vo[1, r, :], vo[7, r, :]], axis=1))
                a2 = _dot(eb[-1].astype(BF), _cat([vo[8, r, :], vo[4, r, :]], axis=1))
                yield 6
                o = [a1[:T, :T], a1[:T, T:], a1[T:, :T] + a2[:, :T], a1[T:, T:] + a2[:, T:]]
                if i:
                    o = [a + b for a, b in zip(o, _combine(m, pord, "P" in defer))]

                def inv_sum(tiles, late):
                    l = functools.reduce(jnp.add, tiles)
                    if i in dep:
                        l = jnp.where(never, late, l)
                    l = jnp.sum(l, axis=1, keepdims=True)
                    rc = pl.reciprocal(l, approx=True)
                    return rc * (2.0 - l * rc)

                if lsum:
                    rt = inv_sum([x[4] for x in ops] + et[-1:], o[0])
                    rb = inv_sum([x[1] for x in ops] + eb[-2:], o[3])
                else:
                    rt, rb = inv_sum(et, o[0]), inv_sum(eb, o[3])
                for n, t in enumerate(_rhs7(o[0] * rt, o[2] * rb, o[1] * rt, o[3] * rb)):
                    co[n, r, :] = t.astype(BF)

            def out_proj(lo, hi):
                m = [None] * 7
                for n in oord:
                    m[n] = _dot_nt(wa[h, n] if wamem else wo[n], co[n, lo * T:hi * T, :])
                    yield 1.75 * (hi - lo)
                for k, a in enumerate(_combine(m, oord, "O" in defer)):
                    rows, cols = slice((k // 2) * Mh, (k // 2 + 1) * Mh), slice((k % 2) * T, (k % 2 + 1) * T)
                    for i in range(lo, hi):
                        x = acc[i, rows, cols] + g_s[i, :, cols] * a[:, (i - lo) * T:(i - lo + 1) * T]
                        acc[i, rows, cols] = x
                        outT[i, rows, cols] = x.astype(BF)
                if early_out:
                    @pl.when(h == H - 1)
                    def _():
                        for i in range(lo, hi):
                            cp_out(i).start()

            def start(op):
                kind, (lo, _, hi) = op[0], op[1:].partition("-")
                lo = int(lo)
                hi = int(hi or lo) + 1
                if kind in "KV":
                    return kv_proj(kind, lo, hi), 28 * (hi - lo)
                if kind == "O":
                    return out_proj(lo, hi), 12.25 * (hi - lo)
                return (scores if kind == "S" else pv)(lo), 7 * lo + 6

            for group in prog.split():
                lanes = [[*start(op), 0] for op in group.split("+")]
                while lanes:
                    lane = min(lanes, key=lambda l: l[2] / l[1])
                    try:
                        lane[2] += next(lane[0])
                    except StopIteration:
                        lanes.remove(lane)
            stage_kv_weights(jnp.minimum(h + 1, H - 1))

        def prologue():
            for i in range(*xchunks[0]):
                cp_x(i).start()
            cp_q(0).start()
            for i in range(xchunks[0][1], nb):
                cp_x(i).start()
            cp_q(1).start()
            for j in range(2, P):
                cp_q(j).start()
                cp_c(j - 2).start()
            cp_c(nb - 2).start()
            cp_c(nb - 1).start()
            for n in (0, 1, 2, 3):
                cp_misc(n).start()
            cp_k(0).start()
            cp_v(0).start()

            with scope("q0"):
                cp_q(0).wait()
                for s, (lo, hi) in enumerate(xchunks):
                    for i in range(lo, hi):
                        cp_x(i).wait()
                    if s == 0:
                        w = wq[0]
                        b = [_cat(p, axis=1) for p in zip(w_ops(w, 16), w_ops(w, 0))]
                    if s == len(xchunks) - 1:
                        cp_q(1).wait()
                    for i in range(lo, hi):
                        x_ops(i)
                        q_proj(0, lambda n: b[n], i, i + 1)
                stage_q_weights(1)
                for u, ref in enumerate((wr_ref, gw_ref)):
                    vec_s[u] = jnp.broadcast_to(ref[...].astype(F32).reshape(1, M), (T, M)).T
                gate_block(nb - 1)

            def q_body(j, _):
                @pl.when(j + 1 < P)
                def _():
                    cp_q(j + 1).wait()

                cp_c(j - 1).wait()
                with scope("q"):
                    for lo in range(0, nb, qstep):
                        q_proj(j, lambda n: wqb[j % 2, n], lo, lo + qstep)
                    c_ops(j - 1)
                    gate_block(j - 1)
                    stage_q_weights(jnp.minimum(j + 1, P - 1))
                return 0

            lax.fori_loop(1, P, q_body, 0)

            with scope("ffn"):
                cp_c(nb - 1).wait()
                for n in (0, 1, 2, 3):
                    cp_misc(n).wait()
                cp_k(0).wait()
                cp_v(0).wait()
                routed_ffn()
                c_ops(nb - 1)
                stage_kv_weights(0)
                if wamem:
                    for h in range(H):
                        for n, t in enumerate(wo_ops(h)):
                            wa[h, n] = t

        if not head_only:
            prologue()
        lax.fori_loop(0, H, head_body, 0)
        if not early_out:
            for i in range(nb):
                cp_out(i).start()
        for i in range(nb):
            cp_out(i).wait()

    def fn(A_x, A_c_kv, A_w_q, A_w_uk, A_w_uv, A_w_o, B_x, B_w_r, B_w_gate, B_w_up, B_w_down, gate_w):
        del B_x
        _, S, M = A_x.shape
        Dc = A_c_kv.shape[2]
        _, H, D = A_w_q.shape
        F = B_w_gate.shape[1]
        nb = S // D
        any_spec = pl.BlockSpec(memory_space=pl.ANY)
        vmem_spec = pl.BlockSpec(memory_space=pltpu.VMEM)
        cp = dict(vmem_limit_bytes=124 * 2**20, disable_bounds_checks=nocheck)
        if flags:
            cp["flags"] = flags
        outT = pl.pallas_call(
            kernel,
            name=name,
            in_specs=[any_spec] * 6 + [vmem_spec] * 2 + [any_spec] * 3,
            out_specs=any_spec,
            out_shape=jax.ShapeDtypeStruct((M, S), BF),
            scratch_shapes=[
                pltpu.VMEM((nb, M, D), BF),
                pltpu.VMEM((7, S // 2, M // 2), BF),
                pltpu.VMEM((S, Dc), BF),
                pltpu.VMEM((7, Dc // D, S // 2, T), BF),
                pltpu.VMEM((H // 2, M, D), jnp.uint32),
                pltpu.VMEM((2, 7, M // 2, D), BF),
                pltpu.VMEM((2, Dc, D), jnp.uint32),
                pltpu.VMEM((2, Dc, D), jnp.uint32),
                pltpu.VMEM((2, 7, Dc // 2, T), BF),
                pltpu.VMEM((H, M, D), BF),
                pltpu.VMEM((H if wamem else 1, 7, M // 2, T), BF),
                pltpu.VMEM((M, F), BF),
                pltpu.VMEM((M, F), BF),
                pltpu.VMEM((M, F), BF),
                pltpu.VMEM((H, 9, S // 2, T), BF),
                pltpu.VMEM((9, S // 2, T), BF),
                pltpu.VMEM((9, S // 2, T), BF),
                pltpu.VMEM((7, S // 2, T), BF),
                pltpu.VMEM((2, M, T), F32),
                pltpu.VMEM((nb, 1, D), F32),
                pltpu.VMEM((nb, 1, D), F32),
                pltpu.VMEM((nb, M, D), F32),
                pltpu.VMEM((nb, M, D), BF),
                pltpu.SemaphoreType.DMA((5,)),
                pltpu.SemaphoreType.DMA((nb,)),
                pltpu.SemaphoreType.DMA((nb,)),
                pltpu.SemaphoreType.DMA((H // 2,)),
                pltpu.SemaphoreType.DMA((2,)),
                pltpu.SemaphoreType.DMA((2,)),
            ],
            compiler_params=pltpu.CompilerParams(**cp),
        )(A_x[0].T, A_c_kv[0], A_w_q, A_w_uk, A_w_uv, jnp.swapaxes(A_w_o, 1, 2), B_w_r, gate_w,
          B_w_gate, B_w_up, B_w_down.T)
        return outT.T[None]

    return fn


_impl = make()


@jax.jit
def pallas_gated_mix__compressed_kv_cla__moe_arch_mod__prompt_kernel(
    A_x, A_c_kv, A_w_q, A_w_uk, A_w_uv, A_w_o, B_x, B_w_r, B_w_gate, B_w_up, B_w_down, gate_w,
):
    return _impl(A_x, A_c_kv, A_w_q, A_w_uk, A_w_uv, A_w_o, B_x, B_w_r, B_w_gate, B_w_up, B_w_down, gate_w)
```

```python
import contextlib
import functools
import math

import jax
import jax.numpy as jnp
from jax import lax
import jax.experimental.pallas as pl
import jax.experimental.pallas.tpu as pltpu

BF = jnp.bfloat16
F32 = jnp.float32
T = 128
_NT = (((1,), (1,)), ((), ()))
_cat = jnp.concatenate

PROG = "K0-1 K2-3 K4-5 K6-7 S7 V0-1 V2-3 S6 V4-5 V6-7 P7 S5 P6 O7 S4 P5 O6 S3 P4 O5 S2 P3 O4 S1 P2 O3 S0 P1 P0 O2 O0-1"
COEF = ({0: 1, 3: 1, 4: -1, 6: 1}, {2: 1, 4: 1}, {1: 1, 3: 1}, {0: 1, 1: -1, 2: 1, 5: 1})


def _dot(a, b):
    return jnp.dot(a, b, preferred_element_type=F32)


def _dot_nt(a, b):
    return lax.dot_general(a, b, _NT, preferred_element_type=F32)


def _sigmoid(z):
    return 1.0 / (1.0 + jnp.exp(-z))


def _lhs7(a11, a12, a21, a22):
    return (a11 + a22, a21 + a22, a11, a22, a11 + a12, a21 - a11, a12 - a22)


def _rhs7(b11, b12, b21, b22):
    return (b11 + b22, b11, b12 - b22, b21 - b11, b22, b11 + b12, b21 + b22)


def _combine(m, order, defer):
    out = []
    for k, cf in enumerate(COEF):
        ns = [n for n in order if n in cf]
        if defer and len(ns) == 4:
            ns = ns[::-1] if k == 3 else [ns[2], ns[1], ns[0], ns[3]]
        acc, sign = None, 1
        for n in ns:
            if acc is None:
                acc, sign = m[n], cf[n]
            elif sign > 0:
                acc = acc + m[n] if cf[n] > 0 else acc - m[n]
            elif cf[n] > 0:
                acc, sign = m[n] - acc, 1
            else:
                acc = acc + m[n]
        out.append(acc)
    return out


def make(prog=PROG, xchunks=((0, 1), (1, 3), (3, 8)), sord=(0, 1, 2, 5, 3, 4, 6), pord=(2, 4, 5, 1, 3, 0, 6),
         kord=(0, 1, 2, 5, 3, 4, 6), oord=(0, 1, 2, 5, 3, 4, 6), qord=(0, 1, 2, 5, 3, 4, 6), schunk=8, pchunk=8,
         defer="SPKOQ", dep=range(8), lsum=False, mxord=False, spk=(0, 0.8), spv=((0.1, 0.3), (0.3, 0.7)), vnext=True, early_out=True, qstep=2,
         qcat=True, head_only=False, nocheck=True, scopes=False, flags=None, ffn_mix=False, sp=(0, 0.72), sp0=(0, 0.75), sp7=(0, 0.97), qonly=False, paced=range(8), spp=(0.15, 0.9), pace_cap=100000, name="k6"):
    scope = jax.named_scope if scopes else (lambda n: contextlib.nullcontext())

    def kernel(xT_hbm, c_hbm, wq_hbm, wuk_hbm, wuv_hbm, woT_hbm, wr_ref, gw_ref, wg_hbm, wu_hbm, wdT_hbm,
               outT_hbm,
               xT, xa, c, ca, wq, wqb, wuk, wuv, wb, woT, wa, wg, wu, wdT, qo, ko, vo, co, vec_s, r_s, g_s, acc, outT,
               sem, sem_x, sem_q, *per_block):
        po, ro = per_block[:8], per_block[8:]
        nb, M, _ = xT.shape
        S = nb * 2 * T
        H = qo.shape[0]
        D = 2 * T
        P = H // 2
        Mh = M // 2
        Ch = c.shape[1] // 2
        qscale = (D ** -0.5) * math.log2(math.e)

        wq32 = wq_hbm.bitcast(jnp.uint32)
        wuk32 = wuk_hbm.bitcast(jnp.uint32)
        wuv32 = wuv_hbm.bitcast(jnp.uint32)

        def blk(i):
            return pl.ds(i * D if isinstance(i, int) else pl.multiple_of(i * D, D), D)

        def half(i):
            return pl.ds(i * T if isinstance(i, int) else pl.multiple_of(i * T, T), T)

        def cp_misc(n):
            src, dst = ((woT_hbm, woT), (wg_hbm, wg), (wu_hbm, wu), (wdT_hbm, wdT))[n]
            return pltpu.make_async_copy(src, dst, sem.at[0 if n else 3])

        def cp_x(i):
            return pltpu.make_async_copy(xT_hbm.at[:, blk(i)], xT.at[i], sem_x.at[[lo <= i < hi for lo, hi in xchunks].index(True)])

        def cp_c(i):
            return pltpu.make_async_copy(c_hbm.at[blk(i), :], c.at[blk(i), :], sem_q.at[jnp.minimum(i + 2, P)])

        def cp_q(j):
            return pltpu.make_async_copy(wq32.at[:, j, :], wq.at[j], sem_q.at[j])

        def cp_k(j):
            return pltpu.make_async_copy(wuk32.at[:, j, :], wuk.at[j], sem.at[0 if j < 2 else 2])

        def cp_v(j):
            return pltpu.make_async_copy(wuv32.at[:, j, :], wuv.at[j], sem.at[0 if j < 2 else 2])

        def cp_out(i):
            return pltpu.make_async_copy(outT.at[i], outT_hbm.at[:, blk(i)], sem.at[1])

        def pad_rows(t):
            return _cat([t, jnp.zeros((D - Mh, t.shape[1]), t.dtype)], axis=0)

        def x_ops(i):
            xt = xT[i].astype(F32)
            ops = _lhs7(xt[:Mh, :T], xt[Mh:, :T], xt[:Mh, T:], xt[Mh:, T:])
            for n, t in enumerate(ops):
                xa[n, half(i), :] = pad_rows(t.astype(BF)).T

        def after(x, pin):
            if pin is None:
                return x
            never, late = pin
            bits = pltpu.bitcast(x, jnp.uint32)
            late = jnp.tile(pltpu.bitcast(late, jnp.uint32), (bits.shape[0] // 8, bits.shape[1] // T))
            return pltpu.bitcast(jnp.where(never, late, bits), x.dtype)

        def spread(jobs, never, marks, lo, hi):
            for k, job in enumerate(jobs):
                job((never, marks[int(len(marks) * (lo + (hi - lo) * k / len(jobs)))]))

        def c_jobs(i):
            r0 = i * D if isinstance(i, int) else pl.multiple_of(i * D, D)
            o0 = i * T if isinstance(i, int) else pl.multiple_of(i * T, T)

            def job(u, r, pin):
                quad = [after(c[pl.ds(r0 + rh * T + r, 16), ch * Ch + u * T:ch * Ch + (u + 1) * T], pin).astype(F32)
                        for rh in range(2) for ch in range(2)]
                for n, t in enumerate(_lhs7(*quad)):
                    ca[n, u, pl.ds(o0 + r, 16), :] = t.astype(BF)

            return [functools.partial(job, u, r) for u in range(Ch // T) for r in range(0, T, 16)]

        def w_jobs(src, shift, dst):
            k = src.shape[0] // 2

            def job(r, pin):
                quad = [pltpu.bitcast((after(src[kh * k + r:kh * k + r + 16, ch * T:(ch + 1) * T], pin) << shift)
                                      & jnp.uint32(0xFFFF0000), F32) for kh in range(2) for ch in range(2)]
                for n, t in enumerate(_rhs7(*quad)):
                    dst[n, r:r + 16, :] = t.astype(BF)

            return [functools.partial(job, r) for r in range(0, k, 16)]

        def w_ops(w32, shift):
            w = pltpu.bitcast((w32 << shift) & jnp.uint32(0xFFFF0000), F32)
            k = w.shape[0] // 2
            return [t.astype(BF) for t in _rhs7(w[:k, :T], w[:k, T:], w[k:, :T], w[k:, T:])]

        def stage_q_weights(j):
            w = wq[j]
            for e in range(2):
                for n, t in enumerate(w_ops(w, 16 * (1 - e))):
                    wqb[n, :Mh, e * T:(e + 1) * T] = t

        def gate_jobs(i):
            sums = {}

            def job(t, r, pin):
                cols = slice(t * T, (t + 1) * T)
                xt = after(xT[i, r:r + 32, cols], pin).astype(F32)
                for u in range(2):
                    p = xt * vec_s[u, r:r + 32, :]
                    p = (p[0:8] + p[8:16]) + (p[16:24] + p[24:32])
                    sums[u] = p if r == 0 else sums[u] + p
                if r + 32 == M:
                    r_s[i, :, cols] = jnp.sum(sums[0], axis=0, keepdims=True)
                    g_s[i, :, cols] = _sigmoid(jnp.sum(sums[1], axis=0, keepdims=True))

            return [functools.partial(job, t, r) for t in range(2) for r in range(0, M, 32)]

        def init_jobs(i):
            keep = 1.0 - g_s[i]

            def job(r, pin):
                acc[i, r:r + 16, :] = keep * after(xT[i, r:r + 16, :], pin).astype(F32)

            return [functools.partial(job, r) for r in range(0, M, 16)]

        def route():
            r = _cat([r_s[i] for i in range(nb)], axis=1).astype(BF).astype(F32)
            tok = lax.broadcasted_iota(jnp.int32, (1, S), 1)
            rs = jnp.where(r != r, -jnp.inf, r)
            i0 = jnp.min(jnp.where(rs == jnp.max(rs, axis=1, keepdims=True), tok, S), axis=1, keepdims=True)
            rs = jnp.where(tok == i0, -jnp.inf, rs)
            i1 = jnp.min(jnp.where((rs == jnp.max(rs, axis=1, keepdims=True)) & (tok != i0), tok, S),
                         axis=1, keepdims=True)
            lane = lax.broadcasted_iota(jnp.int32, (1, D), 1)
            picks = []
            xsT = jnp.zeros((M, T), F32)
            for u, iv in enumerate((i0, i1)):
                idx = iv[0, 0]
                b = idx >> 8
                hot = lane == (idx & (D - 1))
                w = _sigmoid(jnp.sum(jnp.where(tok == iv, r, 0.0), axis=1, keepdims=True))
                col = jnp.sum(jnp.where(hot, xT[b].astype(F32), 0.0), axis=1, keepdims=True)
                xsT = jnp.where(lane[:, :T] == u, col, xsT)
                picks.append((b, hot, w))
            return xsT.T[:16].astype(BF), picks

        def ffn_up(xs, lo, hi):
            gg = _dot(xs, wg[:, lo:hi])
            uu = _dot(xs, wu[:, lo:hi])
            return (gg * _sigmoid(gg) * uu).astype(BF)

        def ffn_scatter(y, picks):
            yT = _cat([y, jnp.zeros((T - 16, M), F32)], axis=0).T
            for u, (b, hot, w) in enumerate(picks):
                acc[b] += jnp.where(hot, (1.0 - g_s[b]) * (yT[:, u:u + 1] * w), 0.0)

        def q_proj(j, weights, lo, hi):
            r = slice(lo * T, hi * T)
            if qcat:
                m = [None] * 7
                for n in qord:
                    m[n] = _dot(xa[n, r, :], weights(n))
                ms = [[t[:, e * T:(e + 1) * T] for t in m] for e in range(2)]
            else:
                ms = [[None] * 7, [None] * 7]
                for e in range(2):
                    for n in qord:
                        ms[e][n] = _dot(xa[n, r, :], weights(n)[:, e * T:(e + 1) * T])
            for e in range(2):
                q11, q12, q21, q22 = (t * qscale for t in _combine(ms[e], qord, "Q" in defer))
                for n, t in enumerate(_lhs7(q11, q12, q21, q22) + (q12, q21)):
                    qo[2 * j + e, n, r, :] = t.astype(BF)
            return [ms[0][n][r:r + 8] for n in qord for r in range(0, (hi - lo) * T, 16)]

        def head_body(h, _):
            @pl.when(h == 2)
            def _():
                for j in range(2, P):
                    cp_k(j).wait()
                    cp_v(j).wait()

            with scope("head"):
                one_head(h)
            return 0

        def one_head(h):
            never = h >= H
            live = {}
            marks = {"K": [], "V": []}
            last_use = {}
            clock = []

            def tick(x, streams):
                n = max(1, int(x.shape[0] * streams / 64))
                clock.extend(x[(k * (x.shape[0] // 8) // n) * 8:][:8, -T:] for k in range(n))
                return x

            def head_w_jobs(kind, hh):
                shift = ((1 - (hh & 1)) * 16).astype(jnp.uint32)
                return w_jobs((wuk if kind == "K" else wuv).at[hh >> 1], shift, wb.at["KV".index(kind)])

            def wo_job(r, pin):
                quad = [after(woT[h, rh * Mh + r:rh * Mh + r + 16, ch * T:(ch + 1) * T], pin).astype(F32)
                        for rh in range(2) for ch in range(2)]
                for n, t in enumerate(_lhs7(*quad)):
                    wa[n, r:r + 16, :] = t.astype(BF)

            def kv_proj(kind, lo, hi):
                r = slice(lo * T, hi * T)
                m = [None] * 7
                for n in kord:
                    m[n] = _dot(_cat([ca[n, u, r, :] for u in range(Ch // T)], axis=1), wb["KV".index(kind), n])
                    tick(m[n], 4)
                    last_use[kind] = len(clock)
                    marks[kind] += [m[n][t:t + 8] for t in range(0, (hi - lo) * T, 16)]
                    yield 4 * (hi - lo)
                c11, c12, c21, c22 = _combine(m, kord, "K" in defer)
                ops = _rhs7(c11, c21, c12, c22) if kind == "K" else _rhs7(c11, c12, c21, c22)
                dst = ko if kind == "K" else vo
                for n, t in enumerate(ops + (c12, c21)):
                    dst[n, r, :] = t.astype(BF)

            def scores(i):
                r = slice(i * T, (i + 1) * T)
                quad = [[], [], [], []]
                for t0 in range(0, i, schunk):
                    t1 = min(i, t0 + schunk)
                    m = [None] * 7
                    for n in sord:
                        m[n] = tick(_dot_nt(qo[h, n, r, :], ko[n, t0 * T:t1 * T, :]), t1 - t0)
                        yield t1 - t0
                    for lst, s in zip(quad, _combine(m, sord, "S" in defer)):
                        lst += [s[:, t * T:(t + 1) * T] for t in range(t1 - t0)]
                q_top = _cat([qo[h, 2, r, :], qo[h, 7, r, :]], axis=1)
                q_bot = _cat([qo[h, 8, r, :], qo[h, 3, r, :]], axis=1)
                d1 = tick(_dot_nt(_cat([q_top, q_bot], axis=0), _cat([ko[1, r, :], ko[7, r, :]], axis=1)), 3)
                d22 = _dot_nt(q_bot, _cat([ko[8, r, :], ko[4, r, :]], axis=1))
                yield 6
                tri = lax.broadcasted_iota(jnp.int32, (T, T), 1) <= lax.broadcasted_iota(jnp.int32, (T, T), 0)
                dt, db = [jnp.where(tri, d1[:T], -1e9)], [d1[T:], jnp.where(tri, d22, -1e9)]

                def expd(ks, d):
                    tiles = quad[ks[0]] + quad[ks[1]] + d
                    seq = tiles
                    if mxord:
                        ko_ = sorted(ks, key=lambda k: max(sord.index(n) for n in COEF[k]))
                        seq = [quad[k][t] for t0 in range(0, i, schunk) for k in ko_
                               for t in range(t0, min(i, t0 + schunk))] + d
                    mx = jnp.max(functools.reduce(jnp.maximum, seq), axis=1, keepdims=True)
                    return tiles, mx

                live[i] = expd((0, 1), dt), expd((2, 3), db), len(clock)

            def softmax_jobs(i, top, bot):
                sums = {}

                def job(t, r0, pin):
                    rr = slice(r0, r0 + 16)
                    mt, mb = (after(jnp.broadcast_to(x[1][rr], (16, T)), pin) for x in (top, bot))
                    if t < i:
                        ops = _lhs7(jnp.exp2(top[0][t][rr] - mt), jnp.exp2(top[0][i + t][rr] - mt),
                                    jnp.exp2(bot[0][t][rr] - mb), jnp.exp2(bot[0][i + t][rr] - mb))
                        for n, x in enumerate(ops):
                            po[i][n * i + t, rr, :] = x.astype(BF)
                        lt, lb = ops[4], ops[1]
                    else:
                        e = jnp.exp2(top[0][-1][rr] - mt), jnp.exp2(bot[0][-2][rr] - mb), jnp.exp2(bot[0][-1][rr] - mb)
                        for n, x in enumerate(e):
                            po[i][7 * i + n, rr, :] = x.astype(BF)
                        lt, lb = e[0], e[1] + e[2]
                    if t:
                        lt, lb = sums["t"] + lt, sums["b"] + lb
                    sums["t"], sums["b"] = lt, lb
                    if t == i:
                        for u, l in enumerate((lt, lb)):
                            l = jnp.sum(l, axis=1, keepdims=True)
                            rc = pl.reciprocal(l, approx=True)
                            ro[i][u * T + r0:u * T + r0 + 16, :] = jnp.broadcast_to(rc * (2.0 - l * rc), (16, T))

                return [functools.partial(job, t, r0) for r0 in range(0, T, 16) for t in range(i + 1)]

            def pv(i):
                top, bot, since = live.pop(i)
                r = slice(i * T, (i + 1) * T)
                if i in paced:
                    window = clock[since:][-pace_cap:] or clock[-1:]
                    spread(softmax_jobs(i, top, bot), never, window, *spp)
                    ops = [[po[i][n * i + t] for n in range(7)] for t in range(i)]
                    ed = [po[i][7 * i + n] for n in range(3)]
                else:
                    et, eb = ([jnp.exp2(t - x[1]) for t in x[0]] for x in (top, bot))
                    ops = [_lhs7(et[t], et[i + t], eb[t], eb[i + t]) for t in range(i)]
                    ed = [et[-1], eb[-2], eb[-1]]
                m = [None] * 7
                for t0 in range(0, i, pchunk):
                    t1 = min(i, t0 + pchunk)
                    for n in pord:
                        x = _dot(_cat([o[n] for o in ops[t0:t1]], axis=1).astype(BF), vo[n, t0 * T:t1 * T, :])
                        tick(x, t1 - t0)
                        m[n] = x if m[n] is None else m[n] + x
                        yield t1 - t0
                a1 = tick(_dot(_cat(ed[:2], axis=0).astype(BF), _cat([vo[1, r, :], vo[7, r, :]], axis=1)), 3)
                a2 = _dot(ed[2].astype(BF), _cat([vo[8, r, :], vo[4, r, :]], axis=1))
                yield 6
                o = [a1[:T, :T], a1[:T, T:], a1[T:, :T] + a2[:, :T], a1[T:, T:] + a2[:, T:]]
                if i:
                    o = [a + b for a, b in zip(o, _combine(m, pord, "P" in defer))]

                def inv_sum(tiles, late):
                    l = functools.reduce(jnp.add, tiles)
                    if i in dep:
                        l = jnp.where(never, late, l)
                    l = jnp.sum(l, axis=1, keepdims=True)
                    rc = pl.reciprocal(l, approx=True)
                    return rc * (2.0 - l * rc)

                if i in paced:
                    z = pl.multiple_of((h >> 4) * T, T)
                    rt, rb = ro[i][pl.ds(z, T), :], ro[i][pl.ds(z + T, T), :]
                elif lsum:
                    rt = inv_sum([x[4] for x in ops] + et[-1:], o[0])
                    rb = inv_sum([x[1] for x in ops] + eb[-2:], o[3])
                else:
                    rt, rb = inv_sum(et, o[0]), inv_sum(eb, o[3])
                for n, t in enumerate(_rhs7(o[0] * rt, o[2] * rb, o[1] * rt, o[3] * rb)):
                    co[n, r, :] = t.astype(BF)

            def out_proj(lo, hi):
                m = [None] * 7
                for n in oord:
                    m[n] = tick(_dot_nt(wa[n], co[n, lo * T:hi * T, :]), hi - lo)
                    yield 1.75 * (hi - lo)
                for k, a in enumerate(_combine(m, oord, "O" in defer)):
                    rows, cols = slice((k // 2) * Mh, (k // 2 + 1) * Mh), slice((k % 2) * T, (k % 2 + 1) * T)
                    for i in range(lo, hi):
                        x = acc[i, rows, cols] + g_s[i, :, cols] * a[:, (i - lo) * T:(i - lo + 1) * T]
                        acc[i, rows, cols] = x
                        outT[i, rows, cols] = x.astype(BF)
                if early_out:
                    @pl.when(h == H - 1)
                    def _():
                        for i in range(lo, hi):
                            cp_out(i).start()

            def start(op):
                kind, (lo, _, hi) = op[0], op[1:].partition("-")
                lo = int(lo)
                hi = int(hi or lo) + 1
                if kind in "KV":
                    return kv_proj(kind, lo, hi), 28 * (hi - lo)
                if kind == "O":
                    return out_proj(lo, hi), 12.25 * (hi - lo)
                return (scores if kind == "S" else pv)(lo), 7 * lo + 6

            for gi, group in enumerate(prog.split()):
                if "V" in group and not marks["V"]:
                    spread(([] if vnext else head_w_jobs("V", h)) + [functools.partial(wo_job, r) for r in range(0, Mh, 16)],
                           never, marks["K"], *spk)
                lanes = [[*start(op), 0] for op in group.split("+")]
                while lanes:
                    lane = min(lanes, key=lambda l: l[2] / l[1])
                    try:
                        lane[2] += next(lane[0])
                    except StopIteration:
                        lanes.remove(lane)
            for kind in ("KV" if vnext else "K"):
                spread(head_w_jobs(kind, jnp.minimum(h + 1, H - 1)), never, clock[last_use[kind]:], *spv["KV".index(kind)])

        def prologue():
            for i in range(*xchunks[0]):
                cp_x(i).start()
            cp_q(0).start()
            for i in range(xchunks[0][1], nb):
                cp_x(i).start()
            cp_q(1).start()
            for j in range(2, P):
                cp_q(j).start()
                cp_c(j - 2).start()
            cp_c(nb - 2).start()
            cp_c(nb - 1).start()
            for n in (1, 2, 3):
                cp_misc(n).start()
            for j in range(P):
                if j == 2:
                    cp_misc(0).start()
                cp_k(j).start()
                cp_v(j).start()

            with scope("q0"):
                for u, ref in enumerate((wr_ref, gw_ref)):
                    vec_s[u] = jnp.broadcast_to(ref[...].astype(F32).reshape(1, M), (T, M)).T
                wqb[:, Mh:, :] = jnp.zeros((7, D - Mh, D), BF)
                cp_q(0).wait()
                for s, (lo, hi) in enumerate(xchunks):
                    for i in range(lo, hi):
                        cp_x(i).wait()
                    if s == 0:
                        stage_q_weights(0)
                    if s == len(xchunks) - 1:
                        cp_q(1).wait()
                    for i in range(lo, hi):
                        x_ops(i)
                        got = q_proj(0, lambda n: wqb[n], i, i + 1)
                        marks = got if i == lo else marks + got
                stage_q_weights(1)
                never = pl.program_id(0) > 0
                spread(gate_jobs(0) + gate_jobs(nb - 1), never, marks, *sp0)

            def q_body(j, _):
                cp_q(j + 1).wait()
                cp_c(j - 1).wait()
                with scope("q"):
                    marks = []
                    for lo in range(0, nb, qstep):
                        marks += q_proj(j, lambda n: wqb[n], lo, lo + qstep)
                    spread(init_jobs(j - 1) + gate_jobs(j) + c_jobs(j - 1), j >= P, marks, *sp)
                    stage_q_weights(j + 1)
                return 0

            lax.fori_loop(1, P - 1, q_body, 0)

            with scope("q7"):
                cp_c(nb - 2).wait()
                cp_c(nb - 1).wait()
                for n in (1, 2, 3):
                    cp_misc(n).wait()
                for j in range(2):
                    cp_k(j).wait()
                    cp_v(j).wait()
                F = wg.shape[1]
                xs, picks = route()
                q7 = functools.partial(q_proj, P - 1, lambda n: wqb[n])
                marks = q7(0, 2) + q7(2, 4)
                hh = ffn_up(xs, 0, F)
                marks += q7(4, 5)
                y = _dot_nt(hh, wdT[...])
                marks += q7(5, 6) + q7(6, 8)
                jobs = init_jobs(nb - 2) + init_jobs(nb - 1) + c_jobs(nb - 2) + c_jobs(nb - 1)
                jobs += w_jobs(wuk.at[0], 16, wb.at[0]) + (w_jobs(wuv.at[0], 16, wb.at[1]) if vnext else [])
                spread(jobs, never, marks, *sp7)
                ffn_scatter(y, picks)
                cp_misc(0).wait()

        if not head_only:
            prologue()
        if qonly:
            z = pl.program_id(0)
            outT[0, :T, :T] = qo[z, z, :T, :] + ca[z, z, :T, :] + acc[z, :T, :T].astype(BF) + wb[z, 1, :T, :]
        else:
            lax.fori_loop(0, H, head_body, 0)
        if not early_out:
            for i in range(nb):
                cp_out(i).start()
        for i in range(nb):
            cp_out(i).wait()

    def fn(A_x, A_c_kv, A_w_q, A_w_uk, A_w_uv, A_w_o, B_x, B_w_r, B_w_gate, B_w_up, B_w_down, gate_w):
        del B_x
        _, S, M = A_x.shape
        Dc = A_c_kv.shape[2]
        _, H, D = A_w_q.shape
        F = B_w_gate.shape[1]
        nb = S // D
        any_spec = pl.BlockSpec(memory_space=pl.ANY)
        vmem_spec = pl.BlockSpec(memory_space=pltpu.VMEM)
        cp = dict(vmem_limit_bytes=124 * 2**20, disable_bounds_checks=nocheck)
        if flags:
            cp["flags"] = flags
        outT = pl.pallas_call(
            kernel,
            name=name,
            grid=(1,),
            in_specs=[any_spec] * 6 + [vmem_spec] * 2 + [any_spec] * 3,
            out_specs=any_spec,
            out_shape=jax.ShapeDtypeStruct((M, S), BF),
            scratch_shapes=[
                pltpu.VMEM((nb, M, D), BF),
                pltpu.VMEM((7, S // 2, D), BF),
                pltpu.VMEM((S, Dc), BF),
                pltpu.VMEM((7, Dc // D, S // 2, T), BF),
                pltpu.VMEM((H // 2, M, D), jnp.uint32),
                pltpu.VMEM((7, D, D), BF),
                pltpu.VMEM((H // 2, Dc, D), jnp.uint32),
                pltpu.VMEM((H // 2, Dc, D), jnp.uint32),
                pltpu.VMEM((2, 7, Dc // 2, T), BF),
                pltpu.VMEM((H, M, D), BF),
                pltpu.VMEM((7, M // 2, T), BF),
                pltpu.VMEM((M, F), BF),
                pltpu.VMEM((M, F), BF),
                pltpu.VMEM((M, F), BF),
                pltpu.VMEM((H, 9, S // 2, T), BF),
                pltpu.VMEM((9, S // 2, T), BF),
                pltpu.VMEM((9, S // 2, T), BF),
                pltpu.VMEM((7, S // 2, T), BF),
                pltpu.VMEM((2, M, T), F32),
                pltpu.VMEM((nb, 1, D), F32),
                pltpu.VMEM((nb, 1, D), F32),
                pltpu.VMEM((nb, M, D), F32),
                pltpu.VMEM((nb, M, D), BF),
                pltpu.SemaphoreType.DMA((4,)),
                pltpu.SemaphoreType.DMA((len(xchunks),)),
                pltpu.SemaphoreType.DMA((H // 2 + 1,)),
                *[pltpu.VMEM((7 * i + 3, T, T), BF) for i in range(nb)],
                *[pltpu.VMEM((D, T), F32)] * nb,
            ],
            compiler_params=pltpu.CompilerParams(**cp),
        )(A_x[0].T, A_c_kv[0], A_w_q, A_w_uk, A_w_uv, jnp.swapaxes(A_w_o, 1, 2), B_w_r, gate_w,
          B_w_gate, B_w_up, B_w_down.T)
        return outT.T[None]

    return fn


_impl = make(sord=[0, 1, 2, 5, 3, 4, 6],pord=[2, 4, 0, 5, 1, 3, 6],kord=[1, 4, 0, 5, 3, 2, 6],oord=[0, 1, 2, 5, 3, 4, 6],schunk=8,pchunk=8,defer='KOS',dep=[0, 1, 2, 4, 5, 6, 7],lsum=False,mxord=False,prog='K0-3 K4-5+K6-7 S7 V4-5 V6-7 V0-1+V2-3 S5 S6 P7 P6 S4 O6-7 P4+P5 S3 S2 O4-5 S1 P3 S0+P2 P1+P0 O2-3 O0 O1',spk=[0, 0.8],paced=[],vnext=False,spv=[[0.1, 0.2], [0.3, 0.7]],spp=[0.15, 0.9])


@jax.jit
def pallas_gated_mix__compressed_kv_cla__moe_arch_mod__prompt_kernel(
    A_x, A_c_kv, A_w_q, A_w_uk, A_w_uv, A_w_o, B_x, B_w_r, B_w_gate, B_w_up, B_w_down, gate_w,
):
    return _impl(A_x, A_c_kv, A_w_q, A_w_uk, A_w_uv, A_w_o, B_x, B_w_r, B_w_gate, B_w_up, B_w_down, gate_w)
```

```python
import contextlib
import functools
import math

import jax
import jax.numpy as jnp
from jax import lax
import jax.experimental.pallas as pl
import jax.experimental.pallas.tpu as pltpu

BF = jnp.bfloat16
F32 = jnp.float32
T = 128
_NT = (((1,), (1,)), ((), ()))
_cat = jnp.concatenate

PROG = "K0-1 K2-3 K4-5 K6-7 S7 V0-1 V2-3 S6 V4-5 V6-7 P7 S5 P6 O7 S4 P5 O6 S3 P4 O5 S2 P3 O4 S1 P2 O3 S0 P1 P0 O2 O0-1"
COEF = ({0: 1, 3: 1, 4: -1, 6: 1}, {2: 1, 4: 1}, {1: 1, 3: 1}, {0: 1, 1: -1, 2: 1, 5: 1})


def _dot(a, b):
    return jnp.dot(a, b, preferred_element_type=F32)


def _dot_nt(a, b):
    return lax.dot_general(a, b, _NT, preferred_element_type=F32)


def _sigmoid(z):
    return 1.0 / (1.0 + jnp.exp(-z))


def _lhs7(a11, a12, a21, a22):
    return (a11 + a22, a21 + a22, a11, a22, a11 + a12, a21 - a11, a12 - a22)


def _rhs7(b11, b12, b21, b22):
    return (b11 + b22, b11, b12 - b22, b21 - b11, b22, b11 + b12, b21 + b22)


def _combine(m, order, defer):
    out = []
    for k, cf in enumerate(COEF):
        ns = [n for n in order if n in cf]
        if defer and len(ns) == 4:
            ns = ns[::-1] if k == 3 else [ns[2], ns[1], ns[0], ns[3]]
        acc, sign = None, 1
        for n in ns:
            if acc is None:
                acc, sign = m[n], cf[n]
            elif sign > 0:
                acc = acc + m[n] if cf[n] > 0 else acc - m[n]
            elif cf[n] > 0:
                acc, sign = m[n] - acc, 1
            else:
                acc = acc + m[n]
        out.append(acc)
    return out


def make(prog=PROG,  sord=(0, 1, 2, 5, 3, 4, 6), pord=(2, 4, 5, 1, 3, 0, 6),
         kord=(0, 1, 2, 5, 3, 4, 6), oord=(0, 1, 2, 5, 3, 4, 6), qord=(0, 1, 2, 5, 3, 4, 6), schunk=8, pchunk=8,
         defer="SPKOQ", dep=range(8), lsum=False, mxord=False, spk=(0, 0.8), spv=((0.1, 0.3), (0.3, 0.7)), vnext=True, early_out=True, qstep=2,
         qcat=True, head_only=False, nocheck=True, scopes=False, flags=None, ffn_mix=True, sp=(0, 0.72), sp0=(0, 0.75), sp7=(0, 0.97), qonly=False, paced=range(8), spp=(0.15, 0.9), pace_cap=100000, conv_s=(), conv_p=(), plan="A", gather_at=3, name="k7"):
    scope = jax.named_scope if scopes else (lambda n: contextlib.nullcontext())

    stages = {"A": (((0, 1), (0, 1), (0, 0)), ((1, 1), (1, 1), (0, 1)), ((1, 3), (1, 3), (1, 2)), ((3, 6), (3, 6), (2, 5)),
                    ((6, 8), (6, 8), (5, 8))),
              "B": (((0, 1), (0, 1), (0, 0)), ((1, 2), (1, 2), (0, 1)), ((2, 4), (2, 4), (1, 3)), ((4, 8), (4, 8), (3, 8))),
              "C": (((0, 1), (0, 1), (0, 0)), ((1, 3), (1, 3), (0, 2)), ((3, 8), (3, 8), (2, 8))),
              }[plan]
    xchunks = [st[0] for st in stages]

    def kernel(xT_hbm, c_hbm, wq_hbm, wuk_hbm, wuv_hbm, woT_hbm, wr_hbm, gw_hbm, wg_hbm, wu_hbm, wdT_hbm,
               outT_hbm,
               xT, xa, c, ca, wq, wq0b, wqb, wuk, wuv, wb, woT, wa, wg, wu, wdT, qo, ko, vo, co, wr_ref, gw_ref, vec_s, r_s, g_s, acc, outT,
               sem, sem_x, sem_q, *per_block):
        po, ro = per_block[:8], per_block[8:]
        nb, M, _ = xT.shape
        S = nb * 2 * T
        H = qo.shape[0]
        D = 2 * T
        P = H // 2
        Mh = M // 2
        Ch = c.shape[1] // 2
        qscale = (D ** -0.5) * math.log2(math.e)

        wq32 = wq_hbm.bitcast(jnp.uint32)
        wuk32 = wuk_hbm.bitcast(jnp.uint32)
        wuv32 = wuv_hbm.bitcast(jnp.uint32)

        def blk(i):
            return pl.ds(i * D if isinstance(i, int) else pl.multiple_of(i * D, D), D)

        def half(i):
            return pl.ds(i * T if isinstance(i, int) else pl.multiple_of(i * T, T), T)

        def cp_misc(n):
            src, dst = ((woT_hbm, woT), (wg_hbm, wg), (wu_hbm, wu), (wdT_hbm, wdT))[n]
            return pltpu.make_async_copy(src, dst, sem.at[0 if n else 3])

        def cp_x(i):
            return pltpu.make_async_copy(xT_hbm.at[:, blk(i)], xT.at[i], sem_x.at[[lo <= i < hi for lo, hi in xchunks].index(True)])

        def cp_c(i):
            return pltpu.make_async_copy(c_hbm.at[blk(i), :], c.at[blk(i), :], sem_q.at[jnp.minimum(i + 2, P)])

        def cp_q(j):
            return pltpu.make_async_copy(wq32.at[:, j, :], wq.at[j], sem_q.at[j])

        def cp_k(j):
            return pltpu.make_async_copy(wuk32.at[:, j, :], wuk.at[j], sem.at[0 if j < 2 else 2])

        def cp_v(j):
            return pltpu.make_async_copy(wuv32.at[:, j, :], wuv.at[j], sem.at[0 if j < 2 else 2])

        def cp_out(i):
            return pltpu.make_async_copy(outT.at[i], outT_hbm.at[:, blk(i)], sem.at[1])

        def pad_rows(t):
            return _cat([t, jnp.zeros((D - Mh, t.shape[1]), t.dtype)], axis=0)

        def x_ops(i):
            xt = xT[i].astype(F32)
            ops = _lhs7(xt[:Mh, :T], xt[Mh:, :T], xt[:Mh, T:], xt[Mh:, T:])
            for n, t in enumerate(ops):
                xa[n, half(i), :] = pad_rows(t.astype(BF)).T

        def after(x, pin):
            if pin is None:
                return x
            never, late = pin
            bits = pltpu.bitcast(x, jnp.uint32)
            late = pltpu.bitcast(late, jnp.uint32)
            out = _cat([_cat([jnp.where(never, late, bits[r:r + 8, u:u + T]) for u in range(0, bits.shape[1], T)], axis=1)
                        for r in range(0, bits.shape[0], 8)], axis=0)
            return pltpu.bitcast(out, x.dtype)

        def never_set():
            t = xT[0, :16, :T].astype(F32)[:8]
            return t * t < 0.0

        def spread(jobs, never, marks, lo, hi):
            for k, job in enumerate(jobs):
                job((never, marks[int(len(marks) * (lo + (hi - lo) * k / len(jobs)))]))

        def c_jobs(i):
            r0 = i * D if isinstance(i, int) else pl.multiple_of(i * D, D)
            o0 = i * T if isinstance(i, int) else pl.multiple_of(i * T, T)

            def job(u, r, pin):
                quad = [after(c[pl.ds(r0 + rh * T + r, 16), ch * Ch + u * T:ch * Ch + (u + 1) * T], pin).astype(F32)
                        for rh in range(2) for ch in range(2)]
                for n, t in enumerate(_lhs7(*quad)):
                    ca[n, u, pl.ds(o0 + r, 16), :] = t.astype(BF)

            return [functools.partial(job, u, r) for u in range(Ch // T) for r in range(0, T, 16)]

        def w_jobs(src, shift, dst, col=0):
            k = src.shape[0] // 2

            def job(r, pin):
                quad = [pltpu.bitcast((after(src[kh * k + r:kh * k + r + 16, ch * T:(ch + 1) * T], pin) << shift)
                                      & jnp.uint32(0xFFFF0000), F32) for kh in range(2) for ch in range(2)]
                for n, t in enumerate(_rhs7(*quad)):
                    dst[n, r:r + 16, col:col + T] = t.astype(BF)

            return [functools.partial(job, r) for r in range(0, k, 16)]

        def q_weight_jobs(j, dst):
            return [job for pair in zip(*(w_jobs(wq.at[j], 16 * (1 - e), dst, e * T) for e in range(2))) for job in pair]

        def gate_jobs(i):
            sums = {}

            def job(t, r, pin):
                cols = slice(t * T, (t + 1) * T)
                xt = after(xT[i, r:r + 32, cols], pin).astype(F32)
                for u in range(2):
                    p = xt * vec_s[u, r:r + 32, :]
                    p = (p[0:8] + p[8:16]) + (p[16:24] + p[24:32])
                    sums[u] = p if r == 0 else sums[u] + p
                if r + 32 == M:
                    r_s[i, :, cols] = jnp.sum(sums[0], axis=0, keepdims=True)
                    g_s[i, :, cols] = _sigmoid(jnp.sum(sums[1], axis=0, keepdims=True))

            return [functools.partial(job, t, r) for t in range(2) for r in range(0, M, 32)]

        def init_jobs(i):
            keep = []

            def job(r, pin):
                if not keep:
                    keep.append(1.0 - g_s[i])
                acc[i, r:r + 16, :] = keep[0] * after(xT[i, r:r + 16, :], pin).astype(F32)

            return [functools.partial(job, r) for r in range(0, M, 16)]

        def route():
            def whole(op, t):
                return op(op(t, axis=0, keepdims=True), axis=1, keepdims=True)

            r = _cat([r_s[i] for i in range(nb)], axis=0).astype(BF).astype(F32)
            tok = (lax.broadcasted_iota(jnp.int32, (nb, D), 0) * D + lax.broadcasted_iota(jnp.int32, (nb, D), 1))
            bits = pltpu.bitcast(jnp.where(r == 0.0, 0.0, r), jnp.int32) >> 16
            rank = jnp.where(r != r, 0, jnp.where(bits < 0, bits ^ 0x7FFF, bits) + 0x8000)
            key = pltpu.bitcast(0x20000000 + rank * S + (S - 1 - tok), F32)
            lane = lax.broadcasted_iota(jnp.int32, (1, D), 1)
            picks = []
            for _ in range(2):
                best = whole(jnp.max, key)
                idx = S - 1 - (pltpu.bitcast(best, jnp.int32)[0, 0] & (S - 1))
                w = _sigmoid(whole(jnp.sum, jnp.where(key == best, r, 0.0)))
                picks.append((idx >> 8, lane == (idx & (D - 1)), w))
                key = jnp.where(key == best, 0.0, key)
            return picks

        def gather(picks):
            row = lax.broadcasted_iota(jnp.int32, (16, D), 0)
            return sum(_dot_nt(jnp.where((row == u) & hot, 1.0, 0.0).astype(BF), xT[b])
                       for u, (b, hot, _) in enumerate(picks)).astype(BF)

        def ffn_up(xs, lo, hi):
            gg = _dot(xs, wg[:, lo:hi])
            uu = _dot(xs, wu[:, lo:hi])
            return (gg * _sigmoid(gg) * uu).astype(BF)

        def scatter_jobs(y, picks):
            jobs = []
            for u, (b, hot, w) in enumerate(picks):
                col = jnp.broadcast_to(y[u:u + 1] * w, (T, M)).T
                keep = 1.0 - g_s[b]

                def job(r, pin, b=b, hot=hot, col=col, keep=keep):
                    yr = after(col[r:r + 32], pin)
                    acc[b, r:r + 32, :] += jnp.where(hot, keep * _cat([yr, yr], axis=1), 0.0)

                jobs += [functools.partial(job, r) for r in range(0, M, 32)]
            return jobs

        def q_proj(j, weights, lo, hi, extra=None):
            r = slice(lo * T, hi * T)
            if qcat:
                m = [None] * 7
                for k, n in enumerate(qord):
                    if extra is not None:
                        extra(k)
                    m[n] = _dot(xa[n, r, :], weights(n))
                ms = [[t[:, e * T:(e + 1) * T] for t in m] for e in range(2)]
            else:
                ms = [[None] * 7, [None] * 7]
                for e in range(2):
                    for n in qord:
                        ms[e][n] = _dot(xa[n, r, :], weights(n)[:, e * T:(e + 1) * T])
            for e in range(2):
                q11, q12, q21, q22 = (t * qscale for t in _combine(ms[e], qord, "Q" in defer))
                for n, t in enumerate(_lhs7(q11, q12, q21, q22) + (q12, q21)):
                    qo[2 * j + e, n, r, :] = t.astype(BF)
            return [ms[0][n][r:r + 8] for n in qord for r in range(0, (hi - lo) * T, 16)]

        def head_body(h, _):
            @pl.when(h == 2)
            def _():
                for j in range(2, P):
                    cp_k(j).wait()
                    cp_v(j).wait()

            with scope("head"):
                one_head(h)
            return 0

        def one_head(h):
            never = h >= H
            live = {}
            marks = {"K": [], "V": []}
            last_use = {}
            clock = []

            def tick(x, streams):
                n = max(1, int(x.shape[0] * streams / 64))
                clock.extend(x[(k * (x.shape[0] // 8) // n) * 8:][:8, -T:] for k in range(n))
                return x

            def head_w_jobs(kind, hh):
                shift = ((1 - (hh & 1)) * 16).astype(jnp.uint32)
                return w_jobs((wuk if kind == "K" else wuv).at[hh >> 1], shift, wb.at["KV".index(kind)])

            def wo_job(r, pin):
                quad = [after(woT[h, rh * Mh + r:rh * Mh + r + 16, ch * T:(ch + 1) * T], pin).astype(F32)
                        for rh in range(2) for ch in range(2)]
                for n, t in enumerate(_lhs7(*quad)):
                    wa[n, r:r + 16, :] = t.astype(BF)

            def kv_proj(kind, lo, hi):
                r = slice(lo * T, hi * T)
                m = [None] * 7
                for n in kord:
                    m[n] = _dot(_cat([ca[n, u, r, :] for u in range(Ch // T)], axis=1), wb["KV".index(kind), n])
                    tick(m[n], 4)
                    last_use[kind] = len(clock)
                    marks[kind] += [m[n][t:t + 8] for t in range(0, (hi - lo) * T, 16)]
                    yield 4 * (hi - lo)
                c11, c12, c21, c22 = _combine(m, kord, "K" in defer)
                ops = _rhs7(c11, c21, c12, c22) if kind == "K" else _rhs7(c11, c12, c21, c22)
                dst = ko if kind == "K" else vo
                for n, t in enumerate(ops + (c12, c21)):
                    dst[n, r, :] = t.astype(BF)

            def scores(i):
                r = slice(i * T, (i + 1) * T)
                quad = [[], [], [], []]
                q_top = _cat([qo[h, 2, r, :], qo[h, 7, r, :]], axis=1)
                q_bot = _cat([qo[h, 8, r, :], qo[h, 3, r, :]], axis=1)
                if i in conv_s and i:
                    for u, (a, b) in enumerate(((1, 7), (8, 4))):
                        x = _dot_nt(_cat([q_top, q_bot], axis=0), _cat([ko[a, :i * T, :], ko[b, :i * T, :]], axis=1))
                        tick(x, 2 * i)
                        for half_ in range(2):
                            quad[2 * half_ + u] = [x[half_ * T:(half_ + 1) * T, t * T:(t + 1) * T] for t in range(i)]
                        yield 3.5 * i
                for t0 in range(0, 0 if i in conv_s else i, schunk):
                    t1 = min(i, t0 + schunk)
                    m = [None] * 7
                    for n in sord:
                        m[n] = tick(_dot_nt(qo[h, n, r, :], ko[n, t0 * T:t1 * T, :]), t1 - t0)
                        yield t1 - t0
                    for lst, s in zip(quad, _combine(m, sord, "S" in defer)):
                        lst += [s[:, t * T:(t + 1) * T] for t in range(t1 - t0)]
                d1 = tick(_dot_nt(_cat([q_top, q_bot], axis=0), _cat([ko[1, r, :], ko[7, r, :]], axis=1)), 3)
                d22 = _dot_nt(q_bot, _cat([ko[8, r, :], ko[4, r, :]], axis=1))
                yield 6
                tri = lax.broadcasted_iota(jnp.int32, (T, T), 1) <= lax.broadcasted_iota(jnp.int32, (T, T), 0)
                dt, db = [jnp.where(tri, d1[:T], -1e9)], [d1[T:], jnp.where(tri, d22, -1e9)]

                def expd(ks, d):
                    tiles = quad[ks[0]] + quad[ks[1]] + d
                    seq = tiles
                    if mxord:
                        ko_ = sorted(ks, key=lambda k: max(sord.index(n) for n in COEF[k]))
                        seq = [quad[k][t] for t0 in range(0, i, schunk) for k in ko_
                               for t in range(t0, min(i, t0 + schunk))] + d
                    mx = jnp.max(functools.reduce(jnp.maximum, seq), axis=1, keepdims=True)
                    return tiles, mx

                live[i] = expd((0, 1), dt), expd((2, 3), db), len(clock)

            def softmax_jobs(i, top, bot):
                sums = {}

                def job(t, r0, pin):
                    rr = slice(r0, r0 + 16)
                    mt, mb = (after(jnp.broadcast_to(x[1][rr], (16, T)), pin) for x in (top, bot))
                    if t < i:
                        ops = _lhs7(jnp.exp2(top[0][t][rr] - mt), jnp.exp2(top[0][i + t][rr] - mt),
                                    jnp.exp2(bot[0][t][rr] - mb), jnp.exp2(bot[0][i + t][rr] - mb))
                        for n, x in enumerate(ops):
                            po[i][n * i + t, rr, :] = x.astype(BF)
                        lt, lb = ops[4], ops[1]
                    else:
                        e = jnp.exp2(top[0][-1][rr] - mt), jnp.exp2(bot[0][-2][rr] - mb), jnp.exp2(bot[0][-1][rr] - mb)
                        for n, x in enumerate(e):
                            po[i][7 * i + n, rr, :] = x.astype(BF)
                        lt, lb = e[0], e[1] + e[2]
                    if t:
                        lt, lb = sums["t"] + lt, sums["b"] + lb
                    sums["t"], sums["b"] = lt, lb
                    if t == i:
                        for u, l in enumerate((lt, lb)):
                            l = jnp.sum(l, axis=1, keepdims=True)
                            rc = pl.reciprocal(l, approx=True)
                            ro[i][u * T + r0:u * T + r0 + 16, :] = jnp.broadcast_to(rc * (2.0 - l * rc), (16, T))

                return [functools.partial(job, t, r0) for r0 in range(0, T, 16) for t in range(i + 1)]

            def pv(i):
                top, bot, since = live.pop(i)
                r = slice(i * T, (i + 1) * T)
                if i in paced:
                    window = clock[since:][-pace_cap:] or clock[-1:]
                    spread(softmax_jobs(i, top, bot), never, window, *spp)
                    ops = [[po[i][n * i + t] for n in range(7)] for t in range(i)]
                    ed = [po[i][7 * i + n] for n in range(3)]
                else:
                    et, eb = ([jnp.exp2(t - x[1]) for t in x[0]] for x in (top, bot))
                    ops = [_lhs7(et[t], et[i + t], eb[t], eb[i + t]) for t in range(i)]
                    ed = [et[-1], eb[-2], eb[-1]]
                m = [None] * 7
                plain = i in conv_p and i not in paced and i > 0
                if plain:
                    x = None
                    for u, (a, b) in enumerate(((1, 7), (8, 4))):
                        p = _cat([_cat(e[u * i:(u + 1) * i], axis=1) for e in (et, eb)], axis=0).astype(BF)
                        y = tick(_dot(p, _cat([vo[a, :i * T, :], vo[b, :i * T, :]], axis=1)), 2 * i)
                        x = y if x is None else x + y
                        yield 3.5 * i
                for t0 in range(0, 0 if plain else i, pchunk):
                    t1 = min(i, t0 + pchunk)
                    for n in pord:
                        x = _dot(_cat([o[n] for o in ops[t0:t1]], axis=1).astype(BF), vo[n, t0 * T:t1 * T, :])
                        tick(x, t1 - t0)
                        m[n] = x if m[n] is None else m[n] + x
                        yield t1 - t0
                a1 = tick(_dot(_cat(ed[:2], axis=0).astype(BF), _cat([vo[1, r, :], vo[7, r, :]], axis=1)), 3)
                a2 = _dot(ed[2].astype(BF), _cat([vo[8, r, :], vo[4, r, :]], axis=1))
                yield 6
                o = [a1[:T, :T], a1[:T, T:], a1[T:, :T] + a2[:, :T], a1[T:, T:] + a2[:, T:]]
                if plain:
                    o = [a + b for a, b in zip(o, (x[:T, :T], x[:T, T:], x[T:, :T], x[T:, T:]))]
                elif i:
                    o = [a + b for a, b in zip(o, _combine(m, pord, "P" in defer))]

                def inv_sum(tiles, late):
                    l = functools.reduce(jnp.add, tiles)
                    if i in dep:
                        l = jnp.where(never, late, l)
                    l = jnp.sum(l, axis=1, keepdims=True)
                    rc = pl.reciprocal(l, approx=True)
                    return rc * (2.0 - l * rc)

                if i in paced:
                    z = pl.multiple_of((h >> 4) * T, T)
                    rt, rb = ro[i][pl.ds(z, T), :], ro[i][pl.ds(z + T, T), :]
                elif lsum:
                    rt = inv_sum([x[4] for x in ops] + et[-1:], o[0])
                    rb = inv_sum([x[1] for x in ops] + eb[-2:], o[3])
                else:
                    rt, rb = inv_sum(et, o[0]), inv_sum(eb, o[3])
                for n, t in enumerate(_rhs7(o[0] * rt, o[2] * rb, o[1] * rt, o[3] * rb)):
                    co[n, r, :] = t.astype(BF)

            def out_proj(lo, hi):
                m = [None] * 7
                for n in oord:
                    m[n] = tick(_dot_nt(wa[n], co[n, lo * T:hi * T, :]), hi - lo)
                    yield 1.75 * (hi - lo)
                for k, a in enumerate(_combine(m, oord, "O" in defer)):
                    rows, cols = slice((k // 2) * Mh, (k // 2 + 1) * Mh), slice((k % 2) * T, (k % 2 + 1) * T)
                    for i in range(lo, hi):
                        x = acc[i, rows, cols] + g_s[i, :, cols] * a[:, (i - lo) * T:(i - lo + 1) * T]
                        acc[i, rows, cols] = x
                        outT[i, rows, cols] = x.astype(BF)
                if early_out:
                    @pl.when(h == H - 1)
                    def _():
                        for i in range(lo, hi):
                            cp_out(i).start()

            def start(op):
                kind, (lo, _, hi) = op[0], op[1:].partition("-")
                lo = int(lo)
                hi = int(hi or lo) + 1
                if kind in "KV":
                    return kv_proj(kind, lo, hi), 28 * (hi - lo)
                if kind == "O":
                    return out_proj(lo, hi), 12.25 * (hi - lo)
                return (scores if kind == "S" else pv)(lo), 7 * lo + 6

            for gi, group in enumerate(prog.split()):
                if "V" in group and not marks["V"]:
                    spread(([] if vnext else head_w_jobs("V", h)) + [functools.partial(wo_job, r) for r in range(0, Mh, 16)],
                           never, marks["K"], *spk)
                lanes = [[*start(op), 0] for op in group.split("+")]
                while lanes:
                    lane = min(lanes, key=lambda l: l[2] / l[1])
                    try:
                        lane[2] += next(lane[0])
                    except StopIteration:
                        lanes.remove(lane)
            for kind in ("KV" if vnext else "K"):
                spread(head_w_jobs(kind, jnp.minimum(h + 1, H - 1)), never, clock[last_use[kind]:], *spv["KV".index(kind)])

        def prologue():
            cp_vec = [pltpu.make_async_copy(src, dst, sem_q.at[1]) for src, dst in ((wr_hbm, wr_ref), (gw_hbm, gw_ref))]
            cp_x(0).start()
            cp_q(0).start()
            for i in range(1, nb):
                cp_x(i).start()
            cp_q(1).start()
            for cp in cp_vec:
                cp.start()
            for j in range(2, P):
                cp_q(j).start()
                cp_c(j - 2).start()
            cp_c(nb - 2).start()
            cp_c(nb - 1).start()
            for n in (1, 2, 3):
                cp_misc(n).start()
            for j in range(P):
                if j == 2:
                    cp_misc(0).start()
                cp_k(j).start()
                cp_v(j).start()

            with scope("q0"):
                for ref in (wq0b, wqb):
                    ref[:, Mh:, :] = jnp.zeros((7, D - Mh, D), BF)
                for s, (waited, built, done) in enumerate(stages):
                    for i in range(*waited):
                        cp_x(i).wait()
                    if s == 1:
                        cp_q(0).wait()
                        for job in q_weight_jobs(0, wq0b):
                            job(None)
                    if s == len(stages) - 1:
                        cp_q(1).wait()
                        for cp in cp_vec:
                            cp.wait()
                    for i in range(*built):
                        x_ops(i)
                    marks = []
                    for i in range(*done):
                        marks += q_proj(0, lambda n: wq0b[n], i, i + 1)
                for u, ref in enumerate((wr_ref, gw_ref)):
                    vec_s[u] = jnp.broadcast_to(ref[...].astype(F32).reshape(1, M), (T, M)).T
                spread(q_weight_jobs(1, wqb), never_set(), marks, *sp0)

            def q_body(j, _):
                cp_q(j + 1).wait()
                cp_c(j - 1).wait()
                with scope("q"):
                    marks = []
                    for lo in range(0, nb, qstep):
                        marks += q_proj(j, lambda n: wqb[n], lo, lo + qstep)
                    b0 = jnp.minimum(2 * j - 2, nb - 2)
                    spread(gate_jobs(b0) + gate_jobs(b0 + 1) + c_jobs(j - 1) + init_jobs(j - 1), j >= P, marks, *sp)
                    w = wq[j + 1]
                    for e in range(2):
                        we = pltpu.bitcast((w << (16 * (1 - e))) & jnp.uint32(0xFFFF0000), F32)
                        for n, t in enumerate(_rhs7(we[:Mh, :T], we[:Mh, T:], we[Mh:, :T], we[Mh:, T:])):
                            wqb[n, :Mh, e * T:(e + 1) * T] = t.astype(BF)
                return 0

            lax.fori_loop(1, P - 1, q_body, 0)

            with scope("q7"):
                cp_c(nb - 2).wait()
                cp_c(nb - 1).wait()
                for n in (1, 2, 3):
                    cp_misc(n).wait()
                for j in range(2):
                    cp_k(j).wait()
                    cp_v(j).wait()
                F = wg.shape[1]
                picks = route()
                never = never_set()
                q7 = functools.partial(q_proj, P - 1, lambda n: wqb[n])
                if ffn_mix:
                    up, parts, xsl = [], [], []

                    def up_tiles(k):
                        up.append(_dot(xs, (wg, wu)[k % 2][:, (k // 2) * T:(k // 2 + 1) * T]))

                    def down_tiles(k):
                        gg, uu = up[2 * k], up[2 * k + 1]
                        parts.append(_dot_nt((gg * _sigmoid(gg) * uu).astype(BF), wdT[:, k * T:(k + 1) * T]))

                    marks = q7(0, 1)
                    marks += q7(1, 2, lambda k: xsl.append(gather(picks)) if k == gather_at else None)
                    xs = xsl[0]
                    for i in range(2, 5):
                        marks += q7(i, i + 1, lambda k, i=i: [up_tiles(t) for t in range(
                            (7 * (i - 2) + k) * 28 // 21, (7 * (i - 2) + k + 1) * 28 // 21)])
                    for i in range(5, 7):
                        marks += q7(i, i + 1, lambda k, i=i: down_tiles(7 * (i - 5) + k))
                    y = functools.reduce(jnp.add, parts)
                    tail = q7(7, 8)
                jobs = init_jobs(nb - 2) + init_jobs(nb - 1) + c_jobs(nb - 2) + c_jobs(nb - 1)
                jobs += w_jobs(wuk.at[0], 16, wb.at[0]) + (w_jobs(wuv.at[0], 16, wb.at[1]) if vnext else [])
                spread(jobs, never, marks, *sp7)
                spread(scatter_jobs(y, picks), never, tail, 0.3, 0.9)
                cp_misc(0).wait()

        if not head_only:
            prologue()
        if qonly:
            z = pl.program_id(0)
            outT[0, :T, :T] = qo[z, z, :T, :] + ca[z, z, :T, :] + acc[z, :T, :T].astype(BF) + wb[z, 1, :T, :]
        else:
            lax.fori_loop(0, H, head_body, 0)
        if not early_out:
            for i in range(nb):
                cp_out(i).start()
        for i in range(nb):
            cp_out(i).wait()

    def fn(A_x, A_c_kv, A_w_q, A_w_uk, A_w_uv, A_w_o, B_x, B_w_r, B_w_gate, B_w_up, B_w_down, gate_w):
        del B_x
        _, S, M = A_x.shape
        Dc = A_c_kv.shape[2]
        _, H, D = A_w_q.shape
        F = B_w_gate.shape[1]
        nb = S // D
        any_spec = pl.BlockSpec(memory_space=pl.ANY)
        cp = dict(vmem_limit_bytes=124 * 2**20, disable_bounds_checks=nocheck, disable_semaphore_checks=nocheck)
        if flags:
            cp["flags"] = flags
        outT = pl.pallas_call(
            kernel,
            name=name,
            in_specs=[any_spec] * 11,
            out_specs=any_spec,
            out_shape=jax.ShapeDtypeStruct((M, S), BF),
            scratch_shapes=[
                pltpu.VMEM((nb, M, D), BF),
                pltpu.VMEM((7, S // 2, D), BF),
                pltpu.VMEM((S, Dc), BF),
                pltpu.VMEM((7, Dc // D, S // 2, T), BF),
                pltpu.VMEM((H // 2, M, D), jnp.uint32),
                pltpu.VMEM((7, D, D), BF),
                pltpu.VMEM((7, D, D), BF),
                pltpu.VMEM((H // 2, Dc, D), jnp.uint32),
                pltpu.VMEM((H // 2, Dc, D), jnp.uint32),
                pltpu.VMEM((2, 7, Dc // 2, T), BF),
                pltpu.VMEM((H, M, D), BF),
                pltpu.VMEM((7, M // 2, T), BF),
                pltpu.VMEM((M, F), BF),
                pltpu.VMEM((M, F), BF),
                pltpu.VMEM((M, F), BF),
                pltpu.VMEM((H, 9, S // 2, T), BF),
                pltpu.VMEM((9, S // 2, T), BF),
                pltpu.VMEM((9, S // 2, T), BF),
                pltpu.VMEM((7, S // 2, T), BF),
                pltpu.VMEM((M,), BF),
                pltpu.VMEM((M,), BF),
                pltpu.VMEM((2, M, T), F32),
                pltpu.VMEM((nb, 1, D), F32),
                pltpu.VMEM((nb, 1, D), F32),
                pltpu.VMEM((nb, M, D), F32),
                pltpu.VMEM((nb, M, D), BF),
                pltpu.SemaphoreType.DMA((4,)),
                pltpu.SemaphoreType.DMA((len(xchunks),)),
                pltpu.SemaphoreType.DMA((H // 2 + 1,)),
                *[pltpu.VMEM((7 * i + 3, T, T), BF) for i in range(nb)],
                *[pltpu.VMEM((D, T), F32)] * nb,
            ],
            compiler_params=pltpu.CompilerParams(**cp),
        )(A_x[0].T, A_c_kv[0], A_w_q, A_w_uk, A_w_uv, jnp.swapaxes(A_w_o, 1, 2), B_w_r, gate_w,
          B_w_gate, B_w_up, B_w_down.T)
        return outT.T[None]

    return fn


_impl = make(sord=[0, 1, 2, 5, 3, 4, 6],pord=[2, 4, 0, 5, 1, 3, 6],kord=[1, 4, 0, 5, 3, 2, 6],oord=[0, 1, 2, 5, 3, 4, 6],schunk=8,pchunk=8,defer='KOS',dep=[0, 1, 2, 4, 5, 6, 7],lsum=False,mxord=False,prog='K0-3 K4-5+K6-7 S7 V4-5 V6-7 V0-1+V2-3 S5 S6 P7 P6 S4 O6-7 P4+P5 S3 S2 O4-5 S1 P3 S0+P2 P1+P0 O2-3 O0 O1',spk=[0, 0.8],paced=[],vnext=False,spv=[[0.1, 0.2], [0.3, 0.7]],spp=[0.15, 0.9],plan='A',sp0=(0.05,0.95),sp=(0,0.8),gather_at=1)


@jax.jit
def pallas_gated_mix__compressed_kv_cla__moe_arch_mod__prompt_kernel(
    A_x, A_c_kv, A_w_q, A_w_uk, A_w_uv, A_w_o, B_x, B_w_r, B_w_gate, B_w_up, B_w_down, gate_w,
):
    return _impl(A_x, A_c_kv, A_w_q, A_w_uk, A_w_uv, A_w_o, B_x, B_w_r, B_w_gate, B_w_up, B_w_down, gate_w)
```

```python
import contextlib
import functools
import math

import jax
import jax.numpy as jnp
from jax import lax
import jax.experimental.pallas as pl
import jax.experimental.pallas.tpu as pltpu

BF = jnp.bfloat16
F32 = jnp.float32
T = 128
_NT = (((1,), (1,)), ((), ()))
_cat = jnp.concatenate

PROG = "K0-1 K2-3 K4-5 K6-7 S7 V0-1 V2-3 S6 V4-5 V6-7 P7 S5 P6 O7 S4 P5 O6 S3 P4 O5 S2 P3 O4 S1 P2 O3 S0 P1 P0 O2 O0-1"
COEF = ({0: 1, 3: 1, 4: -1, 6: 1}, {2: 1, 4: 1}, {1: 1, 3: 1}, {0: 1, 1: -1, 2: 1, 5: 1})


def _dot(a, b):
    return jnp.dot(a, b, preferred_element_type=F32)


def _dot_nt(a, b):
    return lax.dot_general(a, b, _NT, preferred_element_type=F32)


def _sigmoid(z):
    return 1.0 / (1.0 + jnp.exp(-z))


def _lhs7(a11, a12, a21, a22):
    return (a11 + a22, a21 + a22, a11, a22, a11 + a12, a21 - a11, a12 - a22)


def _rhs7(b11, b12, b21, b22):
    return (b11 + b22, b11, b12 - b22, b21 - b11, b22, b11 + b12, b21 + b22)


def _combine(m, order, defer):
    out = []
    for k, cf in enumerate(COEF):
        ns = [n for n in order if n in cf]
        if defer and len(ns) == 4:
            ns = ns[::-1] if k == 3 else [ns[2], ns[1], ns[0], ns[3]]
        acc, sign = None, 1
        for n in ns:
            if acc is None:
                acc, sign = m[n], cf[n]
            elif sign > 0:
                acc = acc + m[n] if cf[n] > 0 else acc - m[n]
            elif cf[n] > 0:
                acc, sign = m[n] - acc, 1
            else:
                acc = acc + m[n]
        out.append(acc)
    return out


def make(prog=PROG,  sord=(0, 1, 2, 5, 3, 4, 6), pord=(2, 4, 5, 1, 3, 0, 6),
         kord=(0, 1, 2, 5, 3, 4, 6), oord=(0, 1, 2, 5, 3, 4, 6), qord=(0, 1, 2, 5, 3, 4, 6), schunk=8, pchunk=8,
         defer="SPKOQ", dep=range(8), lsum=False, mxord=False, spk=(0, 0.8), spv=((0.1, 0.3), (0.3, 0.7)), vnext=True, early_out=True, qstep=2,
         qcat=True, head_only=False, nocheck=True, scopes=False, flags=None, ffn_mix=True, sp=(0, 0.72), sp0=(0, 0.75), sp7=(0, 0.97), qonly=False, paced=range(8), spp=(0.15, 0.9), pace_cap=100000, conv_s=(), conv_p=(), plan="A", gather_at=3, jit=(), lead=24, qcopy=True, qjob=64, q32=True, name="k8"):
    scope = jax.named_scope if scopes else (lambda n: contextlib.nullcontext())

    stages = {"A": (((0, 1), (0, 1), (0, 0)), ((1, 1), (1, 1), (0, 1)), ((1, 3), (1, 3), (1, 2)), ((3, 6), (3, 6), (2, 5)),
                    ((6, 8), (6, 8), (5, 8))),
              "B": (((0, 1), (0, 1), (0, 0)), ((1, 2), (1, 2), (0, 1)), ((2, 4), (2, 4), (1, 3)), ((4, 8), (4, 8), (3, 8))),
              "C": (((0, 1), (0, 1), (0, 0)), ((1, 3), (1, 3), (0, 2)), ((3, 8), (3, 8), (2, 8))),
              }[plan]
    xchunks = [st[0] for st in stages]

    def kernel(xT_hbm, c_hbm, wq_hbm, wuk_hbm, wuv_hbm, woT_hbm, wr_hbm, gw_hbm, wg_hbm, wu_hbm, wdT_hbm,
               outT_hbm,
               xT, xa, c, ca, wq, wq0b, wqb, wuk, wuv, wb, woT, wa, wg, wu, wdT, qo, qs, ko, vo, co, wr_ref, gw_ref, vec_s, r_s, g_s, acc, outT,
               sem, sem_x, sem_q, *per_block):
        po, ro = per_block[:8], per_block[8:]
        nb, M, _ = xT.shape
        S = nb * 2 * T
        H = qo.shape[0]
        D = 2 * T
        P = H // 2
        Mh = M // 2
        Ch = c.shape[1] // 2
        qscale = (D ** -0.5) * math.log2(math.e)

        wq32 = wq_hbm.bitcast(jnp.uint32)
        wuk32 = wuk_hbm.bitcast(jnp.uint32)
        wuv32 = wuv_hbm.bitcast(jnp.uint32)

        def blk(i):
            return pl.ds(i * D if isinstance(i, int) else pl.multiple_of(i * D, D), D)

        def half(i):
            return pl.ds(i * T if isinstance(i, int) else pl.multiple_of(i * T, T), T)

        def cp_misc(n):
            src, dst = ((woT_hbm, woT), (wg_hbm, wg), (wu_hbm, wu), (wdT_hbm, wdT))[n]
            return pltpu.make_async_copy(src, dst, sem.at[0 if n else 3])

        def cp_x(i):
            return pltpu.make_async_copy(xT_hbm.at[:, blk(i)], xT.at[i], sem_x.at[[lo <= i < hi for lo, hi in xchunks].index(True)])

        def cp_c(i):
            return pltpu.make_async_copy(c_hbm.at[blk(i), :], c.at[blk(i), :], sem_q.at[jnp.minimum(i + 2, P)])

        def cp_q(j):
            return pltpu.make_async_copy(wq32.at[:, j, :], wq.at[j], sem_q.at[j])

        def cp_k(j):
            return pltpu.make_async_copy(wuk32.at[:, j, :], wuk.at[j], sem.at[0 if j < 2 else 2])

        def cp_v(j):
            return pltpu.make_async_copy(wuv32.at[:, j, :], wuv.at[j], sem.at[0 if j < 2 else 2])

        def cp_out(i):
            return pltpu.make_async_copy(outT.at[i], outT_hbm.at[:, blk(i)], sem.at[1])

        def pad_rows(t):
            return _cat([t, jnp.zeros((D - Mh, t.shape[1]), t.dtype)], axis=0)

        def x_ops(i):
            xt = xT[i].astype(F32)
            ops = _lhs7(xt[:Mh, :T], xt[Mh:, :T], xt[:Mh, T:], xt[Mh:, T:])
            for n, t in enumerate(ops):
                xa[n, half(i), :] = pad_rows(t.astype(BF)).T

        def after(x, pin):
            if pin is None:
                return x
            never, late = pin
            bits = pltpu.bitcast(x, jnp.uint32)
            late = pltpu.bitcast(late, jnp.uint32)
            out = _cat([_cat([jnp.where(never, late, bits[r:r + 8, u:u + T]) for u in range(0, bits.shape[1], T)], axis=1)
                        for r in range(0, bits.shape[0], 8)], axis=0)
            return pltpu.bitcast(out, x.dtype)

        def never_set():
            t = xT[0, :16, :T].astype(F32)[:8]
            return t * t < 0.0

        def spread(jobs, never, marks, lo, hi):
            for k, job in enumerate(jobs):
                job((never, marks[int(len(marks) * (lo + (hi - lo) * k / len(jobs)))]))

        def c_jobs(i):
            r0 = i * D if isinstance(i, int) else pl.multiple_of(i * D, D)
            o0 = i * T if isinstance(i, int) else pl.multiple_of(i * T, T)

            def job(u, r, pin):
                quad = [after(c[pl.ds(r0 + rh * T + r, 16), ch * Ch + u * T:ch * Ch + (u + 1) * T], pin).astype(F32)
                        for rh in range(2) for ch in range(2)]
                for n, t in enumerate(_lhs7(*quad)):
                    ca[n, u, pl.ds(o0 + r, 16), :] = t.astype(BF)

            return [functools.partial(job, u, r) for u in range(Ch // T) for r in range(0, T, 16)]

        def w_jobs(src, shift, dst, col=0):
            k = src.shape[0] // 2

            def job(r, pin):
                quad = [pltpu.bitcast((after(src[kh * k + r:kh * k + r + 16, ch * T:(ch + 1) * T], pin) << shift)
                                      & jnp.uint32(0xFFFF0000), F32) for kh in range(2) for ch in range(2)]
                for n, t in enumerate(_rhs7(*quad)):
                    dst[n, r:r + 16, col:col + T] = t.astype(BF)

            return [functools.partial(job, r) for r in range(0, k, 16)]

        def q_weight_jobs(j, dst):
            return [job for pair in zip(*(w_jobs(wq.at[j], 16 * (1 - e), dst, e * T) for e in range(2))) for job in pair]

        def gate_jobs(i):
            sums = {}

            def job(t, r, pin):
                cols = slice(t * T, (t + 1) * T)
                xt = after(xT[i, r:r + 32, cols], pin).astype(F32)
                for u in range(2):
                    p = xt * vec_s[u, r:r + 32, :]
                    p = (p[0:8] + p[8:16]) + (p[16:24] + p[24:32])
                    sums[u] = p if r == 0 else sums[u] + p
                if r + 32 == M:
                    r_s[i, :, cols] = jnp.sum(sums[0], axis=0, keepdims=True)
                    g_s[i, :, cols] = _sigmoid(jnp.sum(sums[1], axis=0, keepdims=True))

            return [functools.partial(job, t, r) for t in range(2) for r in range(0, M, 32)]

        def init_jobs(i):
            keep = []

            def job(r, pin):
                if not keep:
                    keep.append(1.0 - g_s[i])
                acc[i, r:r + 16, :] = keep[0] * after(xT[i, r:r + 16, :], pin).astype(F32)

            return [functools.partial(job, r) for r in range(0, M, 16)]

        def route():
            def whole(op, t):
                return op(op(t, axis=0, keepdims=True), axis=1, keepdims=True)

            r = _cat([r_s[i] for i in range(nb)], axis=0).astype(BF).astype(F32)
            tok = (lax.broadcasted_iota(jnp.int32, (nb, D), 0) * D + lax.broadcasted_iota(jnp.int32, (nb, D), 1))
            bits = pltpu.bitcast(jnp.where(r == 0.0, 0.0, r), jnp.int32) >> 16
            rank = jnp.where(r != r, 0, jnp.where(bits < 0, bits ^ 0x7FFF, bits) + 0x8000)
            key = pltpu.bitcast(0x20000000 + rank * S + (S - 1 - tok), F32)
            lane = lax.broadcasted_iota(jnp.int32, (1, D), 1)
            picks = []
            for _ in range(2):
                best = whole(jnp.max, key)
                idx = S - 1 - (pltpu.bitcast(best, jnp.int32)[0, 0] & (S - 1))
                w = _sigmoid(whole(jnp.sum, jnp.where(key == best, r, 0.0)))
                picks.append((idx >> 8, lane == (idx & (D - 1)), w))
                key = jnp.where(key == best, 0.0, key)
            return picks

        def gather(picks):
            row = lax.broadcasted_iota(jnp.int32, (16, D), 0)
            return sum(_dot_nt(jnp.where((row == u) & hot, 1.0, 0.0).astype(BF), xT[b])
                       for u, (b, hot, _) in enumerate(picks)).astype(BF)

        def ffn_up(xs, lo, hi):
            gg = _dot(xs, wg[:, lo:hi])
            uu = _dot(xs, wu[:, lo:hi])
            return (gg * _sigmoid(gg) * uu).astype(BF)

        def scatter_jobs(y, picks):
            jobs = []
            for u, (b, hot, w) in enumerate(picks):
                col = jnp.broadcast_to(y[u:u + 1] * w, (T, M)).T
                keep = 1.0 - g_s[b]

                def job(r, pin, b=b, hot=hot, col=col, keep=keep):
                    yr = after(col[r:r + 32], pin)
                    acc[b, r:r + 32, :] += jnp.where(hot, keep * _cat([yr, yr], axis=1), 0.0)

                jobs += [functools.partial(job, r) for r in range(0, M, 32)]
            return jobs

        def q_proj(j, weights, lo, hi, extra=None):
            r = slice(lo * T, hi * T)
            if qcat:
                m = [None] * 7
                for k, n in enumerate(qord):
                    if extra is not None:
                        extra(k)
                    m[n] = _dot(xa[n, r, :], weights(n))
                ms = [[t[:, e * T:(e + 1) * T] for t in m] for e in range(2)]
            else:
                ms = [[None] * 7, [None] * 7]
                for e in range(2):
                    for n in qord:
                        ms[e][n] = _dot(xa[n, r, :], weights(n)[:, e * T:(e + 1) * T])
            for e in range(2):
                q11, q12, q21, q22 = (t * qscale for t in _combine(ms[e], qord, "Q" in defer))
                for n, t in enumerate(_lhs7(q11, q12, q21, q22) + (q12, q21)):
                    qo[2 * j + e, n, r, :] = t.astype(BF)
            return [ms[0][n][r:r + 8] for n in qord for r in range(0, (hi - lo) * T, 16)]

        def head_body(h, _):
            @pl.when(h == 2)
            def _():
                for j in range(2, P):
                    cp_k(j).wait()
                    cp_v(j).wait()

            with scope("head"):
                one_head(h)
            return 0

        def one_head(h):
            never = h >= H
            live = {}
            marks = {"K": [], "V": []}
            last_use = {}
            qr = qs if qcopy else qo.at[h]
            staged = []

            def q_job(n, r0, pin):
                if q32:
                    rr = slice(r0 // 2, (r0 + qjob) // 2)
                    qs.bitcast(jnp.uint32)[n, rr, :] = after(qo.bitcast(jnp.uint32)[h, n, rr, :], pin)
                else:
                    qs[n, r0:r0 + qjob, :] = after(qo[h, n, r0:r0 + qjob, :], pin)
            clock = []

            def tick(x, streams):
                n = max(1, int(x.shape[0] * streams / 64))
                clock.extend(x[(k * (x.shape[0] // 8) // n) * 8:][:8, -T:] for k in range(n))
                return x

            def head_w_jobs(kind, hh):
                shift = ((1 - (hh & 1)) * 16).astype(jnp.uint32)
                return w_jobs((wuk if kind == "K" else wuv).at[hh >> 1], shift, wb.at["KV".index(kind)])

            def wo_job(r, pin):
                quad = [after(woT[h, rh * Mh + r:rh * Mh + r + 16, ch * T:(ch + 1) * T], pin).astype(F32)
                        for rh in range(2) for ch in range(2)]
                for n, t in enumerate(_lhs7(*quad)):
                    wa[n, r:r + 16, :] = t.astype(BF)

            def kv_proj(kind, lo, hi):
                r = slice(lo * T, hi * T)
                m = [None] * 7
                for n in kord:
                    m[n] = _dot(_cat([ca[n, u, r, :] for u in range(Ch // T)], axis=1), wb["KV".index(kind), n])
                    tick(m[n], 4)
                    last_use[kind] = len(clock)
                    marks[kind] += [m[n][t:t + 8] for t in range(0, (hi - lo) * T, 16)]
                    yield 4 * (hi - lo)
                c11, c12, c21, c22 = _combine(m, kord, "K" in defer)
                ops = _rhs7(c11, c21, c12, c22) if kind == "K" else _rhs7(c11, c12, c21, c22)
                dst = ko if kind == "K" else vo
                for n, t in enumerate(ops + (c12, c21)):
                    dst[n, r, :] = t.astype(BF)

            def scores(i):
                r = slice(i * T, (i + 1) * T)
                quad = [[], [], [], []]
                q_top = _cat([qr[2, r, :], qr[7, r, :]], axis=1)
                q_bot = _cat([qr[8, r, :], qr[3, r, :]], axis=1)
                if i in conv_s and i:
                    for u, (a, b) in enumerate(((1, 7), (8, 4))):
                        x = _dot_nt(_cat([q_top, q_bot], axis=0), _cat([ko[a, :i * T, :], ko[b, :i * T, :]], axis=1))
                        tick(x, 2 * i)
                        for half_ in range(2):
                            quad[2 * half_ + u] = [x[half_ * T:(half_ + 1) * T, t * T:(t + 1) * T] for t in range(i)]
                        yield 3.5 * i
                for t0 in range(0, 0 if i in conv_s else i, schunk):
                    t1 = min(i, t0 + schunk)
                    m = [None] * 7
                    for n in sord:
                        m[n] = tick(_dot_nt(qr[n, r, :], ko[n, t0 * T:t1 * T, :]), t1 - t0)
                        yield t1 - t0
                    for lst, s in zip(quad, _combine(m, sord, "S" in defer)):
                        lst += [s[:, t * T:(t + 1) * T] for t in range(t1 - t0)]
                d1 = tick(_dot_nt(_cat([q_top, q_bot], axis=0), _cat([ko[1, r, :], ko[7, r, :]], axis=1)), 3)
                d22 = _dot_nt(q_bot, _cat([ko[8, r, :], ko[4, r, :]], axis=1))
                yield 6
                tri = lax.broadcasted_iota(jnp.int32, (T, T), 1) <= lax.broadcasted_iota(jnp.int32, (T, T), 0)
                dt, db = [jnp.where(tri, d1[:T], -1e9)], [d1[T:], jnp.where(tri, d22, -1e9)]

                def expd(ks, d):
                    tiles = quad[ks[0]] + quad[ks[1]] + d
                    seq = tiles
                    if mxord:
                        ko_ = sorted(ks, key=lambda k: max(sord.index(n) for n in COEF[k]))
                        seq = [quad[k][t] for t0 in range(0, i, schunk) for k in ko_
                               for t in range(t0, min(i, t0 + schunk))] + d
                    mx = jnp.max(functools.reduce(jnp.maximum, seq), axis=1, keepdims=True)
                    return tiles, mx

                live[i] = expd((0, 1), dt), expd((2, 3), db), len(clock)

            def softmax_jobs(i, top, bot):
                sums = {}

                def job(t, r0, pin):
                    rr = slice(r0, r0 + 16)
                    mt, mb = (after(jnp.broadcast_to(x[1][rr], (16, T)), pin) for x in (top, bot))
                    if t < i:
                        ops = _lhs7(jnp.exp2(top[0][t][rr] - mt), jnp.exp2(top[0][i + t][rr] - mt),
                                    jnp.exp2(bot[0][t][rr] - mb), jnp.exp2(bot[0][i + t][rr] - mb))
                        for n, x in enumerate(ops):
                            po[i][n * i + t, rr, :] = x.astype(BF)
                        lt, lb = ops[4], ops[1]
                    else:
                        e = jnp.exp2(top[0][-1][rr] - mt), jnp.exp2(bot[0][-2][rr] - mb), jnp.exp2(bot[0][-1][rr] - mb)
                        for n, x in enumerate(e):
                            po[i][7 * i + n, rr, :] = x.astype(BF)
                        lt, lb = e[0], e[1] + e[2]
                    if t:
                        lt, lb = sums["t"] + lt, sums["b"] + lb
                    sums["t"], sums["b"] = lt, lb
                    if t == i:
                        for u, l in enumerate((lt, lb)):
                            l = jnp.sum(l, axis=1, keepdims=True)
                            rc = pl.reciprocal(l, approx=True)
                            ro[i][u * T + r0:u * T + r0 + 16, :] = jnp.broadcast_to(rc * (2.0 - l * rc), (16, T))

                return [functools.partial(job, t, r0) for r0 in range(0, T, 16) for t in range(i + 1)]

            def pv(i):
                top, bot, since = live.pop(i)
                r = slice(i * T, (i + 1) * T)
                if i in paced:
                    window = clock[since:][-pace_cap:] or clock[-1:]
                    spread(softmax_jobs(i, top, bot), never, window, *spp)
                    ops = [[po[i][n * i + t] for n in range(7)] for t in range(i)]
                    ed = [po[i][7 * i + n] for n in range(3)]
                elif i in jit:
                    done, sums = {}, {}

                    def quadrant(k):
                        if k not in done:
                            src = ([(0, -1), (1, -2), (1, -1)] if k == 4
                                   else [(k // 2, (k % 2) * i + t) for t in range(i)])
                            done[k] = []
                            for t, (u, idx) in enumerate(src):
                                tiles, mx = (top, bot)[u]
                                rows = []
                                for r0 in range(0, T, 16):
                                    at = min(len(clock) - 1, max(since - 1, len(clock) - lead + (t // 4) * 8 + r0 // 16))
                                    rows.append(jnp.exp2(tiles[idx][r0:r0 + 16] - after(
                                        jnp.broadcast_to(mx[r0:r0 + 16], (16, T)), (never, clock[at]))))
                                e = _cat(rows, axis=0)
                                done[k].append(e)
                                sums[u] = sums[u] + e if u in sums else e
                        return done[k]

                    class Lazy:
                        def __init__(self, t):
                            self.t = t

                        def __getitem__(self, n):
                            need = ((0, 3), (2, 3), (0,), (3,), (0, 1), (2, 0), (1, 3))[n]
                            x = [quadrant(k)[self.t] for k in need]
                            return x[0] if len(x) == 1 else (x[0] + x[1] if n < 5 else x[0] - x[1])

                    ops = [Lazy(t) for t in range(i)]
                else:
                    et, eb = ([jnp.exp2(t - x[1]) for t in x[0]] for x in (top, bot))
                    ops = [_lhs7(et[t], et[i + t], eb[t], eb[i + t]) for t in range(i)]
                    ed = [et[-1], eb[-2], eb[-1]]
                m = [None] * 7
                plain = i in conv_p and i not in paced and i > 0
                if plain:
                    x = None
                    for u, (a, b) in enumerate(((1, 7), (8, 4))):
                        p = _cat([_cat(e[u * i:(u + 1) * i], axis=1) for e in (et, eb)], axis=0).astype(BF)
                        y = tick(_dot(p, _cat([vo[a, :i * T, :], vo[b, :i * T, :]], axis=1)), 2 * i)
                        x = y if x is None else x + y
                        yield 3.5 * i
                for t0 in range(0, 0 if plain else i, pchunk):
                    t1 = min(i, t0 + pchunk)
                    for n in pord:
                        x = _dot(_cat([o[n] for o in ops[t0:t1]], axis=1).astype(BF), vo[n, t0 * T:t1 * T, :])
                        tick(x, t1 - t0)
                        m[n] = x if m[n] is None else m[n] + x
                        yield t1 - t0
                if i in jit and i not in paced:
                    ed = quadrant(4)
                    for u in range(2):
                        l = jnp.sum(sums[u], axis=1, keepdims=True)
                        rc = pl.reciprocal(l, approx=True)
                        ro[i][u * T:(u + 1) * T, :] = jnp.broadcast_to(rc * (2.0 - l * rc), (T, T))
                a1 = tick(_dot(_cat(ed[:2], axis=0).astype(BF), _cat([vo[1, r, :], vo[7, r, :]], axis=1)), 3)
                a2 = _dot(ed[2].astype(BF), _cat([vo[8, r, :], vo[4, r, :]], axis=1))
                yield 6
                o = [a1[:T, :T], a1[:T, T:], a1[T:, :T] + a2[:, :T], a1[T:, T:] + a2[:, T:]]
                if plain:
                    o = [a + b for a, b in zip(o, (x[:T, :T], x[:T, T:], x[T:, :T], x[T:, T:]))]
                elif i:
                    o = [a + b for a, b in zip(o, _combine(m, pord, "P" in defer))]

                def inv_sum(tiles, late):
                    l = functools.reduce(jnp.add, tiles)
                    if i in dep:
                        l = jnp.where(never, late, l)
                    l = jnp.sum(l, axis=1, keepdims=True)
                    rc = pl.reciprocal(l, approx=True)
                    return rc * (2.0 - l * rc)

                if i in paced or i in jit:
                    z = pl.multiple_of((h >> 4) * T, T)
                    rt, rb = ro[i][pl.ds(z, T), :], ro[i][pl.ds(z + T, T), :]
                elif lsum:
                    rt = inv_sum([x[4] for x in ops] + et[-1:], o[0])
                    rb = inv_sum([x[1] for x in ops] + eb[-2:], o[3])
                else:
                    rt, rb = inv_sum(et, o[0]), inv_sum(eb, o[3])
                for n, t in enumerate(_rhs7(o[0] * rt, o[2] * rb, o[1] * rt, o[3] * rb)):
                    co[n, r, :] = t.astype(BF)

            def out_proj(lo, hi):
                m = [None] * 7
                for n in oord:
                    m[n] = tick(_dot_nt(wa[n], co[n, lo * T:hi * T, :]), hi - lo)
                    yield 1.75 * (hi - lo)
                for k, a in enumerate(_combine(m, oord, "O" in defer)):
                    rows, cols = slice((k // 2) * Mh, (k // 2 + 1) * Mh), slice((k % 2) * T, (k % 2 + 1) * T)
                    for i in range(lo, hi):
                        x = acc[i, rows, cols] + g_s[i, :, cols] * a[:, (i - lo) * T:(i - lo + 1) * T]
                        acc[i, rows, cols] = x
                        outT[i, rows, cols] = x.astype(BF)
                if early_out:
                    @pl.when(h == H - 1)
                    def _():
                        for i in range(lo, hi):
                            cp_out(i).start()

            def start(op):
                kind, (lo, _, hi) = op[0], op[1:].partition("-")
                lo = int(lo)
                hi = int(hi or lo) + 1
                if kind in "KV":
                    return kv_proj(kind, lo, hi), 28 * (hi - lo)
                if kind == "O":
                    return out_proj(lo, hi), 12.25 * (hi - lo)
                return (scores if kind == "S" else pv)(lo), 7 * lo + 6

            for gi, group in enumerate(prog.split()):
                if ("V" in group or "S" in group) and not staged:
                    staged.append(True)
                    jobs = [functools.partial(q_job, n, r0) for r0 in range(S // 2 - qjob, -1, -qjob) for n in range(9)] if qcopy else []
                    spread(jobs, never, marks["K"], 0, 0.5)
                    jobs = ([] if vnext else head_w_jobs("V", h)) + [functools.partial(wo_job, r) for r in range(0, Mh, 16)]
                    spread(jobs, never, marks["K"], *spk)
                lanes = [[*start(op), 0] for op in group.split("+")]
                with (jax.named_scope("g" + group) if scopes == 2 else contextlib.nullcontext()):
                    while lanes:
                        lane = min(lanes, key=lambda l: l[2] / l[1])
                        try:
                            lane[2] += next(lane[0])
                        except StopIteration:
                            lanes.remove(lane)
            for kind in ("KV" if vnext else "K"):
                spread(head_w_jobs(kind, jnp.minimum(h + 1, H - 1)), never, clock[last_use[kind]:], *spv["KV".index(kind)])

        def prologue():
            cp_vec = [pltpu.make_async_copy(src, dst, sem_q.at[1]) for src, dst in ((wr_hbm, wr_ref), (gw_hbm, gw_ref))]
            cp_x(0).start()
            cp_q(0).start()
            for i in range(1, nb):
                cp_x(i).start()
            cp_q(1).start()
            for cp in cp_vec:
                cp.start()
            for j in range(2, P):
                cp_q(j).start()
                cp_c(j - 2).start()
            cp_c(nb - 2).start()
            cp_c(nb - 1).start()
            for n in (1, 2, 3):
                cp_misc(n).start()
            for j in range(P):
                if j == 2:
                    cp_misc(0).start()
                cp_k(j).start()
                cp_v(j).start()

            with scope("q0"):
                for ref in (wq0b, wqb):
                    ref[:, Mh:, :] = jnp.zeros((7, D - Mh, D), BF)
                for s, (waited, built, done) in enumerate(stages):
                    for i in range(*waited):
                        cp_x(i).wait()
                    if s == 1:
                        cp_q(0).wait()
                        for job in q_weight_jobs(0, wq0b):
                            job(None)
                    if s == len(stages) - 1:
                        cp_q(1).wait()
                        for cp in cp_vec:
                            cp.wait()
                    for i in range(*built):
                        x_ops(i)
                    marks = []
                    for i in range(*done):
                        marks += q_proj(0, lambda n: wq0b[n], i, i + 1)
                for u, ref in enumerate((wr_ref, gw_ref)):
                    vec_s[u] = jnp.broadcast_to(ref[...].astype(F32).reshape(1, M), (T, M)).T
                spread(q_weight_jobs(1, wqb), never_set(), marks, *sp0)

            def q_body(j, _):
                cp_q(j + 1).wait()
                cp_c(j - 1).wait()
                with scope("q"):
                    marks = []
                    for lo in range(0, nb, qstep):
                        marks += q_proj(j, lambda n: wqb[n], lo, lo + qstep)
                    b0 = jnp.minimum(2 * j - 2, nb - 2)
                    spread(gate_jobs(b0) + gate_jobs(b0 + 1) + c_jobs(j - 1) + init_jobs(j - 1), j >= P, marks, *sp)
                    w = wq[j + 1]
                    for e in range(2):
                        we = pltpu.bitcast((w << (16 * (1 - e))) & jnp.uint32(0xFFFF0000), F32)
                        for n, t in enumerate(_rhs7(we[:Mh, :T], we[:Mh, T:], we[Mh:, :T], we[Mh:, T:])):
                            wqb[n, :Mh, e * T:(e + 1) * T] = t.astype(BF)
                return 0

            lax.fori_loop(1, P - 1, q_body, 0)

            with scope("q7"):
                cp_c(nb - 2).wait()
                cp_c(nb - 1).wait()
                for n in (1, 2, 3):
                    cp_misc(n).wait()
                for j in range(2):
                    cp_k(j).wait()
                    cp_v(j).wait()
                F = wg.shape[1]
                picks = route()
                never = never_set()
                q7 = functools.partial(q_proj, P - 1, lambda n: wqb[n])
                if ffn_mix:
                    up, parts, xsl = [], [], []

                    def up_tiles(k):
                        up.append(_dot(xs, (wg, wu)[k % 2][:, (k // 2) * T:(k // 2 + 1) * T]))

                    def down_tiles(k):
                        gg, uu = up[2 * k], up[2 * k + 1]
                        parts.append(_dot_nt((gg * _sigmoid(gg) * uu).astype(BF), wdT[:, k * T:(k + 1) * T]))

                    marks = q7(0, 1)
                    marks += q7(1, 2, lambda k: xsl.append(gather(picks)) if k == gather_at else None)
                    xs = xsl[0]
                    for i in range(2, 5):
                        marks += q7(i, i + 1, lambda k, i=i: [up_tiles(t) for t in range(
                            (7 * (i - 2) + k) * 28 // 21, (7 * (i - 2) + k + 1) * 28 // 21)])
                    for i in range(5, 7):
                        marks += q7(i, i + 1, lambda k, i=i: down_tiles(7 * (i - 5) + k))
                    y = functools.reduce(jnp.add, parts)
                    tail = q7(7, 8)
                jobs = init_jobs(nb - 2) + init_jobs(nb - 1) + c_jobs(nb - 2) + c_jobs(nb - 1)
                jobs += w_jobs(wuk.at[0], 16, wb.at[0]) + (w_jobs(wuv.at[0], 16, wb.at[1]) if vnext else [])
                spread(jobs, never, marks, *sp7)
                spread(scatter_jobs(y, picks), never, tail, 0.3, 0.9)
                cp_misc(0).wait()

        if not head_only:
            prologue()
        if qonly:
            z = pl.program_id(0)
            outT[0, :T, :T] = qo[z, z, :T, :] + ca[z, z, :T, :] + acc[z, :T, :T].astype(BF) + wb[z, 1, :T, :]
        else:
            lax.fori_loop(0, H, head_body, 0)
        if not early_out:
            for i in range(nb):
                cp_out(i).start()
        for i in range(nb):
            cp_out(i).wait()

    def fn(A_x, A_c_kv, A_w_q, A_w_uk, A_w_uv, A_w_o, B_x, B_w_r, B_w_gate, B_w_up, B_w_down, gate_w):
        del B_x
        _, S, M = A_x.shape
        Dc = A_c_kv.shape[2]
        _, H, D = A_w_q.shape
        F = B_w_gate.shape[1]
        nb = S // D
        any_spec = pl.BlockSpec(memory_space=pl.ANY)
        cp = dict(vmem_limit_bytes=124 * 2**20, disable_bounds_checks=nocheck, disable_semaphore_checks=nocheck)
        if flags:
            cp["flags"] = flags
        outT = pl.pallas_call(
            kernel,
            name=name,
            in_specs=[any_spec] * 11,
            out_specs=any_spec,
            out_shape=jax.ShapeDtypeStruct((M, S), BF),
            scratch_shapes=[
                pltpu.VMEM((nb, M, D), BF),
                pltpu.VMEM((7, S // 2, D), BF),
                pltpu.VMEM((S, Dc), BF),
                pltpu.VMEM((7, Dc // D, S // 2, T), BF),
                pltpu.VMEM((H // 2, M, D), jnp.uint32),
                pltpu.VMEM((7, D, D), BF),
                pltpu.VMEM((7, D, D), BF),
                pltpu.VMEM((H // 2, Dc, D), jnp.uint32),
                pltpu.VMEM((H // 2, Dc, D), jnp.uint32),
                pltpu.VMEM((2, 7, Dc // 2, T), BF),
                pltpu.VMEM((H, M, D), BF),
                pltpu.VMEM((7, M // 2, T), BF),
                pltpu.VMEM((M, F), BF),
                pltpu.VMEM((M, F), BF),
                pltpu.VMEM((M, F), BF),
                pltpu.VMEM((H, 9, S // 2, T), BF),
                pltpu.VMEM((9, S // 2, T), BF),
                pltpu.VMEM((9, S // 2, T), BF),
                pltpu.VMEM((9, S // 2, T), BF),
                pltpu.VMEM((7, S // 2, T), BF),
                pltpu.VMEM((M,), BF),
                pltpu.VMEM((M,), BF),
                pltpu.VMEM((2, M, T), F32),
                pltpu.VMEM((nb, 1, D), F32),
                pltpu.VMEM((nb, 1, D), F32),
                pltpu.VMEM((nb, M, D), F32),
                pltpu.VMEM((nb, M, D), BF),
                pltpu.SemaphoreType.DMA((4,)),
                pltpu.SemaphoreType.DMA((len(xchunks),)),
                pltpu.SemaphoreType.DMA((H // 2 + 1,)),
                *[pltpu.VMEM((7 * i + 3, T, T), BF) for i in range(nb)],
                *[pltpu.VMEM((D, T), F32)] * nb,
            ],
            compiler_params=pltpu.CompilerParams(**cp),
        )(A_x[0].T, A_c_kv[0], A_w_q, A_w_uk, A_w_uv, jnp.swapaxes(A_w_o, 1, 2), B_w_r, gate_w,
          B_w_gate, B_w_up, B_w_down.T)
        return outT.T[None]

    return fn


_impl = make(sord=[0, 1, 2, 5, 3, 4, 6],pord=[2, 4, 0, 5, 1, 3, 6],kord=[4, 1, 0, 5, 3, 2, 6],oord=[0, 1, 2, 5, 3, 4, 6],schunk=8,pchunk=8,defer='KOPS',dep=[0, 1, 4, 5, 6, 7],lsum=False,mxord=True,prog='K0-3 K4-5+K6 K7 S7 V4-5+V6-7 S5 S6 V0-1+V2-3 P7 P6 S4 O6-7 S3 P4+P5 S1 P3 O4-5 S2 S0+P2 P1+P0 O2-3 O1 O0',spk=[0.5, 0.9],paced=[],vnext=False,spv=[[0.08, 0.16], [0.3, 0.7]],spp=[0.15, 0.9],jit=[4, 5],lead=32,plan='A',sp0=(0.05,0.95),sp=(0,0.8),gather_at=1)


@jax.jit
def pallas_gated_mix__compressed_kv_cla__moe_arch_mod__prompt_kernel(
    A_x, A_c_kv, A_w_q, A_w_uk, A_w_uv, A_w_o, B_x, B_w_r, B_w_gate, B_w_up, B_w_down, gate_w,
):
    return _impl(A_x, A_c_kv, A_w_q, A_w_uk, A_w_uv, A_w_o, B_x, B_w_r, B_w_gate, B_w_up, B_w_down, gate_w)
```

```python
import functools
import math

import jax
import jax.numpy as jnp
from jax import lax
import jax.experimental.pallas as pl
import jax.experimental.pallas.tpu as pltpu

BF = jnp.bfloat16
F32 = jnp.float32
U32 = jnp.uint32
T = 128
_cat = jnp.concatenate

_HEAD_PROGRAM = "K0-3 K4-5+K6 K7 S7 V4-5+V6-7 S5 S6 V0-1+V2-3 P7 P6 S4 O6-7 S3 P4+P5 S1 P3 O4-5 S2 S0+P2 P1+P0 O2-3 O1 O0"
_FIRST_PASS = (((0, 1), (0, 0)), ((1, 1), (0, 1)), ((1, 3), (1, 2)), ((3, 6), (2, 5)), ((6, 8), (5, 8)))

_LHS = ((0, 1, 3), (2, 1, 3), (0,), (3,), (0, 1, 1), (2, -1, 0), (1, -1, 3))
_RHS = ((0, 1, 3), (0,), (1, -1, 3), (2, -1, 0), (3,), (0, 1, 1), (2, 1, 3))
_OUT = ({0: 1, 3: 1, 4: -1, 6: 1}, {2: 1, 4: 1}, {1: 1, 3: 1}, {0: 1, 1: -1, 2: 1, 5: 1})


def _operand(rule, quadrant):
    if len(rule) == 1:
        return quadrant(rule[0])
    a, b = quadrant(rule[0]), quadrant(rule[2])
    return a + b if rule[1] > 0 else a - b


def _operands(rules, quads):
    return tuple(_operand(rule, quads.__getitem__) for rule in rules)


def _combine(m, order):
    out = []
    for k, signs in enumerate(_OUT):
        ns = [n for n in order if n in signs]
        if len(ns) == 4:
            ns = ns[::-1] if k == 3 else [ns[2], ns[1], ns[0], ns[3]]
        acc, sign = m[ns[0]], signs[ns[0]]
        for n in ns[1:]:
            if sign > 0:
                acc = acc + m[n] if signs[n] > 0 else acc - m[n]
            else:
                acc, sign = m[n] - acc, 1
        out.append(acc)
    return out


def _dot(a, b):
    return jnp.dot(a, b, preferred_element_type=F32)


def _dot_nt(a, b):
    return lax.dot_general(a, b, (((1,), (1,)), ((), ())), preferred_element_type=F32)


def _sigmoid(z):
    return 1.0 / (1.0 + jnp.exp(-z))


def _inverse_row_sum(partial_sums):
    l = jnp.sum(partial_sums, axis=1, keepdims=True)
    r = pl.reciprocal(l, approx=True)
    return r * (2.0 - l * r)


def _after(x, pin):
    if pin is None:
        return x
    never, late = pin
    bits, late = pltpu.bitcast(x, U32), pltpu.bitcast(late, U32)
    out = _cat([_cat([jnp.where(never, late, bits[r:r + 8, u:u + T]) for u in range(0, bits.shape[1], T)], axis=1)
                for r in range(0, bits.shape[0], 8)], axis=0)
    return pltpu.bitcast(out, x.dtype)


def _spread(jobs, never, marks, lo, hi):
    for k, job in enumerate(jobs):
        job((never, marks[int(len(marks) * (lo + (hi - lo) * k / len(jobs)))]))


def make(prog=_HEAD_PROGRAM, qord=(0, 1, 2, 5, 3, 4, 6), kord=(4, 1, 0, 5, 3, 2, 6), sord=(0, 1, 2, 5, 3, 4, 6),
         pord=(2, 4, 0, 5, 1, 3, 6), oord=(0, 1, 2, 5, 3, 4, 6), late_sum=(0, 1, 4, 5, 6, 7), timed_exp=(4, 5), lead=32,
         spk=(0.5, 0.9), spv=(0.08, 0.16), qjob=64, head_only=False, nocheck=True, name="kf"):
    def kernel(xT_hbm, c_hbm, wq_hbm, wuk_hbm, wuv_hbm, woT_hbm, wr_hbm, gw_hbm, wg_hbm, wu_hbm, wdT_hbm, outT_hbm,
               xT, c, wq, wuk, wuv, woT, wr, gw, wg, wu, wdT,
               x7, c7, wq7_first, wq7, wkv7, wo7, q_all, q9, k9, v9, ctx7,
               vec_cols, score, gate, acc, outT, sem, sem_x, sem_q, *inv_sums):
        nb, M, D = xT.shape
        S, H = nb * D, q_all.shape[0]
        P, Mh, Ch = H // 2, M // 2, c.shape[1] // 2
        q_scale = D ** -0.5 * math.log2(math.e)

        def start_of(i, size):
            return i * size if isinstance(i, int) else pl.multiple_of(i * size, size)

        def cp_x(i):
            group = [lo <= i < hi for (lo, hi), _ in _FIRST_PASS].index(True)
            return pltpu.make_async_copy(xT_hbm.at[:, pl.ds(i * D, D)], xT.at[i], sem_x.at[group])

        def cp_q(j):
            return pltpu.make_async_copy(wq_hbm.bitcast(U32).at[:, j, :], wq.at[j], sem_q.at[j])

        def cp_c(i):
            rows = pl.ds(start_of(i, D), D)
            slot = min(i + 2, P) if isinstance(i, int) else i + 2
            return pltpu.make_async_copy(c_hbm.at[rows, :], c.at[rows, :], sem_q.at[slot])

        def cp_vectors():
            return [pltpu.make_async_copy(src, dst, sem_q.at[1]) for src, dst in ((wr_hbm, wr), (gw_hbm, gw))]

        def cp_kv(pairs, slot):
            return [pltpu.make_async_copy(src.bitcast(U32).at[:, j, :], dst.at[j], sem.at[slot])
                    for j in pairs for src, dst in ((wuk_hbm, wuk), (wuv_hbm, wuv))]

        def cp_early():
            ffn = ((wg_hbm, wg), (wu_hbm, wu), (wdT_hbm, wdT))
            return [pltpu.make_async_copy(src, dst, sem.at[0]) for src, dst in ffn] + cp_kv(range(2), 0)

        def cp_wo():
            return pltpu.make_async_copy(woT_hbm, woT, sem.at[1])

        def cp_late():
            return cp_kv(range(2, P), 2)

        def cp_out(i):
            return pltpu.make_async_copy(outT.at[i], outT_hbm.at[:, pl.ds(i * D, D)], sem.at[3])

        def build_x7(i):
            xt = xT[i].astype(F32)
            pad = jnp.zeros((D - Mh, T), F32)
            quads = [_cat([t, pad], axis=0).T for t in (xt[:Mh, :T], xt[Mh:, :T], xt[:Mh, T:], xt[Mh:, T:])]
            for n, t in enumerate(_operands(_LHS, quads)):
                x7[n, i * T:(i + 1) * T, :] = t.astype(BF)

        def c7_jobs(i):
            src, dst = start_of(i, D), start_of(i, T)

            def job(u, r, pin):
                quads = [_after(c[pl.ds(src + rh * T + r, 16), ch * Ch + u * T:ch * Ch + (u + 1) * T], pin).astype(F32)
                         for rh in range(2) for ch in range(2)]
                for n, t in enumerate(_operands(_LHS, quads)):
                    c7[n, u, pl.ds(dst + r, 16), :] = t.astype(BF)

            return [functools.partial(job, u, r) for u in range(Ch // T) for r in range(0, T, 16)]

        def weight_jobs(words, shift, dst, col=0):
            k = words.shape[0] // 2

            def job(r, pin):
                quads = [pltpu.bitcast((_after(words[kh * k + r:kh * k + r + 16, ch * T:(ch + 1) * T], pin) << shift)
                                       & U32(0xFFFF0000), F32) for kh in range(2) for ch in range(2)]
                for n, t in enumerate(_operands(_RHS, quads)):
                    dst[n, r:r + 16, col:col + T] = t.astype(BF)

            return [functools.partial(job, r) for r in range(0, k, 16)]

        def wq7_jobs(j, dst):
            heads = [weight_jobs(wq.at[j], 16 * (1 - e), dst, e * T) for e in range(2)]
            return [job for both in zip(*heads) for job in both]

        def gate_jobs(i):
            sums = {}

            def job(t, r, pin):
                cols = slice(t * T, (t + 1) * T)
                xt = _after(xT[i, r:r + 32, cols], pin).astype(F32)
                for u in range(2):
                    p = xt * vec_cols[u, r:r + 32, :]
                    p = (p[0:8] + p[8:16]) + (p[16:24] + p[24:32])
                    sums[u] = p if r == 0 else sums[u] + p
                if r + 32 == M:
                    score[i, :, cols] = jnp.sum(sums[0], axis=0, keepdims=True)
                    gate[i, :, cols] = _sigmoid(jnp.sum(sums[1], axis=0, keepdims=True))

            return [functools.partial(job, t, r) for t in range(2) for r in range(0, M, 32)]

        def residual_jobs(i):
            keep = []

            def job(r, pin):
                if not keep:
                    keep.append(1.0 - gate[i])
                acc[i, r:r + 16, :] = keep[0] * _after(xT[i, r:r + 16, :], pin).astype(F32)

            return [functools.partial(job, r) for r in range(0, M, 16)]

        def route():
            def whole(op, t):
                return op(op(t, axis=0, keepdims=True), axis=1, keepdims=True)

            r = _cat([score[i] for i in range(nb)], axis=0).astype(BF).astype(F32)
            tok = lax.broadcasted_iota(jnp.int32, (nb, D), 0) * D + lax.broadcasted_iota(jnp.int32, (nb, D), 1)
            bits = pltpu.bitcast(jnp.where(r == 0.0, 0.0, r), jnp.int32) >> 16
            rank = jnp.where(r != r, 0, jnp.where(bits < 0, bits ^ 0x7FFF, bits) + 0x8000)
            key = pltpu.bitcast(0x20000000 + rank * S + (S - 1 - tok), F32)
            lane = lax.broadcasted_iota(jnp.int32, (1, D), 1)
            picks = []
            for _ in range(2):
                best = whole(jnp.max, key)
                idx = S - 1 - (pltpu.bitcast(best, jnp.int32)[0, 0] & (S - 1))
                weight = _sigmoid(whole(jnp.sum, jnp.where(key == best, r, 0.0)))
                picks.append((idx >> (D.bit_length() - 1), lane == (idx & (D - 1)), weight))
                key = jnp.where(key == best, 0.0, key)
            return picks

        def gather(picks):
            row = lax.broadcasted_iota(jnp.int32, (16, D), 0)
            return sum(_dot_nt(jnp.where((row == u) & hot, 1.0, 0.0).astype(BF), xT[b])
                       for u, (b, hot, _) in enumerate(picks)).astype(BF)

        def scatter_jobs(y, picks):
            def job(b, hot, col, keep, r, pin):
                yr = _after(col[r:r + 32], pin)
                acc[b, r:r + 32, :] += jnp.where(hot, keep * _cat([yr, yr], axis=1), 0.0)

            jobs = []
            for u, (b, hot, weight) in enumerate(picks):
                col = jnp.broadcast_to(y[u:u + 1] * weight, (T, M)).T
                keep = 1.0 - gate[b]
                jobs += [functools.partial(job, b, hot, col, keep, r) for r in range(0, M, 32)]
            return jobs

        def q_proj(j, w7, lo, hi, before=None):
            m = [None] * 7
            for k, n in enumerate(qord):
                if before is not None:
                    before(k)
                m[n] = _dot(x7[n, lo * T:hi * T, :], w7[n])
            for e in range(2):
                q = [t * q_scale for t in _combine([t[:, e * T:(e + 1) * T] for t in m], qord)]
                for n, t in enumerate(_operands(_LHS, q) + (q[1], q[2])):
                    q_all[2 * j + e, n, lo * T:hi * T, :] = t.astype(BF)
            return [m[n][r:r + 8, :T] for n in qord for r in range(0, (hi - lo) * T, 16)]

        def never_set():
            t = xT[0, :16, :T].astype(F32)[:8]
            return t * t < 0.0

        def first_pair():
            for ref in (wq7_first, wq7):
                ref[:, Mh:, :] = jnp.zeros((7, D - Mh, D), BF)
            for s, (arrived, projected) in enumerate(_FIRST_PASS):
                for i in range(*arrived):
                    cp_x(i).wait()
                if s == 1:
                    cp_q(0).wait()
                    for job in wq7_jobs(0, wq7_first):
                        job(None)
                if s == len(_FIRST_PASS) - 1:
                    for cp in [cp_q(1)] + cp_vectors():
                        cp.wait()
                for i in range(*arrived):
                    build_x7(i)
                marks = [t for i in range(*projected) for t in q_proj(0, wq7_first, i, i + 1)]
            for u, ref in enumerate((wr, gw)):
                vec_cols[u] = jnp.broadcast_to(ref[...].astype(F32).reshape(1, M), (T, M)).T
            _spread(wq7_jobs(1, wq7), never_set(), marks, 0.05, 0.95)

        def middle_pair(j, carry):
            cp_q(j + 1).wait()
            cp_c(j - 1).wait()
            never = j >= P
            marks = q_proj(j, wq7, 0, nb)
            b = jnp.minimum(2 * j - 2, nb - 2)
            _spread(gate_jobs(b) + gate_jobs(b + 1) + c7_jobs(j - 1) + residual_jobs(j - 1), never, marks, 0, 0.45)

            def next_weights(n, r, pin):
                for e in range(2):
                    def quadrant(k):
                        rows, cols = slice(k // 2 * Mh + r, k // 2 * Mh + r + 16), slice(k % 2 * T, (k % 2 + 1) * T)
                        w = _after(wq[j + 1, rows, cols], pin)
                        return pltpu.bitcast(w & U32(0xFFFF0000) if e else w << 16, F32)

                    wq7[n, r:r + 16, e * T:(e + 1) * T] = _operand(_RHS[n], quadrant).astype(BF)

            for k, n in enumerate(qord):
                jobs = [functools.partial(next_weights, n, r) for r in range(0, Mh, 16)]
                _spread(jobs, never, marks, k / 7 + 0.005, k / 7 + 0.1)
            return carry

        def last_pair():
            for cp in [cp_c(nb - 2), cp_c(nb - 1)] + cp_early():
                cp.wait()
            picks, never = route(), never_set()
            slabs = wg.shape[1] // T
            xs, hidden, y = [], [], []

            def take(k):
                if k == 1:
                    xs.append(gather(picks))

            def up(step, k):
                for t in range((step + k) * 2 * slabs // 21, (step + k + 1) * 2 * slabs // 21):
                    hidden.append(_dot(xs[0], (wg, wu)[t % 2][:, t // 2 * T:(t // 2 + 1) * T]))

            def down(step, k):
                for t in range((step + k) * slabs // 14, (step + k + 1) * slabs // 14):
                    g, u = hidden[2 * t], hidden[2 * t + 1]
                    y.append(_dot_nt((g * _sigmoid(g) * u).astype(BF), wdT[:, t * T:(t + 1) * T]))

            extras = ([None, take] + [functools.partial(up, 7 * s) for s in range(3)]
                      + [functools.partial(down, 7 * s) for s in range(2)])
            marks = [t for i, extra in enumerate(extras) for t in q_proj(P - 1, wq7, i, i + 1, extra)]
            y = functools.reduce(jnp.add, y)
            tail = q_proj(P - 1, wq7, nb - 1, nb)
            jobs = residual_jobs(nb - 2) + residual_jobs(nb - 1) + c7_jobs(nb - 2) + c7_jobs(nb - 1)
            _spread(jobs + weight_jobs(wuk.at[0], 16, wkv7.at[0]), never, marks, 0, 0.97)
            _spread(scatter_jobs(y, picks), never, tail, 0.3, 0.9)
            cp_wo().wait()

        def head(h, carry):
            @pl.when(h == 2)
            def _():
                for cp in cp_late():
                    cp.wait()

            never = h >= H
            clock, k_marks, scores_of, keys_done = [], [], {}, []

            def tick(x, tiles):
                n = max(1, x.shape[0] * tiles // 64)
                clock.extend(x[(k * (x.shape[0] // 8) // n) * 8:][:8, -T:] for k in range(n))
                return x

            def kv_weight_jobs(u, hh):
                shift = ((1 - (hh & 1)) * 16).astype(U32)
                return weight_jobs((wuk, wuv)[u].at[hh >> 1], shift, wkv7.at[u])

            def wo_job(r, pin):
                quads = [_after(woT[h, rh * Mh + r:rh * Mh + r + 16, ch * T:(ch + 1) * T], pin).astype(F32)
                         for rh in range(2) for ch in range(2)]
                for n, t in enumerate(_operands(_LHS, quads)):
                    wo7[n, r:r + 16, :] = t.astype(BF)

            def q_job(n, r, pin):
                rows = slice(r // 2, (r + qjob) // 2)
                q9.bitcast(U32)[n, rows, :] = _after(q_all.bitcast(U32)[h, n, rows, :], pin)

            def kv_proj(u, lo, hi):
                r = slice(lo * T, hi * T)
                m = [None] * 7
                for n in kord:
                    m[n] = tick(_dot(_cat([c7[n, t, r, :] for t in range(Ch // T)], axis=1), wkv7[u, n]), 4)
                    if u == 0:
                        k_marks.extend(m[n][t:t + 8] for t in range(0, (hi - lo) * T, 16))
                        keys_done.append(len(clock))
                    yield 4 * (hi - lo)
                a = _combine(m, kord)
                ops = _operands(_RHS, a if u else (a[0], a[2], a[1], a[3]))
                for n, t in enumerate(ops + (a[1], a[2])):
                    (k9, v9)[u][n, r, :] = t.astype(BF)

            def scores(i):
                r = slice(i * T, (i + 1) * T)
                q_top, q_bot = _cat([q9[2, r, :], q9[7, r, :]], axis=1), _cat([q9[8, r, :], q9[3, r, :]], axis=1)
                past = [[], [], [], []]
                if i:
                    m = [None] * 7
                    for n in sord:
                        m[n] = tick(_dot_nt(q9[n, r, :], k9[n, :i * T, :]), i)
                        yield i
                    past = [[s[:, t * T:(t + 1) * T] for t in range(i)] for s in _combine(m, sord)]
                d1 = tick(_dot_nt(_cat([q_top, q_bot], axis=0), _cat([k9[1, r, :], k9[7, r, :]], axis=1)), 3)
                d2 = _dot_nt(q_bot, _cat([k9[8, r, :], k9[4, r, :]], axis=1))
                yield 6
                causal = lax.broadcasted_iota(jnp.int32, (T, T), 1) <= lax.broadcasted_iota(jnp.int32, (T, T), 0)
                diagonal = [jnp.where(causal, d1[:T], -1e9)], [d1[T:], jnp.where(causal, d2, -1e9)]
                rows = []
                for u in range(2):
                    first, second = sorted((2 * u, 2 * u + 1), key=lambda k: max(sord.index(n) for n in _OUT[k]))
                    row_max = functools.reduce(jnp.maximum, past[first] + past[second] + diagonal[u])
                    rows.append((past[2 * u] + past[2 * u + 1] + diagonal[u],
                                 jnp.max(row_max, axis=1, keepdims=True)))
                scores_of[i] = rows, len(clock)

            def attend(i):
                rows, since = scores_of.pop(i)
                r = slice(i * T, (i + 1) * T)
                exps, sums = {}, {}

                def timed(k):
                    if k not in exps:
                        exps[k] = []
                        where = [(0, -1), (1, -2), (1, -1)] if k == 4 else [(k // 2, k % 2 * i + t) for t in range(i)]
                        for t, (u, idx) in enumerate(where):
                            tiles, row_max = rows[u]
                            parts = []
                            for r0 in range(0, T, 16):
                                at = min(len(clock) - 1, max(since - 1, len(clock) - lead + t // 4 * 8 + r0 // 16))
                                parts.append(jnp.exp2(tiles[idx][r0:r0 + 16] - _after(
                                    jnp.broadcast_to(row_max[r0:r0 + 16], (16, T)), (never, clock[at]))))
                            exps[k].append(_cat(parts, axis=0))
                            sums[u] = sums[u] + exps[k][-1] if u in sums else exps[k][-1]
                    return exps[k]

                if i in timed_exp:
                    def p7(n, t):
                        return _operand(_LHS[n], lambda k: timed(k)[t])
                else:
                    top, bot = ([jnp.exp2(t - row_max) for t in tiles] for tiles, row_max in rows)
                    ops = [_operands(_LHS, (top[t], top[i + t], bot[t], bot[i + t])) for t in range(i)]

                    def p7(n, t):
                        return ops[t][n]

                m = [None] * 7
                for n in pord if i else ():
                    m[n] = tick(_dot(_cat([p7(n, t) for t in range(i)], axis=1).astype(BF), v9[n, :i * T, :]), i)
                    yield i
                if i in timed_exp:
                    diagonal = timed(4)
                    for u in range(2):
                        inv_sums[i][u * T:(u + 1) * T, :] = jnp.broadcast_to(_inverse_row_sum(sums[u]), (T, T))
                else:
                    diagonal = [top[-1], bot[-2], bot[-1]]
                d1 = tick(_dot(_cat(diagonal[:2], axis=0).astype(BF), _cat([v9[1, r, :], v9[7, r, :]], axis=1)), 3)
                d2 = _dot(diagonal[2].astype(BF), _cat([v9[8, r, :], v9[4, r, :]], axis=1))
                yield 6
                o = [d1[:T, :T], d1[:T, T:], d1[T:, :T] + d2[:, :T], d1[T:, T:] + d2[:, T:]]
                if i:
                    o = [a + b for a, b in zip(o, _combine(m, pord))]
                if i in timed_exp:
                    zero = pl.multiple_of((h >> H.bit_length() - 1) * T, T)
                    inv = inv_sums[i][pl.ds(zero, T), :], inv_sums[i][pl.ds(zero + T, T), :]
                else:
                    inv = []
                    for e, late in ((top, o[0]), (bot, o[3])):
                        partial_sums = functools.reduce(jnp.add, e)
                        if i in late_sum:
                            partial_sums = jnp.where(never, late, partial_sums)
                        inv.append(_inverse_row_sum(partial_sums))
                ctx = (o[0] * inv[0], o[2] * inv[1], o[1] * inv[0], o[3] * inv[1])
                for n, t in enumerate(_operands(_RHS, ctx)):
                    ctx7[n, r, :] = t.astype(BF)

            def out_proj(lo, hi):
                m = [None] * 7
                for n in oord:
                    m[n] = tick(_dot_nt(wo7[n], ctx7[n, lo * T:hi * T, :]), hi - lo)
                    yield 1.75 * (hi - lo)
                for k, a in enumerate(_combine(m, oord)):
                    rows, cols = slice(k // 2 * Mh, (k // 2 + 1) * Mh), slice(k % 2 * T, (k % 2 + 1) * T)
                    for i in range(lo, hi):
                        total = acc[i, rows, cols] + gate[i, :, cols] * a[:, (i - lo) * T:(i - lo + 1) * T]
                        acc[i, rows, cols] = total
                        outT[i, rows, cols] = total.astype(BF)

                @pl.when(h == H - 1)
                def _():
                    for i in range(lo, hi):
                        cp_out(i).start()

            def begin(step):
                kind, (lo, _, hi) = step[0], step[1:].partition("-")
                lo, hi = int(lo), int(hi or lo) + 1
                if kind in "KV":
                    return [kv_proj("KV".index(kind), lo, hi), 28 * (hi - lo), 0]
                if kind == "O":
                    return [out_proj(lo, hi), 12.25 * (hi - lo), 0]
                return [(scores if kind == "S" else attend)(lo), 7 * lo + 6, 0]

            staged = False
            for group in prog.split():
                if not staged and ("V" in group or "S" in group):
                    staged = True
                    jobs = [functools.partial(q_job, n, r) for r in range(S // 2 - qjob, -1, -qjob) for n in range(9)]
                    _spread(jobs, never, k_marks, 0, 0.5)
                    jobs = kv_weight_jobs(1, h) + [functools.partial(wo_job, r) for r in range(0, Mh, 16)]
                    _spread(jobs, never, k_marks, *spk)
                running = [begin(step) for step in group.split("+")]
                while running:
                    step = min(running, key=lambda s: s[2] / s[1])
                    try:
                        step[2] += next(step[0])
                    except StopIteration:
                        running.remove(step)
            _spread(kv_weight_jobs(0, jnp.minimum(h + 1, H - 1)), never, clock[keys_done[-1]:], *spv)
            return carry

        if not head_only:
            copies = [cp_x(0), cp_q(0)] + [cp_x(i) for i in range(1, nb)] + [cp_q(1)] + cp_vectors()
            for j in range(2, P):
                copies += [cp_q(j), cp_c(j - 2)]
            for cp in copies + [cp_c(nb - 2), cp_c(nb - 1)] + cp_early() + [cp_wo()] + cp_late():
                cp.start()
            first_pair()
            lax.fori_loop(1, P - 1, middle_pair, 0)
            last_pair()
        lax.fori_loop(0, H, head, 0)
        for i in range(nb):
            cp_out(i).wait()

    def fn(A_x, A_c_kv, A_w_q, A_w_uk, A_w_uv, A_w_o, B_x, B_w_r, B_w_gate, B_w_up, B_w_down, gate_w):
        del B_x
        _, S, M = A_x.shape
        Dc = A_c_kv.shape[2]
        _, H, D = A_w_q.shape
        F = B_w_gate.shape[1]
        nb = S // D
        assert (D, nb, H) == (2 * T, 8, 16) and A_c_kv.shape[:2] == (1, S)
        vmem = pltpu.VMEM
        outT = pl.pallas_call(
            kernel,
            name=name,
            in_specs=[pl.BlockSpec(memory_space=pl.ANY)] * 11,
            out_specs=pl.BlockSpec(memory_space=pl.ANY),
            out_shape=jax.ShapeDtypeStruct((M, S), BF),
            scratch_shapes=[
                vmem((nb, M, D), BF),
                vmem((S, Dc), BF),
                vmem((H // 2, M, D), U32),
                vmem((H // 2, Dc, D), U32),
                vmem((H // 2, Dc, D), U32),
                vmem((H, M, D), BF),
                vmem((M,), BF),
                vmem((M,), BF),
                vmem((M, F), BF),
                vmem((M, F), BF),
                vmem((M, F), BF),
                vmem((7, S // 2, D), BF),
                vmem((7, Dc // D, S // 2, T), BF),
                vmem((7, D, D), BF),
                vmem((7, D, D), BF),
                vmem((2, 7, Dc // 2, T), BF),
                vmem((7, M // 2, T), BF),
                vmem((H, 9, S // 2, T), BF),
                vmem((9, S // 2, T), BF),
                vmem((9, S // 2, T), BF),
                vmem((9, S // 2, T), BF),
                vmem((7, S // 2, T), BF),
                vmem((2, M, T), F32),
                vmem((nb, 1, D), F32),
                vmem((nb, 1, D), F32),
                vmem((nb, M, D), F32),
                vmem((nb, M, D), BF),
                pltpu.SemaphoreType.DMA((4,)),
                pltpu.SemaphoreType.DMA((len(_FIRST_PASS),)),
                pltpu.SemaphoreType.DMA((H // 2 + 1,)),
                *[vmem((D, T), F32)] * nb,
            ],
            compiler_params=pltpu.CompilerParams(vmem_limit_bytes=124 * 2**20, disable_bounds_checks=nocheck,
                                                 disable_semaphore_checks=nocheck),
        )(A_x[0].T, A_c_kv[0], A_w_q, A_w_uk, A_w_uv, jnp.swapaxes(A_w_o, 1, 2), B_w_r, gate_w,
          B_w_gate, B_w_up, B_w_down.T)
        return outT.T[None]

    return fn


_impl = make()


@jax.jit
def pallas_gated_mix__compressed_kv_cla__moe_arch_mod__prompt_kernel(
    A_x, A_c_kv, A_w_q, A_w_uk, A_w_uv, A_w_o, B_x, B_w_r, B_w_gate, B_w_up, B_w_down, gate_w,
):
    return _impl(A_x, A_c_kv, A_w_q, A_w_uk, A_w_uv, A_w_o, B_x, B_w_r, B_w_gate, B_w_up, B_w_down, gate_w)
```

```python
import functools
import math

import jax
import jax.numpy as jnp
from jax import lax
import jax.experimental.pallas as pl
import jax.experimental.pallas.tpu as pltpu

BF = jnp.bfloat16
F32 = jnp.float32
U32 = jnp.uint32
T = 128
_cat = jnp.concatenate

_HEAD_PROGRAM = "K0-3 K4-5+K6 K7 S7 V4-5+V6-7 S5 S6 V0-1+V2-3 P7 P6 S4 O6-7 S3 P4+P5 S1 P3 O4-5 S2 S0+P2 P1+P0 O2-3 O1 O0"
_Q_ORDER, _KV_ORDER, _S_ORDER = (0, 1, 2, 5, 3, 4, 6), (4, 1, 0, 5, 3, 2, 6), (0, 1, 2, 5, 3, 4, 6)
_P_ORDER, _O_ORDER = (2, 4, 0, 5, 1, 3, 6), (0, 1, 2, 5, 3, 4, 6)
_LATE_SUM, _TIMED_EXP, _LEAD = (0, 1, 4, 5, 6, 7), (4, 5), 32
_FIRST_PASS = (((0, 1), ()), ((1, 1), (0, 1)), ((1, 3), (1, 2)), ((3, 6), (2, 3, 5)), ((6, 8), (5, 6, 8)))

_LHS = ((0, 1, 3), (2, 1, 3), (0,), (3,), (0, 1, 1), (2, -1, 0), (1, -1, 3))
_RHS = ((0, 1, 3), (0,), (1, -1, 3), (2, -1, 0), (3,), (0, 1, 1), (2, 1, 3))
_OUT = ({0: 1, 3: 1, 4: -1, 6: 1}, {2: 1, 4: 1}, {1: 1, 3: 1}, {0: 1, 1: -1, 2: 1, 5: 1})


def _operand(rule, quadrant):
    if len(rule) == 1:
        return quadrant(rule[0])
    a, b = quadrant(rule[0]), quadrant(rule[2])
    return a + b if rule[1] > 0 else a - b


def _operands(rules, quads):
    return tuple(_operand(rule, quads.__getitem__) for rule in rules)


def _combine(m, order):
    out = []
    for k, signs in enumerate(_OUT):
        ns = [n for n in order if n in signs]
        if len(ns) == 4:
            ns = ns[::-1] if k == 3 else [ns[2], ns[1], ns[0], ns[3]]
        acc, sign = m[ns[0]], signs[ns[0]]
        for n in ns[1:]:
            if sign > 0:
                acc = acc + m[n] if signs[n] > 0 else acc - m[n]
            else:
                acc, sign = m[n] - acc, 1
        out.append(acc)
    return out


def _dot(a, b):
    return jnp.dot(a, b, preferred_element_type=F32)


def _dot_nt(a, b):
    return lax.dot_general(a, b, (((1,), (1,)), ((), ())), preferred_element_type=F32)


def _sigmoid(z):
    return 1.0 / (1.0 + jnp.exp(-z))


def _inverse_row_sum(partial_sums):
    l = jnp.sum(partial_sums, axis=1, keepdims=True)
    r = pl.reciprocal(l, approx=True)
    return r * (2.0 - l * r)


def _after(x, pin):
    if pin is None:
        return x
    never, late = pin
    bits, late = pltpu.bitcast(x, U32), pltpu.bitcast(late, U32)
    out = _cat([_cat([jnp.where(never, late, bits[r:r + 8, u:u + T]) for u in range(0, bits.shape[1], T)], axis=1)
                for r in range(0, bits.shape[0], 8)], axis=0)
    return pltpu.bitcast(out, x.dtype)


def _spread(jobs, never, marks, lo, hi):
    for k, job in enumerate(jobs):
        job((never, marks[int(len(marks) * (lo + (hi - lo) * k / len(jobs)))]))


def _kernel(xT_hbm, c_hbm, wq_hbm, wuk_hbm, wuv_hbm, woT_hbm, wr_hbm, gw_hbm, wg_hbm, wu_hbm, wdT_hbm, outT_hbm,
            xT, c, wq, wuk, wuv, woT, wr, gw, wg, wu, wdT,
            x7, c7, wq7_first, wq7, wkv7, wo7, q_all, q9, k9, v9, ctx7,
            vec_cols, score, gate, acc, outT, sem, sem_x, sem_q, *inv_sums):
    nb, M, D = xT.shape
    S, H = nb * D, q_all.shape[0]
    P, Mh, Ch = H // 2, M // 2, c.shape[1] // 2
    q_scale = D ** -0.5 * math.log2(math.e)

    def start_of(i, size):
        return i * size if isinstance(i, int) else pl.multiple_of(i * size, size)

    def cp_x(i):
        group = [lo <= i < hi for (lo, hi), _ in _FIRST_PASS].index(True)
        return pltpu.make_async_copy(xT_hbm.at[:, pl.ds(i * D, D)], xT.at[i], sem_x.at[group])

    def cp_q(j):
        return pltpu.make_async_copy(wq_hbm.bitcast(U32).at[:, j, :], wq.at[j], sem_q.at[j])

    def cp_c(i):
        rows = pl.ds(start_of(i, D), D)
        slot = min(i + 2, P) if isinstance(i, int) else i + 2
        return pltpu.make_async_copy(c_hbm.at[rows, :], c.at[rows, :], sem_q.at[slot])

    def cp_vectors():
        return [pltpu.make_async_copy(src, dst, sem_q.at[1]) for src, dst in ((wr_hbm, wr), (gw_hbm, gw))]

    def cp_kv(pairs, slot):
        return [pltpu.make_async_copy(src.bitcast(U32).at[:, j, :], dst.at[j], sem.at[slot])
                for j in pairs for src, dst in ((wuk_hbm, wuk), (wuv_hbm, wuv))]

    def cp_early():
        ffn = ((wg_hbm, wg), (wu_hbm, wu), (wdT_hbm, wdT))
        return [pltpu.make_async_copy(src, dst, sem.at[0]) for src, dst in ffn] + cp_kv(range(2), 0)

    def cp_wo():
        return pltpu.make_async_copy(woT_hbm, woT, sem.at[1])

    def cp_late():
        return cp_kv(range(2, P), 2)

    def cp_out(i):
        return pltpu.make_async_copy(outT.at[i], outT_hbm.at[:, pl.ds(i * D, D)], sem.at[3])

    def build_x7(i):
        xt = xT[i].astype(F32)
        pad = jnp.zeros((D - Mh, T), F32)
        quads = [_cat([t, pad], axis=0).T for t in (xt[:Mh, :T], xt[Mh:, :T], xt[:Mh, T:], xt[Mh:, T:])]
        for n, t in enumerate(_operands(_LHS, quads)):
            x7[n, i * T:(i + 1) * T, :] = t.astype(BF)

    def c7_jobs(i):
        src, dst = start_of(i, D), start_of(i, T)

        def job(u, r, pin):
            quads = [_after(c[pl.ds(src + rh * T + r, 16), ch * Ch + u * T:ch * Ch + (u + 1) * T], pin).astype(F32)
                     for rh in range(2) for ch in range(2)]
            for n, t in enumerate(_operands(_LHS, quads)):
                c7[n, u, pl.ds(dst + r, 16), :] = t.astype(BF)

        return [functools.partial(job, u, r) for u in range(Ch // T) for r in range(0, T, 16)]

    def weight_jobs(words, shift, dst, col=0):
        k = words.shape[0] // 2

        def job(r, pin):
            quads = [pltpu.bitcast((_after(words[kh * k + r:kh * k + r + 16, ch * T:(ch + 1) * T], pin) << shift)
                                   & U32(0xFFFF0000), F32) for kh in range(2) for ch in range(2)]
            for n, t in enumerate(_operands(_RHS, quads)):
                dst[n, r:r + 16, col:col + T] = t.astype(BF)

        return [functools.partial(job, r) for r in range(0, k, 16)]

    def wq7_jobs(j, dst):
        heads = [weight_jobs(wq.at[j], 16 * (1 - e), dst, e * T) for e in range(2)]
        return [job for both in zip(*heads) for job in both]

    def gate_jobs(i):
        sums = {}

        def job(t, r, pin):
            cols = slice(t * T, (t + 1) * T)
            xt = _after(xT[i, r:r + 32, cols], pin).astype(F32)
            for u in range(2):
                p = xt * vec_cols[u, r:r + 32, :]
                p = (p[0:8] + p[8:16]) + (p[16:24] + p[24:32])
                sums[u] = p if r == 0 else sums[u] + p
            if r + 32 == M:
                score[i, :, cols] = jnp.sum(sums[0], axis=0, keepdims=True)
                gate[i, :, cols] = _sigmoid(jnp.sum(sums[1], axis=0, keepdims=True))

        return [functools.partial(job, t, r) for t in range(2) for r in range(0, M, 32)]

    def residual_jobs(i):
        keep = []

        def job(r, pin):
            if not keep:
                keep.append(1.0 - gate[i])
            acc[i, r:r + 16, :] = keep[0] * _after(xT[i, r:r + 16, :], pin).astype(F32)

        return [functools.partial(job, r) for r in range(0, M, 16)]

    def route():
        def whole(op, t):
            return op(op(t, axis=0, keepdims=True), axis=1, keepdims=True)

        r = _cat([score[i] for i in range(nb)], axis=0).astype(BF).astype(F32)
        tok = lax.broadcasted_iota(jnp.int32, (nb, D), 0) * D + lax.broadcasted_iota(jnp.int32, (nb, D), 1)
        bits = pltpu.bitcast(jnp.where(r == 0.0, 0.0, r), jnp.int32) >> 16
        rank = jnp.where(r != r, 0, jnp.where(bits < 0, bits ^ 0x7FFF, bits) + 0x8000)
        key = pltpu.bitcast(0x20000000 + rank * S + (S - 1 - tok), F32)
        lane = lax.broadcasted_iota(jnp.int32, (1, D), 1)
        picks = []
        for _ in range(2):
            best = whole(jnp.max, key)
            idx = S - 1 - (pltpu.bitcast(best, jnp.int32)[0, 0] & (S - 1))
            weight = _sigmoid(whole(jnp.sum, jnp.where(key == best, r, 0.0)))
            picks.append((idx >> (D.bit_length() - 1), lane == (idx & (D - 1)), weight))
            key = jnp.where(key == best, 0.0, key)
        return picks

    def gather(picks):
        row = lax.broadcasted_iota(jnp.int32, (16, D), 0)
        return sum(_dot_nt(jnp.where((row == u) & hot, 1.0, 0.0).astype(BF), xT[b])
                   for u, (b, hot, _) in enumerate(picks)).astype(BF)

    def scatter_jobs(y, picks):
        def job(b, hot, col, keep, r, pin):
            yr = _after(col[r:r + 32], pin)
            acc[b, r:r + 32, :] += jnp.where(hot, keep * _cat([yr, yr], axis=1), 0.0)

        jobs = []
        for u, (b, hot, weight) in enumerate(picks):
            col = jnp.broadcast_to(y[u:u + 1] * weight, (T, M)).T
            keep = 1.0 - gate[b]
            jobs += [functools.partial(job, b, hot, col, keep, r) for r in range(0, M, 32)]
        return jobs

    def q_proj(j, w7, lo, hi, before=None):
        m = [None] * 7
        for k, n in enumerate(_Q_ORDER):
            if before is not None:
                before(k)
            m[n] = _dot(x7[n, lo * T:hi * T, :], w7[n])
        for e in range(2):
            q = [t * q_scale for t in _combine([t[:, e * T:(e + 1) * T] for t in m], _Q_ORDER)]
            for n, t in enumerate(_operands(_LHS, q) + (q[1], q[2])):
                q_all[2 * j + e, n, lo * T:hi * T, :] = t.astype(BF)
        return [m[n][r:r + 8, :T] for n in _Q_ORDER for r in range(0, (hi - lo) * T, 16)]

    def never_set():
        t = xT[0, :16, :T].astype(F32)[:8]
        return t * t < 0.0

    def first_pair():
        for ref in (wq7_first, wq7):
            ref[:, Mh:, :] = jnp.zeros((7, D - Mh, D), BF)
        for s, (arrived, projected) in enumerate(_FIRST_PASS):
            for i in range(*arrived):
                cp_x(i).wait()
            if s == 1:
                cp_q(0).wait()
                for job in wq7_jobs(0, wq7_first):
                    job(None)
            if s == len(_FIRST_PASS) - 1:
                for cp in [cp_q(1)] + cp_vectors():
                    cp.wait()
            for i in range(*arrived):
                build_x7(i)
            marks = [t for lo, hi in zip(projected, projected[1:]) for t in q_proj(0, wq7_first, lo, hi)]
        for u, ref in enumerate((wr, gw)):
            vec_cols[u] = jnp.broadcast_to(ref[...].astype(F32).reshape(1, M), (T, M)).T
        _spread(wq7_jobs(1, wq7), never_set(), marks, 0.35, 0.7)

    def middle_pair(j, carry):
        cp_q(j + 1).wait()
        cp_c(j - 1).wait()
        never = j >= P
        marks = q_proj(j, wq7, 0, nb)
        b = jnp.minimum(2 * j - 2, nb - 2)
        _spread(gate_jobs(b) + gate_jobs(b + 1) + c7_jobs(j - 1) + residual_jobs(j - 1), never, marks, 0, 0.45)

        def next_weights(n, r, pin):
            for e in range(2):
                def quadrant(k):
                    rows, cols = slice(k // 2 * Mh + r, k // 2 * Mh + r + 16), slice(k % 2 * T, (k % 2 + 1) * T)
                    w = _after(wq[j + 1, rows, cols], pin)
                    return pltpu.bitcast(w & U32(0xFFFF0000) if e else w << 16, F32)

                wq7[n, r:r + 16, e * T:(e + 1) * T] = _operand(_RHS[n], quadrant).astype(BF)

        for k, n in enumerate(_Q_ORDER):
            jobs = [functools.partial(next_weights, n, r) for r in range(0, Mh, 16)]
            _spread(jobs, never, marks, k / 7 + 0.005, k / 7 + 0.1)
        return carry

    def last_pair():
        for cp in [cp_c(nb - 2), cp_c(nb - 1)] + cp_early():
            cp.wait()
        picks, never = route(), never_set()
        slabs = wg.shape[1] // T
        xs, hidden, y = [], [], []

        def take(k):
            if k == 1:
                xs.append(gather(picks))

        def up(step, k):
            for t in range((step + k) * 2 * slabs // 21, (step + k + 1) * 2 * slabs // 21):
                hidden.append(_dot(xs[0], (wg, wu)[t % 2][:, t // 2 * T:(t // 2 + 1) * T]))

        def down(step, k):
            for t in range((step + k) * slabs // 14, (step + k + 1) * slabs // 14):
                g, u = hidden[2 * t], hidden[2 * t + 1]
                y.append(_dot_nt((g * _sigmoid(g) * u).astype(BF), wdT[:, t * T:(t + 1) * T]))

        extras = ([None, take] + [functools.partial(up, 7 * s) for s in range(3)]
                  + [functools.partial(down, 7 * s) for s in range(2)])
        marks = [t for i, extra in enumerate(extras) for t in q_proj(P - 1, wq7, i, i + 1, extra)]
        y = functools.reduce(jnp.add, y)
        tail = q_proj(P - 1, wq7, nb - 1, nb)
        jobs = residual_jobs(nb - 2) + residual_jobs(nb - 1) + c7_jobs(nb - 2) + c7_jobs(nb - 1)
        _spread(jobs + weight_jobs(wuk.at[0], 16, wkv7.at[0]), never, marks, 0, 0.97)
        _spread(scatter_jobs(y, picks), never, tail, 0.3, 0.9)
        cp_wo().wait()

    def head(h, carry):
        @pl.when(h == 2)
        def _():
            for cp in cp_late():
                cp.wait()

        never = h >= H
        clock, k_marks, scores_of, keys_done = [], [], {}, []

        def tick(x, tiles):
            n = max(1, x.shape[0] * tiles // 64)
            clock.extend(x[(k * (x.shape[0] // 8) // n) * 8:][:8, -T:] for k in range(n))
            return x

        def kv_weight_jobs(u, hh):
            shift = ((1 - (hh & 1)) * 16).astype(U32)
            return weight_jobs((wuk, wuv)[u].at[hh >> 1], shift, wkv7.at[u])

        def wo_job(r, pin):
            quads = [_after(woT[h, rh * Mh + r:rh * Mh + r + 16, ch * T:(ch + 1) * T], pin).astype(F32)
                     for rh in range(2) for ch in range(2)]
            for n, t in enumerate(_operands(_LHS, quads)):
                wo7[n, r:r + 16, :] = t.astype(BF)

        def q_job(n, r, pin):
            words = _after(q_all.bitcast(U32)[h, n, r // 2:(r + 16) // 2, :], pin)
            q9[n, r:r + 16, :] = pltpu.bitcast(words, BF)

        def kv_proj(u, lo, hi):
            r = slice(lo * T, hi * T)
            m = [None] * 7
            for n in _KV_ORDER:
                m[n] = tick(_dot(_cat([c7[n, t, r, :] for t in range(Ch // T)], axis=1), wkv7[u, n]), 4)
                if u == 0:
                    k_marks.extend(m[n][t:t + 8] for t in range(0, (hi - lo) * T, 16))
                    keys_done.append(len(clock))
                yield 4 * (hi - lo)
            a = _combine(m, _KV_ORDER)
            ops = _operands(_RHS, a if u else (a[0], a[2], a[1], a[3]))
            for n, t in enumerate(ops + (a[1], a[2])):
                (k9, v9)[u][n, r, :] = t.astype(BF)

        def scores(i):
            r = slice(i * T, (i + 1) * T)
            q_top, q_bot = _cat([q9[2, r, :], q9[7, r, :]], axis=1), _cat([q9[8, r, :], q9[3, r, :]], axis=1)
            past = [[], [], [], []]
            if i:
                m = [None] * 7
                for n in _S_ORDER:
                    m[n] = tick(_dot_nt(q9[n, r, :], k9[n, :i * T, :]), i)
                    yield i
                past = [[s[:, t * T:(t + 1) * T] for t in range(i)] for s in _combine(m, _S_ORDER)]
            d1 = tick(_dot_nt(_cat([q_top, q_bot], axis=0), _cat([k9[1, r, :], k9[7, r, :]], axis=1)), 3)
            d2 = _dot_nt(q_bot, _cat([k9[8, r, :], k9[4, r, :]], axis=1))
            yield 6
            causal = lax.broadcasted_iota(jnp.int32, (T, T), 1) <= lax.broadcasted_iota(jnp.int32, (T, T), 0)
            diagonal = [jnp.where(causal, d1[:T], -1e9)], [d1[T:], jnp.where(causal, d2, -1e9)]
            rows = []
            for u in range(2):
                first, second = sorted((2 * u, 2 * u + 1), key=lambda k: max(_S_ORDER.index(n) for n in _OUT[k]))
                row_max = functools.reduce(jnp.maximum, past[first] + past[second] + diagonal[u])
                rows.append((past[2 * u] + past[2 * u + 1] + diagonal[u],
                             jnp.max(row_max, axis=1, keepdims=True)))
            scores_of[i] = rows, len(clock)

        def attend(i):
            rows, since = scores_of.pop(i)
            r = slice(i * T, (i + 1) * T)
            exps, sums = {}, {}

            def timed(k):
                if k not in exps:
                    exps[k] = []
                    where = [(0, -1), (1, -2), (1, -1)] if k == 4 else [(k // 2, k % 2 * i + t) for t in range(i)]
                    for t, (u, idx) in enumerate(where):
                        tiles, row_max = rows[u]
                        parts = []
                        for r0 in range(0, T, 16):
                            at = min(len(clock) - 1, max(since - 1, len(clock) - _LEAD + t // 4 * 8 + r0 // 16))
                            parts.append(jnp.exp2(tiles[idx][r0:r0 + 16] - _after(
                                jnp.broadcast_to(row_max[r0:r0 + 16], (16, T)), (never, clock[at]))))
                        exps[k].append(_cat(parts, axis=0))
                        sums[u] = sums[u] + exps[k][-1] if u in sums else exps[k][-1]
                return exps[k]

            if i in _TIMED_EXP:
                def p7(n, t):
                    return _operand(_LHS[n], lambda k: timed(k)[t])
            else:
                top, bot = ([jnp.exp2(t - row_max) for t in tiles] for tiles, row_max in rows)
                ops = [_operands(_LHS, (top[t], top[i + t], bot[t], bot[i + t])) for t in range(i)]

                def p7(n, t):
                    return ops[t][n]

            m = [None] * 7
            for n in _P_ORDER if i else ():
                m[n] = tick(_dot(_cat([p7(n, t) for t in range(i)], axis=1).astype(BF), v9[n, :i * T, :]), i)
                yield i
            if i in _TIMED_EXP:
                diagonal = timed(4)
                for u in range(2):
                    inv_sums[i][u * T:(u + 1) * T, :] = jnp.broadcast_to(_inverse_row_sum(sums[u]), (T, T))
            else:
                diagonal = [top[-1], bot[-2], bot[-1]]
            d1 = tick(_dot(_cat(diagonal[:2], axis=0).astype(BF), _cat([v9[1, r, :], v9[7, r, :]], axis=1)), 3)
            d2 = _dot(diagonal[2].astype(BF), _cat([v9[8, r, :], v9[4, r, :]], axis=1))
            yield 6
            o = [d1[:T, :T], d1[:T, T:], d1[T:, :T] + d2[:, :T], d1[T:, T:] + d2[:, T:]]
            if i:
                o = [a + b for a, b in zip(o, _combine(m, _P_ORDER))]
            if i in _TIMED_EXP:
                zero = pl.multiple_of((h >> H.bit_length() - 1) * T, T)
                inv = inv_sums[i][pl.ds(zero, T), :], inv_sums[i][pl.ds(zero + T, T), :]
            else:
                inv = []
                for e, late in ((top, o[0]), (bot, o[3])):
                    partial_sums = functools.reduce(jnp.add, e)
                    if i in _LATE_SUM:
                        partial_sums = jnp.where(never, late, partial_sums)
                    inv.append(_inverse_row_sum(partial_sums))
            ctx = (o[0] * inv[0], o[2] * inv[1], o[1] * inv[0], o[3] * inv[1])
            for n, t in enumerate(_operands(_RHS, ctx)):
                ctx7[n, r, :] = t.astype(BF)

        def out_proj(lo, hi):
            m = [None] * 7
            for n in _O_ORDER:
                m[n] = tick(_dot_nt(wo7[n], ctx7[n, lo * T:hi * T, :]), hi - lo)
                yield 1.75 * (hi - lo)
            for k, a in enumerate(_combine(m, _O_ORDER)):
                rows, cols = slice(k // 2 * Mh, (k // 2 + 1) * Mh), slice(k % 2 * T, (k % 2 + 1) * T)
                for i in range(lo, hi):
                    total = acc[i, rows, cols] + gate[i, :, cols] * a[:, (i - lo) * T:(i - lo + 1) * T]
                    acc[i, rows, cols] = total
                    outT[i, rows, cols] = total.astype(BF)

            @pl.when(h == H - 1)
            def _():
                for i in range(lo, hi):
                    cp_out(i).start()

        def begin(step):
            kind, (lo, _, hi) = step[0], step[1:].partition("-")
            lo, hi = int(lo), int(hi or lo) + 1
            if kind in "KV":
                return [kv_proj("KV".index(kind), lo, hi), 28 * (hi - lo), 0]
            if kind == "O":
                return [out_proj(lo, hi), 12.25 * (hi - lo), 0]
            return [(scores if kind == "S" else attend)(lo), 7 * lo + 6, 0]

        staged = False
        for group in _HEAD_PROGRAM.split():
            if not staged and ("V" in group or "S" in group):
                staged = True
                jobs = [functools.partial(q_job, n, r) for r in range(S // 2 - 16, -1, -16) for n in range(9)]
                _spread(jobs, never, k_marks, 0, 0.5)
                jobs = kv_weight_jobs(1, h) + [functools.partial(wo_job, r) for r in range(0, Mh, 16)]
                _spread(jobs, never, k_marks, 0.5, 0.9)
            running = [begin(step) for step in group.split("+")]
            while running:
                step = min(running, key=lambda s: s[2] / s[1])
                try:
                    step[2] += next(step[0])
                except StopIteration:
                    running.remove(step)
        _spread(kv_weight_jobs(0, jnp.minimum(h + 1, H - 1)), never, clock[keys_done[-1]:], 0.08, 0.16)
        return carry

    copies = [cp_x(0), cp_q(0)] + [cp_x(i) for i in range(1, nb)] + [cp_q(1)] + cp_vectors()
    for j in range(2, P):
        copies += [cp_q(j), cp_c(j - 2)]
    for cp in copies + [cp_c(nb - 2), cp_c(nb - 1)] + cp_early() + [cp_wo()] + cp_late():
        cp.start()
    first_pair()
    lax.fori_loop(1, P - 1, middle_pair, 0)
    last_pair()
    lax.fori_loop(0, H, head, 0)
    for i in range(nb):
        cp_out(i).wait()


@jax.jit
def pallas_gated_mix__compressed_kv_cla__moe_arch_mod__prompt_kernel(
    A_x, A_c_kv, A_w_q, A_w_uk, A_w_uv, A_w_o, B_x, B_w_r, B_w_gate, B_w_up, B_w_down, gate_w,
):
    del B_x
    _, S, M = A_x.shape
    Dc = A_c_kv.shape[2]
    _, H, D = A_w_q.shape
    F = B_w_gate.shape[1]
    nb = S // D
    assert (D, nb, H) == (2 * T, 8, 16) and A_c_kv.shape[:2] == (1, S)
    vmem = pltpu.VMEM
    outT = pl.pallas_call(
        _kernel,
        in_specs=[pl.BlockSpec(memory_space=pl.ANY)] * 11,
        out_specs=pl.BlockSpec(memory_space=pl.ANY),
        out_shape=jax.ShapeDtypeStruct((M, S), BF),
        scratch_shapes=[
            vmem((nb, M, D), BF),
            vmem((S, Dc), BF),
            vmem((H // 2, M, D), U32),
            vmem((H // 2, Dc, D), U32),
            vmem((H // 2, Dc, D), U32),
            vmem((H, M, D), BF),
            vmem((M,), BF),
            vmem((M,), BF),
            vmem((M, F), BF),
            vmem((M, F), BF),
            vmem((M, F), BF),
            vmem((7, S // 2, D), BF),
            vmem((7, Dc // D, S // 2, T), BF),
            vmem((7, D, D), BF),
            vmem((7, D, D), BF),
            vmem((2, 7, Dc // 2, T), BF),
            vmem((7, M // 2, T), BF),
            vmem((H, 9, S // 2, T), BF),
            vmem((9, S // 2, T), BF),
            vmem((9, S // 2, T), BF),
            vmem((9, S // 2, T), BF),
            vmem((7, S // 2, T), BF),
            vmem((2, M, T), F32),
            vmem((nb, 1, D), F32),
            vmem((nb, 1, D), F32),
            vmem((nb, M, D), F32),
            vmem((nb, M, D), BF),
            pltpu.SemaphoreType.DMA((4,)),
            pltpu.SemaphoreType.DMA((len(_FIRST_PASS),)),
            pltpu.SemaphoreType.DMA((H // 2 + 1,)),
            *[vmem((D, T), F32)] * nb,
        ],
        compiler_params=pltpu.CompilerParams(vmem_limit_bytes=124 * 2**20),
    )(A_x[0].T, A_c_kv[0], A_w_q, A_w_uk, A_w_uv, jnp.swapaxes(A_w_o, 1, 2), B_w_r, gate_w,
      B_w_gate, B_w_up, B_w_down.T)
    return outT.T[None]
```

```python
import functools
import math

import jax
import jax.numpy as jnp
from jax import lax
import jax.experimental.pallas as pl
import jax.experimental.pallas.tpu as pltpu

BF = jnp.bfloat16
F32 = jnp.float32
U32 = jnp.uint32
T = 128
_cat = jnp.concatenate

_HEAD_PROGRAM = "S7 S6 P7 S5 P6 S4 O6-7 S3 P4+P5 S1 P3 O4-5 S2 S0+P2 P1+P0 O2-3 O1 O0"
_FIRST_PASS = (((0, 1), ()), ((1, 1), (0, 1)), ((1, 3), (1, 2)), ((3, 6), (2, 3, 5)), ((6, 8), (5, 6, 8)))

_LHS = ((0, 1, 3), (2, 1, 3), (0,), (3,), (0, 1, 1), (2, -1, 0), (1, -1, 3))
_RHS = ((0, 1, 3), (0,), (1, -1, 3), (2, -1, 0), (3,), (0, 1, 1), (2, 1, 3))
_OUT = ({0: 1, 3: 1, 4: -1, 6: 1}, {2: 1, 4: 1}, {1: 1, 3: 1}, {0: 1, 1: -1, 2: 1, 5: 1})


def _operand(rule, quadrant):
    if len(rule) == 1:
        return quadrant(rule[0])
    a, b = quadrant(rule[0]), quadrant(rule[2])
    return a + b if rule[1] > 0 else a - b


def _operands(rules, quads):
    return tuple(_operand(rule, quads.__getitem__) for rule in rules)


def _combine(m, order):
    out = []
    for k, signs in enumerate(_OUT):
        ns = [n for n in order if n in signs]
        if len(ns) == 4:
            ns = ns[::-1] if k == 3 else [ns[2], ns[1], ns[0], ns[3]]
        acc, sign = m[ns[0]], signs[ns[0]]
        for n in ns[1:]:
            if sign > 0:
                acc = acc + m[n] if signs[n] > 0 else acc - m[n]
            else:
                acc, sign = m[n] - acc, 1
        out.append(acc)
    return out


def _dot(a, b):
    return jnp.dot(a, b, preferred_element_type=F32)


def _dot_nt(a, b):
    return lax.dot_general(a, b, (((1,), (1,)), ((), ())), preferred_element_type=F32)


def _sigmoid(z):
    return 1.0 / (1.0 + jnp.exp(-z))


def _inverse_row_sum(partial_sums):
    l = jnp.sum(partial_sums, axis=1, keepdims=True)
    r = pl.reciprocal(l, approx=True)
    return r * (2.0 - l * r)


def _after(x, pin):
    if pin is None:
        return x
    never, late = pin
    bits, late = pltpu.bitcast(x, U32), pltpu.bitcast(late, U32)
    out = _cat([_cat([jnp.where(never, late, bits[r:r + 8, u:u + T]) for u in range(0, bits.shape[1], T)], axis=1)
                for r in range(0, bits.shape[0], 8)], axis=0)
    return pltpu.bitcast(out, x.dtype)


def _spread(jobs, never, marks, lo, hi):
    for k, job in enumerate(jobs):
        job((never, marks[int(len(marks) * (lo + (hi - lo) * k / len(jobs)))]))


def make(prog=_HEAD_PROGRAM, qord=(0, 1, 2, 5, 3, 4, 6), sord=(0, 1, 2, 5, 3, 4, 6),
         pord=(2, 4, 0, 5, 1, 3, 6), oord=(0, 1, 2, 5, 3, 4, 6), late_sum=(0, 1, 4, 5, 6, 7), timed_exp=(4, 5), lead=32,
         vnow=3, span=60, delay=0, plane_only=False, scopes=False, head_only=False, nocheck=False, name="ka"):
    def loop(lo, hi, f, init):
        def g(i, c):
            with jax.named_scope(f.__name__):
                return f(i, c)
        return lax.fori_loop(lo, hi, g if scopes else f, init)

    def kernel(xT_hbm, c_hbm, wq_hbm, wuk_hbm, wuv_hbm, woT_hbm, wr_hbm, gw_hbm, wg_hbm, wu_hbm, wdT_hbm, outT_hbm,
               woT, q_all, kv_all, gate, acc, sem, sem_x, sem_q):
        nb, M, D = acc.shape
        S, H = nb * D, q_all.shape[0]
        P, Mh, Dc, F = H // 2, M // 2, c_hbm.shape[1], wg_hbm.shape[1]
        vmem = pltpu.VMEM
        q_scale = D ** -0.5 * math.log2(math.e)

        def start_of(i, size):
            return i * size if isinstance(i, int) else pl.multiple_of(i * size, size)

        def queries(c, w_kv, u_sum, xT, wq, wr, gw, wg, wu, wdT, x7, wq7_first, wq7, vec_cols, score):
            def cp_x(i):
                group = [lo <= i < hi for (lo, hi), _ in _FIRST_PASS].index(True)
                return pltpu.make_async_copy(xT_hbm.at[:, pl.ds(i * D, D)], xT.at[i], sem_x.at[group])

            def cp_q(j):
                return pltpu.make_async_copy(wq_hbm.bitcast(U32).at[:, j, :], wq.at[j], sem_q.at[j])

            def cp_c(i):
                rows = pl.ds(start_of(i, D), D)
                slot = min(i + 2, P) if isinstance(i, int) else i + 2
                return pltpu.make_async_copy(c_hbm.at[rows, :], c.at[rows, :], sem_q.at[slot])

            def cp_vectors():
                return [pltpu.make_async_copy(src, dst, sem_q.at[1]) for src, dst in ((wr_hbm, wr), (gw_hbm, gw))]

            def cp_early():
                ffn = ((wg_hbm, wg), (wu_hbm, wu), (wdT_hbm, wdT))
                return [pltpu.make_async_copy(src, dst, sem.at[0]) for src, dst in ffn]

            def build_x7(i):
                xt = xT[i].astype(F32)
                pad = jnp.zeros((D - Mh, T), F32)
                quads = [_cat([t, pad], axis=0).T for t in (xt[:Mh, :T], xt[Mh:, :T], xt[:Mh, T:], xt[Mh:, T:])]
                for n, t in enumerate(_operands(_LHS, quads)):
                    x7[n, i * T:(i + 1) * T, :] = t.astype(BF)

            def c_sum_jobs(i, first=False):
                def job(k, r, pin):
                    t = _after(c[pl.ds(start_of(i, D) + r, 64), k * T:(k + 1) * T], pin).astype(F32)
                    u_sum[k, r:r + 64, :] = t if first else u_sum[k, r:r + 64, :] + t

                return [functools.partial(job, k, r) for k in range(nb) for r in range(0, D, 64)]

            def weight_jobs(words, shift, dst, col=0):
                k = words.shape[0] // 2

                def job(r, pin):
                    quads = [pltpu.bitcast((_after(words[kh * k + r:kh * k + r + 16, ch * T:(ch + 1) * T], pin) << shift)
                                           & U32(0xFFFF0000), F32) for kh in range(2) for ch in range(2)]
                    for n, t in enumerate(_operands(_RHS, quads)):
                        dst[n, r:r + 16, col:col + T] = t.astype(BF)

                return [functools.partial(job, r) for r in range(0, k, 16)]

            def wq7_jobs(j, dst):
                heads = [weight_jobs(wq.at[j], 16 * (1 - e), dst, e * T) for e in range(2)]
                return [job for both in zip(*heads) for job in both]

            def gate_jobs(i):
                sums = {}

                def job(t, r, pin):
                    cols = slice(t * T, (t + 1) * T)
                    xt = _after(xT[i, r:r + 32, cols], pin).astype(F32)
                    for u in range(2):
                        p = xt * vec_cols[u, r:r + 32, :]
                        p = (p[0:8] + p[8:16]) + (p[16:24] + p[24:32])
                        sums[u] = p if r == 0 else sums[u] + p
                    if r + 32 == M:
                        score[i, :, cols] = jnp.sum(sums[0], axis=0, keepdims=True)
                        gate[i, :, cols] = _sigmoid(jnp.sum(sums[1], axis=0, keepdims=True))

                return [functools.partial(job, t, r) for t in range(2) for r in range(0, M, 32)]

            def residual_jobs(i):
                keep = []

                def job(r, pin):
                    if not keep:
                        keep.append(1.0 - gate[i])
                    acc[i, r:r + 16, :] = keep[0] * _after(xT[i, r:r + 16, :], pin).astype(F32)

                return [functools.partial(job, r) for r in range(0, M, 16)]

            def route():
                def whole(op, t):
                    return op(op(t, axis=0, keepdims=True), axis=1, keepdims=True)

                r = _cat([score[i] for i in range(nb)], axis=0).astype(BF).astype(F32)
                tok = lax.broadcasted_iota(jnp.int32, (nb, D), 0) * D + lax.broadcasted_iota(jnp.int32, (nb, D), 1)
                bits = pltpu.bitcast(jnp.where(r == 0.0, 0.0, r), jnp.int32) >> 16
                rank = jnp.where(r != r, 0, jnp.where(bits < 0, bits ^ 0x7FFF, bits) + 0x8000)
                key = pltpu.bitcast(0x20000000 + rank * S + (S - 1 - tok), F32)
                lane = lax.broadcasted_iota(jnp.int32, (1, D), 1)
                picks = []
                for _ in range(2):
                    best = whole(jnp.max, key)
                    idx = S - 1 - (pltpu.bitcast(best, jnp.int32)[0, 0] & (S - 1))
                    weight = _sigmoid(whole(jnp.sum, jnp.where(key == best, r, 0.0)))
                    picks.append((idx >> (D.bit_length() - 1), lane == (idx & (D - 1)), weight))
                    key = jnp.where(key == best, 0.0, key)
                return picks

            def gather(picks):
                row = lax.broadcasted_iota(jnp.int32, (16, D), 0)
                return sum(_dot_nt(jnp.where((row == u) & hot, 1.0, 0.0).astype(BF), xT[b])
                           for u, (b, hot, _) in enumerate(picks)).astype(BF)

            def scatter_jobs(y, picks):
                def job(b, hot, col, keep, r, pin):
                    yr = _after(col[r:r + 32], pin)
                    acc[b, r:r + 32, :] += jnp.where(hot, keep * _cat([yr, yr], axis=1), 0.0)

                jobs = []
                for u, (b, hot, weight) in enumerate(picks):
                    col = jnp.broadcast_to(y[u:u + 1] * weight, (T, M)).T
                    keep = 1.0 - gate[b]
                    jobs += [functools.partial(job, b, hot, col, keep, r) for r in range(0, M, 32)]
                return jobs

            def q_proj(j, w7, lo, hi, before=None):
                m = [None] * 7
                for k, n in enumerate(qord):
                    if before is not None:
                        before(k)
                    m[n] = _dot(x7[n, lo * T:hi * T, :], w7[n])
                for e in range(2):
                    q = [t * q_scale for t in _combine([t[:, e * T:(e + 1) * T] for t in m], qord)]
                    for n, t in enumerate(q):
                        q_all[2 * j + e, n, lo * T:hi * T, :] = t.astype(BF)
                return [m[n][r:r + 8, :T] for n in qord for r in range(0, (hi - lo) * T, 16)]

            def never_set():
                t = xT[0, :16, :T].astype(F32)[:8]
                return t * t < 0.0

            def first_pair():
                u_sum[...] = jnp.zeros(u_sum.shape, F32)
                for ref in (wq7_first, wq7):
                    ref[:, Mh:, :] = jnp.zeros((7, D - Mh, D), BF)
                for s, (arrived, projected) in enumerate(_FIRST_PASS):
                    for i in range(*arrived):
                        cp_x(i).wait()
                    if s == 1:
                        cp_q(0).wait()
                        for job in wq7_jobs(0, wq7_first):
                            job(None)
                    if s == len(_FIRST_PASS) - 1:
                        for cp in [cp_q(1)] + cp_vectors():
                            cp.wait()
                    for i in range(*arrived):
                        build_x7(i)
                    marks = [t for lo, hi in zip(projected, projected[1:]) for t in q_proj(0, wq7_first, lo, hi)]
                for u, ref in enumerate((wr, gw)):
                    vec_cols[u] = jnp.broadcast_to(ref[...].astype(F32).reshape(1, M), (T, M)).T
                _spread(wq7_jobs(1, wq7), never_set(), marks, 0.35, 0.7)

            def middle_pair(j, carry):
                cp_q(j + 1).wait()
                cp_c(j - 1).wait()
                never = j >= P
                marks = q_proj(j, wq7, 0, nb)
                b = jnp.minimum(2 * j - 2, nb - 2)
                _spread(gate_jobs(b) + gate_jobs(b + 1) + c_sum_jobs(j - 1) + residual_jobs(j - 1), never, marks, 0, 0.45)

                def next_weights(n, r, pin):
                    for e in range(2):
                        def quadrant(k):
                            rows, cols = slice(k // 2 * Mh + r, k // 2 * Mh + r + 16), slice(k % 2 * T, (k % 2 + 1) * T)
                            w = _after(wq[j + 1, rows, cols], pin)
                            return pltpu.bitcast(w & U32(0xFFFF0000) if e else w << 16, F32)

                        wq7[n, r:r + 16, e * T:(e + 1) * T] = _operand(_RHS[n], quadrant).astype(BF)

                for k, n in enumerate(qord):
                    jobs = [functools.partial(next_weights, n, r) for r in range(0, Mh, 16)]
                    _spread(jobs, never, marks, k / 7 + 0.005, k / 7 + 0.1)
                return carry

            def last_pair():
                for cp in [cp_c(nb - 2), cp_c(nb - 1)] + cp_early():
                    cp.wait()
                picks, never = route(), never_set()
                slabs = wg.shape[1] // T
                xs, hidden, y = [], [], []

                def take(k):
                    if k == 1:
                        xs.append(gather(picks))

                def up(step, k):
                    for t in range((step + k) * 2 * slabs // 21, (step + k + 1) * 2 * slabs // 21):
                        hidden.append(_dot(xs[0], (wg, wu)[t % 2][:, t // 2 * T:(t // 2 + 1) * T]))

                def down(step, k):
                    for t in range((step + k) * slabs // 14, (step + k + 1) * slabs // 14):
                        g, u = hidden[2 * t], hidden[2 * t + 1]
                        y.append(_dot_nt((g * _sigmoid(g) * u).astype(BF), wdT[:, t * T:(t + 1) * T]))

                extras = ([None, take] + [functools.partial(up, 7 * s) for s in range(3)]
                          + [functools.partial(down, 7 * s) for s in range(2)])
                marks = [t for i, extra in enumerate(extras) for t in q_proj(P - 1, wq7, i, i + 1, extra)]
                y = functools.reduce(jnp.add, y)
                tail = q_proj(P - 1, wq7, nb - 1, nb)
                jobs = residual_jobs(nb - 2) + residual_jobs(nb - 1) + c_sum_jobs(nb - 2) + c_sum_jobs(nb - 1)
                _spread(jobs, never, marks, 0, 0.97)
                _spread(scatter_jobs(y, picks), never, tail, 0.3, 0.9)

            copies = [cp_x(0), cp_q(0)] + [cp_x(i) for i in range(1, nb)] + [cp_q(1)] + cp_vectors()
            for j in range(2, P):
                copies += [cp_q(j), cp_c(j - 2)]
            early, late = cp_kv(w_kv, range(P // 2 + 1), 1), cp_kv(w_kv, range(P // 2 + 1, P), 2)
            for cp in copies + [cp_c(nb - 2), cp_c(nb - 1)] + cp_early() + early + late + [cp_wo()]:
                cp.start()
            first_pair()
            loop(1, P - 1, middle_pair, 0)
            last_pair()
            for cp in early:
                cp.wait()

        def keys_values(c, w_kv, u_sum, b_sum, start, a32, v32, lhs, a_fix, v_fix, u_fix, b_fix):
            def u_block(j, k):
                return c[j * D:(j + 1) * D, k * T:(k + 1) * T]

            def weights(t, j, pair):
                return w_kv[t // 2, pair, j * T:(j + 1) * T, t % 2 * T:(t % 2 + 1) * T]

            def groups():
                return [(j, k) for j in range(0, nb, 2) for k in range(0, nb, 2)]

            def add_group(first, second, t, j, k, m):
                for e in range(2):
                    first[k + e, t] = first[k + e, t] + (m[0][e] + m[1][e])
                    second[j + e, t] = second[j + e, t] + (m[e][0] + m[e][1])

            def stage_jobs(i):
                shift = (1 - (i & 1)) * 16
                shift = shift if isinstance(i, int) else shift.astype(U32)

                def a_job(j, r, pin):
                    a32[j, r:r + 64, :] = _after(c[pl.ds(start_of(i, D) + r, 64), j * T:(j + 1) * T], pin).astype(F32)

                def v_job(k, t, r, pin):
                    w = w_kv[t // 2, P // 2 + (i >> 1), k * T + r:k * T + r + 64, t % 2 * T:(t % 2 + 1) * T]
                    v32[k, t, r:r + 64, :] = pltpu.bitcast((_after(w, pin) << shift) & U32(0xFFFF0000), F32)

                return ([functools.partial(a_job, j, r) for j in range(nb) for r in range(0, D, 64)]
                        + [functools.partial(v_job, k, t, r) for k in range(nb) for t in range(4) for r in range(0, T, 64)])

            def common(u, carry):
                marks = []
                for ch in range(2):
                    first, second, sums = {}, {}, {}
                    for j, k in groups():
                        m = [[None, None], [None, None]]
                        for dj in range(2):
                            w = w_kv[u, k // 2, (j + dj) * T:(j + dj + 1) * T, ch * T:(ch + 1) * T]
                            b = pltpu.bitcast(w << 16, F32), pltpu.bitcast(w & U32(0xFFFF0000), F32)
                            sums[j + dj] = sums[j + dj] + (b[0] + b[1]) if k else b[0] + b[1]
                            for dk in range(2):
                                m[dj][dk] = _dot(u_block(j + dj, k + dk), b[dk].astype(BF))
                        for e in range(2):
                            x, y = m[0][e] + m[1][e], m[e][0] + m[e][1]
                            first[k + e] = first[k + e] - x if j else -x
                            second[j + e] = second[j + e] - y if k else -y
                        marks += [m[0][0][r:r + 8] for r in range(0, D, 16)]
                    for n in range(nb):
                        start[2 * u + ch, n], start[2 * u + ch, nb + n], b_sum[2 * u + ch, n] = first[n], second[n], sums[n]
                _spread(stage_jobs(0), u >= 2, marks, 0, 0.9)
                return carry

            def plane(i, carry):
                never = i >= nb
                first = {(k, t): start[t, k] for k in range(nb) for t in range(4)}
                second = {(j, t): start[t, nb + j] for j in range(nb) for t in range(4)}
                marks = []
                for j, k in groups():
                    for dj in range(2):
                        for dk in range(2):
                            lhs[j + dj, k + dk] = (a32[j + dj] + u_block(j + dj, k + dk).astype(F32)).astype(BF)
                    for t in range(4):
                        m = [[None, None], [None, None]]
                        for dj in range(2):
                            w = weights(t, j + dj, k // 2)
                            b = pltpu.bitcast(w << 16, F32), pltpu.bitcast(w & U32(0xFFFF0000), F32)
                            for dk in range(2):
                                m[dj][dk] = _dot(lhs[j + dj, k + dk], (b[dk] + v32[k + dk, t]).astype(BF))
                        add_group(first, second, t, j, k, m)
                        marks += [m[0][0][r:r + 8] for r in range(0, D, 16)]

                def a_job(r, pin):
                    a = [_after(a32[j, r:r + 16, :], pin) for j in range(nb)]
                    total = functools.reduce(jnp.add, a)
                    for n in range(nb):
                        a_fix[n, r:r + 16, :] = a[n].astype(BF)
                        u_fix[n, r:r + 16, :] = (total + u_sum[n, r:r + 16, :]).astype(BF)

                def v_job(t, r, pin):
                    v = [_after(v32[k, t, r:r + 16, :], pin) for k in range(nb)]
                    total = functools.reduce(jnp.add, v)
                    for n in range(nb):
                        v_fix[n, t, r:r + 16, :] = v[n].astype(BF)
                        b_fix[n, t, r:r + 16, :] = (total + b_sum[t, n, r:r + 16, :]).astype(BF)

                jobs = [functools.partial(a_job, r) for r in range(0, D, 16)]
                jobs += [functools.partial(v_job, t, r) for t in range(4) for r in range(0, T, 16)]
                _spread(jobs, never, marks, 0.02, 0.95)
                marks = []
                for n in range(nb):
                    v = _cat([v_fix[n, t] for t in range(4)], axis=1)
                    x = _dot(u_fix[n], v)
                    for t in range(4):
                        kv_all[n, t, pl.ds(start_of(i, D), D), :] = (first[n, t] - x[:, t * T:(t + 1) * T]).astype(BF)
                    y = _dot(a_fix[n], _cat([b_fix[n, t] for t in range(4)], axis=1))
                    for t in range(4):
                        kv_all[nb + i, t, n * D:(n + 1) * D, :] = (second[n, t] - y[:, t * T:(t + 1) * T]).astype(BF)
                    marks += [z[r:r + 8, :T] for z in (x, y) for r in range(0, D, 16)]
                _spread(stage_jobs(jnp.minimum(i + 1, nb - 1)), never, marks, 0, 0.95)
                return carry

            loop(0, 2, common, 0)
            for cp in cp_kv(w_kv, range(P // 2 + 1, P), 2):
                cp.wait()
            loop(0, nb, plane, 0)

        def attention(q9, k9, v9, ctx7, wo7, outT, *inv_sums):
            def cp_out(i):
                return pltpu.make_async_copy(outT.at[i], outT_hbm.at[:, pl.ds(i * D, D)], sem.at[0])

            def operand_jobs(kind, h, g):
                def job(r, pin):
                    if kind == "Q":
                        words = [q_all.bitcast(U32)[h, k, (g * T + r) // 2:(g * T + r) // 2 + 8, :] for k in range(4)]
                    else:
                        words = [kv_all.bitcast(U32)[h, 2 * (kind == "V") + ch, (g * D + rh * T + r) // 2:(g * D + rh * T + r) // 2 + 8, :]
                                 for rh in range(2) for ch in range(2)]
                    a = [pltpu.bitcast(_after(w, pin), BF).astype(F32) for w in words]
                    if kind == "Q":
                        ops = _operands(_LHS, a)
                    else:
                        ops = _operands(_RHS, a if kind == "V" else (a[0], a[2], a[1], a[3]))
                    for n, t in enumerate(ops + (a[1], a[2])):
                        {"Q": q9, "K": k9, "V": v9}[kind][n, g * T + r:g * T + r + 16, :] = t.astype(BF)

                return [functools.partial(job, r) for r in range(0, T, 16)]

            def head(h, carry):
                never = h >= H
                clock, scores_of, last_use = [], {}, {}

                def tick(x, tiles):
                    n = max(1, x.shape[0] * tiles // 64)
                    clock.extend(x[(k * (x.shape[0] // 8) // n) * 8:][:8, -T:] for k in range(n))
                    return x

                def wo_job(r, pin):
                    quads = [_after(woT[h, rh * Mh + r:rh * Mh + r + 16, ch * T:(ch + 1) * T], pin).astype(F32)
                             for rh in range(2) for ch in range(2)]
                    for n, t in enumerate(_operands(_LHS, quads)):
                        wo7[n, r:r + 16, :] = t.astype(BF)

                def scores(i):
                    r = slice(i * T, (i + 1) * T)
                    q_top, q_bot = _cat([q9[2, r, :], q9[7, r, :]], axis=1), _cat([q9[8, r, :], q9[3, r, :]], axis=1)
                    past = [[], [], [], []]
                    if i:
                        m = [None] * 7
                        for n in sord:
                            m[n] = tick(_dot_nt(q9[n, r, :], k9[n, :i * T, :]), i)
                            yield i
                        past = [[s[:, t * T:(t + 1) * T] for t in range(i)] for s in _combine(m, sord)]
                    d1 = tick(_dot_nt(_cat([q_top, q_bot], axis=0), _cat([k9[1, r, :], k9[7, r, :]], axis=1)), 3)
                    d2 = _dot_nt(q_bot, _cat([k9[8, r, :], k9[4, r, :]], axis=1))
                    yield 6
                    causal = lax.broadcasted_iota(jnp.int32, (T, T), 1) <= lax.broadcasted_iota(jnp.int32, (T, T), 0)
                    diagonal = [jnp.where(causal, d1[:T], -1e9)], [d1[T:], jnp.where(causal, d2, -1e9)]
                    rows = []
                    for u in range(2):
                        first, second = sorted((2 * u, 2 * u + 1), key=lambda k: max(sord.index(n) for n in _OUT[k]))
                        row_max = functools.reduce(jnp.maximum, past[first] + past[second] + diagonal[u])
                        rows.append((past[2 * u] + past[2 * u + 1] + diagonal[u],
                                     jnp.max(row_max, axis=1, keepdims=True)))
                    scores_of[i] = rows, len(clock)
                    last_use.update({("K", g): len(clock) for g in range(i + 1)})
                    last_use["Q", i] = len(clock)

                def attend(i):
                    rows, since = scores_of.pop(i)
                    r = slice(i * T, (i + 1) * T)
                    exps, sums = {}, {}

                    def timed(k):
                        if k not in exps:
                            exps[k] = []
                            where = [(0, -1), (1, -2), (1, -1)] if k == 4 else [(k // 2, k % 2 * i + t) for t in range(i)]
                            for t, (u, idx) in enumerate(where):
                                tiles, row_max = rows[u]
                                parts = []
                                for r0 in range(0, T, 16):
                                    at = min(len(clock) - 1, max(since - 1, len(clock) - lead + t // 4 * 8 + r0 // 16))
                                    parts.append(jnp.exp2(tiles[idx][r0:r0 + 16] - _after(
                                        jnp.broadcast_to(row_max[r0:r0 + 16], (16, T)), (never, clock[at]))))
                                exps[k].append(_cat(parts, axis=0))
                                sums[u] = sums[u] + exps[k][-1] if u in sums else exps[k][-1]
                        return exps[k]

                    if i in timed_exp:
                        def p7(n, t):
                            return _operand(_LHS[n], lambda k: timed(k)[t])
                    else:
                        top, bot = ([jnp.exp2(t - row_max) for t in tiles] for tiles, row_max in rows)
                        ops = [_operands(_LHS, (top[t], top[i + t], bot[t], bot[i + t])) for t in range(i)]

                        def p7(n, t):
                            return ops[t][n]

                    m = [None] * 7
                    for n in pord if i else ():
                        m[n] = tick(_dot(_cat([p7(n, t) for t in range(i)], axis=1).astype(BF), v9[n, :i * T, :]), i)
                        yield i
                    if i in timed_exp:
                        diagonal = timed(4)
                        for u in range(2):
                            inv_sums[i][u * T:(u + 1) * T, :] = jnp.broadcast_to(_inverse_row_sum(sums[u]), (T, T))
                    else:
                        diagonal = [top[-1], bot[-2], bot[-1]]
                    d1 = tick(_dot(_cat(diagonal[:2], axis=0).astype(BF), _cat([v9[1, r, :], v9[7, r, :]], axis=1)), 3)
                    d2 = _dot(diagonal[2].astype(BF), _cat([v9[8, r, :], v9[4, r, :]], axis=1))
                    yield 6
                    last_use.update({("V", g): len(clock) for g in range(i + 1)})
                    o = [d1[:T, :T], d1[:T, T:], d1[T:, :T] + d2[:, :T], d1[T:, T:] + d2[:, T:]]
                    if i:
                        o = [a + b for a, b in zip(o, _combine(m, pord))]
                    if i in timed_exp:
                        zero = pl.multiple_of((h >> H.bit_length() - 1) * T, T)
                        inv = inv_sums[i][pl.ds(zero, T), :], inv_sums[i][pl.ds(zero + T, T), :]
                    else:
                        inv = []
                        for e, late in ((top, o[0]), (bot, o[3])):
                            partial_sums = functools.reduce(jnp.add, e)
                            if i in late_sum:
                                partial_sums = jnp.where(never, late, partial_sums)
                            inv.append(_inverse_row_sum(partial_sums))
                    ctx = (o[0] * inv[0], o[2] * inv[1], o[1] * inv[0], o[3] * inv[1])
                    for n, t in enumerate(_operands(_RHS, ctx)):
                        ctx7[n, r, :] = t.astype(BF)

                def out_proj(lo, hi):
                    m = [None] * 7
                    for n in oord:
                        m[n] = tick(_dot_nt(wo7[n], ctx7[n, lo * T:hi * T, :]), hi - lo)
                        yield 1.75 * (hi - lo)
                    for k, a in enumerate(_combine(m, oord)):
                        rows, cols = slice(k // 2 * Mh, (k // 2 + 1) * Mh), slice(k % 2 * T, (k % 2 + 1) * T)
                        for i in range(lo, hi):
                            total = acc[i, rows, cols] + gate[i, :, cols] * a[:, (i - lo) * T:(i - lo + 1) * T]
                            acc[i, rows, cols] = total
                            outT[i, rows, cols] = total.astype(BF)

                    @pl.when(h == H - 1)
                    def _():
                        for i in range(lo, hi):
                            cp_out(i).start()

                def begin(step):
                    kind, (lo, _, hi) = step[0], step[1:].partition("-")
                    lo, hi = int(lo), int(hi or lo) + 1
                    if kind == "O":
                        return [out_proj(lo, hi), 12.25 * (hi - lo), 0]
                    return [(scores if kind == "S" else attend)(lo), 7 * lo + 6, 0]

                staged = False
                for group in prog.split():
                    if not staged and "P" in group:
                        staged = True
                        jobs = [job for g in range(vnow) for job in operand_jobs("V", h, g)]
                        _spread(jobs + [functools.partial(wo_job, r) for r in range(0, Mh, 16)], never, clock, 0, 0.85)
                    running = [begin(step) for step in group.split("+")]
                    while running:
                        step = min(running, key=lambda s: s[2] / s[1])
                        try:
                            step[2] += next(step[0])
                        except StopIteration:
                            running.remove(step)
                at = 0
                for (kind, g), free in sorted(last_use.items(), key=lambda item: item[1]):
                    if kind != "V" or g >= vnow:
                        at = min(max(at, free + delay), len(clock) - span)
                        at = max(at, min(free, len(clock) - 1))
                        _spread(operand_jobs(kind, jnp.minimum(h + 1, H - 1), g), never, clock[at:at + span], 0, 1)
                        at += span
                return carry

            if not head_only:
                cp_wo().wait()
                for kind in "QKV":
                    for g in range(vnow if kind == "V" else 0, nb):
                        for job in operand_jobs(kind, 0, g):
                            job(None)
            loop(0, H, head, 0)
            for i in range(nb):
                cp_out(i).wait()

        def cp_kv(w_kv, pairs, slot):
            return [pltpu.make_async_copy(src.bitcast(U32).at[:, j, :], w_kv.at[u, j], sem.at[slot])
                    for u, src in enumerate((wuk_hbm, wuv_hbm)) for j in pairs]

        def cp_wo():
            return pltpu.make_async_copy(woT_hbm, woT, sem.at[3])

        def projections(*shared):
            if not plane_only:
                pl.run_scoped(
                    functools.partial(queries, *shared),
                    vmem((nb, M, D), BF), vmem((P, M, D), U32), vmem((M,), BF), vmem((M,), BF),
                    vmem((M, F), BF), vmem((M, F), BF), vmem((M, F), BF),
                    vmem((7, S // 2, D), BF), vmem((7, D, D), BF), vmem((7, D, D), BF),
                    vmem((2, M, T), F32), vmem((nb, 1, D), F32))
            pl.run_scoped(
                functools.partial(keys_values, *shared),
                vmem((4, nb, T, T), F32), vmem((4, 2 * nb, D, T), F32), vmem((nb, D, T), F32), vmem((nb, 4, T, T), F32),
                vmem((nb, nb, D, T), BF), vmem((nb, D, T), BF), vmem((nb, 4, T, T), BF), vmem((nb, D, T), BF),
                vmem((nb, 4, T, T), BF))

        if not head_only:
            pl.run_scoped(projections, vmem((S, Dc), BF), vmem((2, P, Dc, D), U32), vmem((nb, D, T), F32))
        pl.run_scoped(
            attention, *[vmem((9, S // 2, T), BF)] * 3, vmem((7, S // 2, T), BF), vmem((7, Mh, T), BF),
            vmem((nb, M, D), BF), *[vmem((D, T), F32)] * nb)

    def fn(A_x, A_c_kv, A_w_q, A_w_uk, A_w_uv, A_w_o, B_x, B_w_r, B_w_gate, B_w_up, B_w_down, gate_w):
        del B_x
        _, S, M = A_x.shape
        Dc = A_c_kv.shape[2]
        _, H, D = A_w_q.shape
        F = B_w_gate.shape[1]
        nb = S // D
        assert (D, nb, H) == (2 * T, 8, 16) and A_c_kv.shape[:2] == (1, S)
        vmem = pltpu.VMEM
        outT = pl.pallas_call(
            kernel,
            name=name,
            in_specs=[pl.BlockSpec(memory_space=pl.ANY)] * 11,
            out_specs=pl.BlockSpec(memory_space=pl.ANY),
            out_shape=jax.ShapeDtypeStruct((M, S), BF),
            scratch_shapes=[
                vmem((H, M, D), BF),
                vmem((H, 4, S // 2, T), BF),
                vmem((H, 4, S, T), BF),
                vmem((nb, 1, D), F32),
                vmem((nb, M, D), F32),
                pltpu.SemaphoreType.DMA((4,)),
                pltpu.SemaphoreType.DMA((len(_FIRST_PASS),)),
                pltpu.SemaphoreType.DMA((H // 2 + 1,)),
            ],
            compiler_params=pltpu.CompilerParams(vmem_limit_bytes=124 * 2**20, disable_bounds_checks=nocheck,
                                                 disable_semaphore_checks=nocheck),
        )(A_x[0].T, A_c_kv[0], A_w_q, A_w_uk, A_w_uv, jnp.swapaxes(A_w_o, 1, 2), B_w_r, gate_w,
          B_w_gate, B_w_up, B_w_down.T)
        return outT.T[None]

    return fn


_impl = make(prog='S7 S6 P7 P6 S5 S4 O6-7 S3 P4+P5 S1 P3 O4-5 S2 S0+P2 P0 P1 O2-3 O0 O1',sord=[1, 2, 0, 5, 3, 6, 4],pord=[2, 4, 0, 5, 1, 3, 6],oord=[0, 1, 3, 4, 5, 6, 2],late_sum=[0, 1, 5, 6, 7],timed_exp=[4, 5],lead=32,vnow=5,span=40,delay=16)


@jax.jit
def pallas_gated_mix__compressed_kv_cla__moe_arch_mod__prompt_kernel(
    A_x, A_c_kv, A_w_q, A_w_uk, A_w_uv, A_w_o, B_x, B_w_r, B_w_gate, B_w_up, B_w_down, gate_w,
):
    return _impl(A_x, A_c_kv, A_w_q, A_w_uk, A_w_uv, A_w_o, B_x, B_w_r, B_w_gate, B_w_up, B_w_down, gate_w)
```

```python
import functools
import math

import jax
import jax.numpy as jnp
from jax import lax
import jax.experimental.pallas as pl
import jax.experimental.pallas.tpu as pltpu

BF = jnp.bfloat16
F32 = jnp.float32
U32 = jnp.uint32
T = 128
_cat = jnp.concatenate

_HEAD_PROGRAM = "S7 S6 P7 S4 P6 S5 O6-7 S3 P4+P5 S1 P3 O4 O5 S2 S0+P2 P0+P1 O2-3 O0 O1"
_FIRST_PASS = (((0, 1), ()), ((1, 1), (0, 1)), ((1, 3), (1, 2)), ((3, 6), (2, 3, 5)), ((6, 8), (5, 6, 8)))

_LHS = ((0, 1, 3), (2, 1, 3), (0,), (3,), (0, 1, 1), (2, -1, 0), (1, -1, 3))
_RHS = ((0, 1, 3), (0,), (1, -1, 3), (2, -1, 0), (3,), (0, 1, 1), (2, 1, 3))
_OUT = ({0: 1, 3: 1, 4: -1, 6: 1}, {2: 1, 4: 1}, {1: 1, 3: 1}, {0: 1, 1: -1, 2: 1, 5: 1})


def _operand(rule, quadrant):
    if len(rule) == 1:
        return quadrant(rule[0])
    a, b = quadrant(rule[0]), quadrant(rule[2])
    return a + b if rule[1] > 0 else a - b


def _operands(rules, quads):
    return tuple(_operand(rule, quads.__getitem__) for rule in rules)


def _combine(m, order):
    out = []
    for k, signs in enumerate(_OUT):
        ns = [n for n in order if n in signs]
        if len(ns) == 4:
            ns = ns[::-1] if k == 3 else [ns[2], ns[1], ns[0], ns[3]]
        acc, sign = m[ns[0]], signs[ns[0]]
        for n in ns[1:]:
            if sign > 0:
                acc = acc + m[n] if signs[n] > 0 else acc - m[n]
            else:
                acc, sign = m[n] - acc, 1
        out.append(acc)
    return out


def _dot(a, b):
    return jnp.dot(a, b, preferred_element_type=F32)


def _dot_nt(a, b):
    return lax.dot_general(a, b, (((1,), (1,)), ((), ())), preferred_element_type=F32)


def _sigmoid(z):
    return 1.0 / (1.0 + jnp.exp(-z))


def _inverse_row_sum(partial_sums):
    l = jnp.sum(partial_sums, axis=1, keepdims=True)
    r = pl.reciprocal(l, approx=True)
    return r * (2.0 - l * r)


def _head_of(words, odd):
    if isinstance(odd, int):
        return pltpu.bitcast(words & U32(0xFFFF0000) if odd else words << 16, F32)
    return pltpu.bitcast((words << ((1 - odd) * 16).astype(U32)) & U32(0xFFFF0000), F32)


def _after(x, pin):
    if pin is None:
        return x
    never, late = pin
    bits, late = pltpu.bitcast(x, U32), pltpu.bitcast(late, U32)
    out = _cat([_cat([jnp.where(never, late, bits[r:r + 8, u:u + T]) for u in range(0, bits.shape[1], T)], axis=1)
                for r in range(0, bits.shape[0], 8)], axis=0)
    return pltpu.bitcast(out, x.dtype)


def _spread(jobs, never, marks, lo, hi):
    for k, job in enumerate(jobs):
        job((never, marks[int(len(marks) * (lo + (hi - lo) * k / len(jobs)))]))


def make(prog=_HEAD_PROGRAM, qord=(0, 1, 2, 5, 3, 4, 6), sord=(1, 2, 0, 3, 5, 6, 4), pord=(2, 4, 0, 5, 1, 6, 3),
         oord=(0, 1, 2, 4, 3, 5, 6), late_sum=(0, 1, 6, 7), timed_exp=(4, 5), lead=32, vnow=2, qnow=4, delay=32, tail=12,
         room_s=(4, 4, 3, 1, 1, 1, 1, 1), room_p=(1, 1, 2, 4, 8, 7, 6, 3), room_o=(4, 5, 3, 2, 1, 0, 0),
         head_only=False, name="kb"):
    def kernel(xT_hbm, c_hbm, wq_hbm, wuk_hbm, wuv_hbm, woT_hbm, wr_hbm, gw_hbm, wg_hbm, wu_hbm, wdT_hbm, outT_hbm,
               woT, q_all, kv_all, q9, k9, v9, gate, acc, sem, sem_x, sem_q, sem_c):
        nb, M, D = acc.shape
        S, H, Dc, F = nb * D, q_all.shape[0], c_hbm.shape[1], wg_hbm.shape[1]
        P, Mh = H // 2, M // 2
        q_scale = D ** -0.5 * math.log2(math.e)
        vmem = pltpu.VMEM

        def start_of(i, size):
            return i * size if isinstance(i, int) else pl.multiple_of(i * size, size)

        def cp_kv(w_kv, late):
            return [pltpu.make_async_copy((wuk_hbm, wuv_hbm)[t // 2].bitcast(U32).at[:, j, pl.ds(t % 2 * T, T)],
                                          w_kv.at[t, j], sem.at[1 + late])
                    for t in range(4) for j in range(P) if (j > P // 2) == late]

        def cp_wo():
            return pltpu.make_async_copy(woT_hbm, woT, sem.at[3])

        def put_operands(kind, rows, a):
            if kind == "Q":
                ops = _operands(_LHS, a)
            else:
                ops = _operands(_RHS, a if kind == "V" else (a[0], a[2], a[1], a[3]))
            for n, t in enumerate(ops + (a[1], a[2])):
                {"Q": q9, "K": k9, "V": v9}[kind][n, rows, :] = t.astype(BF)

        def operand_jobs(kind, h, g):
            def job(r, pin):
                if kind == "Q":
                    words = [q_all.bitcast(U32)[h, k, pl.ds((g * T + r) // 2, 8), :] for k in range(4)]
                else:
                    words = [kv_all.bitcast(U32)[h, 2 * (kind == "V") + ch, pl.ds((g * D + rh * T + r) // 2, 8), :]
                             for rh in range(2) for ch in range(2)]
                put_operands(kind, pl.ds(g * T + r, 16), [pltpu.bitcast(_after(w, pin), BF).astype(F32) for w in words])

            return [functools.partial(job, r) for r in range(0, T, 16)]

        def queries(c, w_kv, u_sum, xT, wq, wr, gw, wg, wu, wdT, x7, wq7, vec_cols, score):
            def cp_x(i):
                group = [lo <= i < hi for (lo, hi), _ in _FIRST_PASS].index(True)
                return pltpu.make_async_copy(xT_hbm.at[:, pl.ds(i * D, D)], xT.at[i], sem_x.at[group])

            def cp_q(j):
                return pltpu.make_async_copy(wq_hbm.bitcast(U32).at[:, j, :], wq.at[j], sem_q.at[j])

            def cp_c(i):
                rows = pl.ds(start_of(i, 2 * D), 2 * D)
                return pltpu.make_async_copy(c_hbm.at[rows, :], c.at[rows, :], sem_c.at[i])

            def cp_vectors():
                return [pltpu.make_async_copy(src, dst, sem_q.at[1]) for src, dst in ((wr_hbm, wr), (gw_hbm, gw))]

            def cp_ffn():
                return [pltpu.make_async_copy(src, dst, sem.at[0])
                        for src, dst in ((wg_hbm, wg), (wu_hbm, wu), (wdT_hbm, wdT))]

            def build_x7(i):
                xt = xT[i].astype(F32)
                pad = jnp.zeros((D - Mh, T), F32)
                quads = [_cat([t, pad], axis=0).T for t in (xt[:Mh, :T], xt[Mh:, :T], xt[:Mh, T:], xt[Mh:, T:])]
                for n, t in enumerate(_operands(_LHS, quads)):
                    x7[n, i * T:(i + 1) * T, :] = t.astype(BF)

            def wq_quadrant(h, r, pin, k):
                return _head_of(_after(wq[h >> 1, pl.ds(k // 2 * Mh + r, 16), pl.ds(k % 2 * T, T)], pin), h & 1)

            def wq7_jobs(h, slot):
                def job(r, pin):
                    for n, t in enumerate(_operands(_RHS, [wq_quadrant(h, r, pin, k) for k in range(4)])):
                        wq7[slot, n, r:r + 16, :] = t.astype(BF)

                return [functools.partial(job, r) for r in range(0, Mh, 16)]

            def u_sum_jobs(i, fresh):
                def job(k, r, pin):
                    t = _after(c[pl.ds(start_of(i, D) + r, 64), k * T:(k + 1) * T], pin).astype(F32)
                    u_sum[k, r:r + 64, :] += jnp.where(fresh, t, 0.0)

                return [functools.partial(job, k, r) for k in range(nb) for r in range(0, D, 64)]

            def gate_jobs(i):
                sums = {}

                def job(t, r, pin):
                    cols = slice(t * T, (t + 1) * T)
                    xt = _after(xT[i, r:r + 32, cols], pin).astype(F32)
                    for u in range(2):
                        p = xt * vec_cols[u, r:r + 32, :]
                        p = (p[0:8] + p[8:16]) + (p[16:24] + p[24:32])
                        sums[u] = p if r == 0 else sums[u] + p
                    if r + 32 == M:
                        score[i, :, cols] = jnp.sum(sums[0], axis=0, keepdims=True)
                        gate[i, :, cols] = _sigmoid(jnp.sum(sums[1], axis=0, keepdims=True))

                return [functools.partial(job, t, r) for t in range(2) for r in range(0, M, 32)]

            def residual_jobs(i):
                keep = []

                def job(r, pin):
                    if not keep:
                        keep.append(1.0 - gate[i])
                    acc[i, r:r + 16, :] = keep[0] * _after(xT[i, r:r + 16, :], pin).astype(F32)

                return [functools.partial(job, r) for r in range(0, M, 16)]

            def route():
                def whole(op, t):
                    return op(op(t, axis=0, keepdims=True), axis=1, keepdims=True)

                r = _cat([score[i] for i in range(nb)], axis=0).astype(BF).astype(F32)
                tok = lax.broadcasted_iota(jnp.int32, (nb, D), 0) * D + lax.broadcasted_iota(jnp.int32, (nb, D), 1)
                bits = pltpu.bitcast(jnp.where(r == 0.0, 0.0, r), jnp.int32) >> 16
                rank = jnp.where(r != r, 0, jnp.where(bits < 0, bits ^ 0x7FFF, bits) + 0x8000)
                key = pltpu.bitcast(0x20000000 + rank * S + (S - 1 - tok), F32)
                lane = lax.broadcasted_iota(jnp.int32, (1, D), 1)
                picks = []
                for _ in range(2):
                    best = whole(jnp.max, key)
                    idx = S - 1 - (pltpu.bitcast(best, jnp.int32)[0, 0] & (S - 1))
                    weight = _sigmoid(whole(jnp.sum, jnp.where(key == best, r, 0.0)))
                    picks.append((idx >> (D.bit_length() - 1), lane == (idx & (D - 1)), weight))
                    key = jnp.where(key == best, 0.0, key)
                return picks

            def gather(picks):
                row = lax.broadcasted_iota(jnp.int32, (16, D), 0)
                return sum(_dot_nt(jnp.where((row == u) & hot, 1.0, 0.0).astype(BF), xT[b])
                           for u, (b, hot, _) in enumerate(picks)).astype(BF)

            def scatter_jobs(y, picks):
                def job(b, hot, col, keep, r, pin):
                    yr = _after(col[r:r + 32], pin)
                    acc[b, r:r + 32, :] += jnp.where(hot, keep * _cat([yr, yr], axis=1), 0.0)

                jobs = []
                for u, (b, hot, weight) in enumerate(picks):
                    col = jnp.broadcast_to(y[u:u + 1] * weight, (T, M)).T
                    keep = 1.0 - gate[b]
                    jobs += [functools.partial(job, b, hot, col, keep, r) for r in range(0, M, 32)]
                return jobs

            def q_proj(h, slots, lo, hi, before=None):
                m = [None] * 7
                for k, n in enumerate(qord):
                    if before is not None:
                        before(k)
                    m[n] = _dot(x7[n, lo * T:hi * T, :], _cat([wq7[slot, n] for slot in slots], axis=1))
                for e in range(len(slots)):
                    for k, t in enumerate(_combine([t[:, e * T:(e + 1) * T] for t in m], qord)):
                        q_all[h + e, k, lo * T:hi * T, :] = (t * q_scale).astype(BF)
                return [m[n][r:r + 8, :T] for n in qord for r in range(0, (hi - lo) * T, 16)]

            def never_set():
                t = xT[0, :16, :T].astype(F32)[:8]
                return t * t < 0.0

            def first_pair():
                u_sum[...] = jnp.zeros(u_sum.shape, F32)
                wq7[:, :, Mh:, :] = jnp.zeros((3, 7, D - Mh, T), BF)
                for s, (arrived, projected) in enumerate(_FIRST_PASS):
                    for i in range(*arrived):
                        cp_x(i).wait()
                    if s == 1:
                        cp_q(0).wait()
                        for both in zip(wq7_jobs(0, 1), wq7_jobs(1, 2)):
                            for job in both:
                                job(None)
                    if s == len(_FIRST_PASS) - 1:
                        for cp in [cp_q(1)] + cp_vectors():
                            cp.wait()
                    for i in range(*arrived):
                        build_x7(i)
                    marks = [t for lo, hi in zip(projected, projected[1:]) for t in q_proj(0, (1, 2), lo, hi)]
                for u, ref in enumerate((wr, gw)):
                    vec_cols[u] = jnp.broadcast_to(ref[...].astype(F32).reshape(1, M), (T, M)).T
                _spread(wq7_jobs(2, 0), never_set(), marks, 0.35, 0.7)

            def middle_head(h, carry):
                @pl.when((h & 1) == 1)
                def _():
                    cp_q((h + 1) >> 1).wait()

                @pl.when(jnp.logical_and((h & 1) == 0, h - 2 < nb))
                def _():
                    cp_c((h - 2) >> 1).wait()

                never = h >= H
                marks, rest = q_proj(h, (0,), 0, nb // 2), q_proj(h, (0,), nb // 2, nb)
                i = jnp.minimum(h - 2, nb - 1)
                _spread(gate_jobs(i) + u_sum_jobs(i, h - 2 < nb) + residual_jobs(i), never, marks + rest, 0, 0.75)

                def next_weights(n, r, pin):
                    wq7[0, n, r:r + 16, :] = _operand(_RHS[n], functools.partial(wq_quadrant, h + 1, r, pin)).astype(BF)

                for k, n in enumerate(qord):
                    jobs = [functools.partial(next_weights, n, r) for r in range(0, Mh, 16)]
                    _spread(jobs, never, rest, k / 7 + 0.005, k / 7 + 0.1)
                return carry

            def last_pair():
                for cp in cp_ffn():
                    cp.wait()
                for job in wq7_jobs(H - 1, 1):
                    job(None)
                picks, never = route(), never_set()
                xs, hidden, y = [], [], []

                def take(k):
                    if k == 1:
                        xs.append(gather(picks))

                def up(step, k):
                    for t in range((step + k) * 2 * (F // T) // 21, (step + k + 1) * 2 * (F // T) // 21):
                        hidden.append(_dot(xs[0], (wg, wu)[t % 2][:, t // 2 * T:(t // 2 + 1) * T]))

                def down(step, k):
                    for t in range((step + k) * (F // T) // 14, (step + k + 1) * (F // T) // 14):
                        g, u = hidden[2 * t], hidden[2 * t + 1]
                        y.append(_dot_nt((g * _sigmoid(g) * u).astype(BF), wdT[:, t * T:(t + 1) * T]))

                extras = ([None, take] + [functools.partial(up, 7 * s) for s in range(3)]
                          + [functools.partial(down, 7 * s) for s in range(2)])
                marks = [t for i, extra in enumerate(extras) for t in q_proj(H - 2, (0, 1), i, i + 1, extra)]
                y = functools.reduce(jnp.add, y)
                rest = q_proj(H - 2, (0, 1), nb - 1, nb)
                _spread([job for g in range(qnow, nb) for job in operand_jobs("Q", 0, g)], never, marks, 0, 0.97)
                _spread(scatter_jobs(y, picks), never, rest, 0.3, 0.9)

            copies = [cp_x(0), cp_q(0)] + [cp_x(i) for i in range(1, nb)] + [cp_q(1)] + cp_vectors()
            for j in range(2, P):
                copies += ([cp_c(j - 2)] if j - 2 < nb // 2 else []) + [cp_q(j)]
            for cp in copies + cp_ffn() + cp_kv(w_kv, False) + cp_kv(w_kv, True) + [cp_wo()]:
                cp.start()
            first_pair()
            lax.fori_loop(2, H - 2, middle_head, 0)
            last_pair()

        def keys_values(c, w_kv, u_sum, b_sum, common, a32, v32, lhs, a_fix, v_fix, u_fix, b_fix):
            groups = [(j, k) for j in range(0, nb, 2) for k in range(0, nb, 2)]

            def u_block(j, k):
                return c[j * D:(j + 1) * D, k * T:(k + 1) * T]

            def stage_jobs(i, tiles):
                def a_job(j, r, pin):
                    a32[j, r:r + 32, :] = _after(c[pl.ds(start_of(i, D) + r, 32), j * T:(j + 1) * T], pin).astype(F32)

                def v_job(k, t, r, pin):
                    words = w_kv[t, P // 2 + (i >> 1), pl.ds(k * T + r, 32), :]
                    v32[k, t, r:r + 32, :] = _head_of(_after(words, pin), i & 1)

                return ([functools.partial(a_job, j, r) for j in range(nb) for r in range(0, D, 32)]
                        + [functools.partial(v_job, k, t, r)
                           for k in range(nb) for t in tiles for r in range(0, T, 32)])

            def common_terms(t, carry):
                first, second, sums, marks = {}, {}, {}, []
                for j, k in groups:
                    m = [[None, None], [None, None]]
                    for dj in range(2):
                        words = w_kv[t, k // 2, pl.ds((j + dj) * T, T), :]
                        b = _head_of(words, 0), _head_of(words, 1)
                        sums[j + dj] = sums[j + dj] + (b[0] + b[1]) if k else b[0] + b[1]
                        for dk in range(2):
                            m[dj][dk] = _dot(u_block(j + dj, k + dk), b[dk].astype(BF))
                    for e in range(2):
                        over_j, over_k = m[0][e] + m[1][e], m[e][0] + m[e][1]
                        first[k + e] = first[k + e] - over_j if j else -over_j
                        second[j + e] = second[j + e] - over_k if k else -over_k
                    marks += [m[0][0][r:r + 8] for r in range(0, D, 16)]
                for n in range(nb):
                    common[t, n], common[t, nb + n], b_sum[t, n] = first[n], second[n], sums[n]
                _spread(stage_jobs(0, [t]), t >= 4, marks, 0, 0.7)
                return carry

            def plane(i, carry):
                never = i >= nb
                first = {(k, t): common[t, k] for k in range(nb) for t in range(4)}
                second = {(j, t): common[t, nb + j] for j in range(nb) for t in range(4)}
                marks = []
                for j, k in groups:
                    for dj in range(2):
                        for dk in range(2):
                            lhs[j + dj, k + dk] = (a32[j + dj] + u_block(j + dj, k + dk).astype(F32)).astype(BF)
                    for t in range(4):
                        m = [[None, None], [None, None]]
                        for dj in range(2):
                            words = w_kv[t, k // 2, pl.ds((j + dj) * T, T), :]
                            b = _head_of(words, 0), _head_of(words, 1)
                            for dk in range(2):
                                m[dj][dk] = _dot(lhs[j + dj, k + dk], (b[dk] + v32[k + dk, t]).astype(BF))
                        for e in range(2):
                            first[k + e, t] = first[k + e, t] + (m[0][e] + m[1][e])
                            second[j + e, t] = second[j + e, t] + (m[e][0] + m[e][1])
                        marks += [m[0][0][r:r + 8] for r in range(0, D, 16)]

                def a_job(r, pin):
                    a = [_after(a32[j, r:r + 16, :], pin) for j in range(nb)]
                    total = functools.reduce(jnp.add, a)
                    for n in range(nb):
                        a_fix[n, r:r + 16, :] = a[n].astype(BF)
                        u_fix[n, r:r + 16, :] = (total + u_sum[n, r:r + 16, :]).astype(BF)

                def v_job(t, r, pin):
                    v = [_after(v32[k, t, r:r + 16, :], pin) for k in range(nb)]
                    total = functools.reduce(jnp.add, v)
                    for n in range(nb):
                        v_fix[n, t, r:r + 16, :] = v[n].astype(BF)
                        b_fix[n, t, r:r + 16, :] = (total + b_sum[t, n, r:r + 16, :]).astype(BF)

                jobs = [functools.partial(a_job, r) for r in range(0, D, 16)]
                jobs += [functools.partial(v_job, t, r) for t in range(4) for r in range(0, T, 16)]
                _spread(jobs, never, marks, 0.1, 0.7)
                marks = []
                for n in range(nb):
                    x = _dot(u_fix[n], _cat([v_fix[n, t] for t in range(4)], axis=1))
                    done = [first[n, t] - x[:, t * T:(t + 1) * T] for t in range(4)]
                    for t in range(4):
                        kv_all[n, t, pl.ds(start_of(i, D), D), :] = done[t].astype(BF)
                    if n == 0:
                        for kind, (lo, hi) in (("K", done[:2]), ("V", done[2:])):
                            put_operands(kind, pl.ds(start_of(i, T), T), (lo[:T], hi[:T], lo[T:], hi[T:]))
                    y = _dot(a_fix[n], _cat([b_fix[n, t] for t in range(4)], axis=1))
                    for t in range(4):
                        kv_all[nb + i, t, n * D:(n + 1) * D, :] = (second[n, t] - y[:, t * T:(t + 1) * T]).astype(BF)
                    marks += [z[r:r + 8, :T] for z in (x, y) for r in range(0, D, 16)]
                _spread(stage_jobs(jnp.minimum(i + 1, nb - 1), range(4)), never, marks, 0, 0.95)
                return carry

            for cp in cp_kv(w_kv, False):
                cp.wait()
            lax.fori_loop(0, 4, common_terms, 0)
            for cp in cp_kv(w_kv, True) + [cp_wo()]:
                cp.wait()
            lax.fori_loop(0, nb, plane, 0)

        def attention(ctx7, wo7, outT, *inv_sums):
            def cp_out(i):
                return pltpu.make_async_copy(outT.at[i], outT_hbm.at[:, pl.ds(i * D, D)], sem.at[0])

            def head(h, carry):
                never = h >= H
                clock, room, scores_of, last_use = [], [], {}, {}

                def tick(x, tiles, free):
                    n = max(1, x.shape[0] * tiles // 64)
                    clock.extend(x[(k * (x.shape[0] // 8) // n) * 8:][:8, -T:] for k in range(n))
                    room.extend([free] * n)
                    return x

                def wo_job(r, pin):
                    quads = [_after(woT[h, pl.ds(rh * Mh + r, 16), pl.ds(ch * T, T)], pin).astype(F32)
                             for rh in range(2) for ch in range(2)]
                    for n, t in enumerate(_operands(_LHS, quads)):
                        wo7[n, r:r + 16, :] = t.astype(BF)

                def scores(i):
                    r = slice(i * T, (i + 1) * T)
                    q_top, q_bot = _cat([q9[2, r, :], q9[7, r, :]], axis=1), _cat([q9[8, r, :], q9[3, r, :]], axis=1)
                    past = [[], [], [], []]
                    if i:
                        m = [None] * 7
                        for n, free in zip(sord, room_s):
                            m[n] = tick(_dot_nt(q9[n, r, :], k9[n, :i * T, :]), i, free)
                            yield i
                        past = [[s[:, t * T:(t + 1) * T] for t in range(i)] for s in _combine(m, sord)]
                    d1 = _dot_nt(_cat([q_top, q_bot], axis=0), _cat([k9[1, r, :], k9[7, r, :]], axis=1))
                    d2 = _dot_nt(q_bot, _cat([k9[8, r, :], k9[4, r, :]], axis=1))
                    tick(d1, 3, room_s[7])
                    yield 6
                    causal = lax.broadcasted_iota(jnp.int32, (T, T), 1) <= lax.broadcasted_iota(jnp.int32, (T, T), 0)
                    diagonal = [jnp.where(causal, d1[:T], -1e9)], [d1[T:], jnp.where(causal, d2, -1e9)]
                    rows = []
                    for u in range(2):
                        first, second = sorted((2 * u, 2 * u + 1), key=lambda k: max(sord.index(n) for n in _OUT[k]))
                        row_max = functools.reduce(jnp.maximum, past[first] + past[second] + diagonal[u])
                        rows.append((past[2 * u] + past[2 * u + 1] + diagonal[u],
                                     jnp.max(row_max, axis=1, keepdims=True)))
                    scores_of[i] = rows, len(clock)
                    last_use.update({("K", g): len(clock) for g in range(i + 1)})
                    last_use["Q", i] = len(clock)

                def attend(i):
                    rows, since = scores_of.pop(i)
                    r = slice(i * T, (i + 1) * T)
                    exps, sums = {}, {}

                    def timed(k):
                        if k not in exps:
                            exps[k] = []
                            where = [(0, -1), (1, -2), (1, -1)] if k == 4 else [(k // 2, k % 2 * i + t) for t in range(i)]
                            for t, (u, idx) in enumerate(where):
                                tiles, row_max = rows[u]
                                parts = []
                                for r0 in range(0, T, 16):
                                    at = min(len(clock) - 1, max(since - 1, len(clock) - lead + t // 4 * 8 + r0 // 16))
                                    parts.append(jnp.exp2(tiles[idx][r0:r0 + 16] - _after(
                                        jnp.broadcast_to(row_max[r0:r0 + 16], (16, T)), (never, clock[at]))))
                                exps[k].append(_cat(parts, axis=0))
                                sums[u] = sums[u] + exps[k][-1] if u in sums else exps[k][-1]
                        return exps[k]

                    if i in timed_exp:
                        def p7(n, t):
                            return _operand(_LHS[n], lambda k: timed(k)[t])
                    else:
                        top, bot = ([jnp.exp2(t - row_max) for t in tiles] for tiles, row_max in rows)
                        ops = [_operands(_LHS, (top[t], top[i + t], bot[t], bot[i + t])) for t in range(i)]

                        def p7(n, t):
                            return ops[t][n]

                    m = [None] * 7
                    for n, free in zip(pord, room_p) if i else ():
                        p = _cat([p7(n, t) for t in range(i)], axis=1).astype(BF)
                        m[n] = tick(_dot(p, v9[n, :i * T, :]), i, free)
                        yield i
                    if i in timed_exp:
                        diagonal = timed(4)
                        for u in range(2):
                            inv_sums[i][u * T:(u + 1) * T, :] = jnp.broadcast_to(_inverse_row_sum(sums[u]), (T, T))
                    else:
                        diagonal = [top[-1], bot[-2], bot[-1]]
                    d1 = _dot(_cat(diagonal[:2], axis=0).astype(BF), _cat([v9[1, r, :], v9[7, r, :]], axis=1))
                    d2 = _dot(diagonal[2].astype(BF), _cat([v9[8, r, :], v9[4, r, :]], axis=1))
                    tick(d1, 3, room_p[7])
                    yield 6
                    last_use.update({("V", g): len(clock) for g in range(i + 1)})
                    o = [d1[:T, :T], d1[:T, T:], d1[T:, :T] + d2[:, :T], d1[T:, T:] + d2[:, T:]]
                    if i:
                        o = [a + b for a, b in zip(o, _combine(m, pord))]
                    if i in timed_exp:
                        zero = pl.multiple_of((h >> H.bit_length() - 1) * T, T)
                        inv = inv_sums[i][pl.ds(zero, T), :], inv_sums[i][pl.ds(zero + T, T), :]
                    else:
                        inv = []
                        for e, late in ((top, o[0]), (bot, o[3])):
                            partial_sums = functools.reduce(jnp.add, e)
                            if i in late_sum:
                                partial_sums = jnp.where(never, late, partial_sums)
                            inv.append(_inverse_row_sum(partial_sums))
                    ctx = (o[0] * inv[0], o[2] * inv[1], o[1] * inv[0], o[3] * inv[1])
                    for n, t in enumerate(_operands(_RHS, ctx)):
                        ctx7[n, r, :] = t.astype(BF)

                def out_proj(lo, hi):
                    m = [None] * 7
                    for n, free in zip(oord, room_o):
                        m[n] = tick(_dot_nt(wo7[n], ctx7[n, lo * T:hi * T, :]), hi - lo, free)
                        yield 1.75 * (hi - lo)
                    for k, a in enumerate(_combine(m, oord)):
                        rows, cols = slice(k // 2 * Mh, (k // 2 + 1) * Mh), slice(k % 2 * T, (k % 2 + 1) * T)
                        for i in range(lo, hi):
                            total = acc[i, rows, cols] + gate[i, :, cols] * a[:, (i - lo) * T:(i - lo + 1) * T]
                            acc[i, rows, cols] = total
                            outT[i, rows, cols] = total.astype(BF)

                    @pl.when(h == H - 1)
                    def _():
                        for i in range(lo, hi):
                            cp_out(i).start()

                def begin(step):
                    kind, (lo, _, hi) = step[0], step[1:].partition("-")
                    lo, hi = int(lo), int(hi or lo) + 1
                    if kind == "O":
                        return [out_proj(lo, hi), 12.25 * (hi - lo), 0]
                    return [(scores if kind == "S" else attend)(lo), 7 * lo + 6, 0]

                def fit(jobs, lo, hi):
                    for cost in range(256, 0, -1):
                        at, saved = [], 0
                        for t in range(lo, hi):
                            if len(at) < len(jobs) and min(jobs[len(at)][0], hi - 1) <= t:
                                saved += room[t]
                                if saved >= cost:
                                    saved = 0
                                    at.append(t)
                        if len(at) == len(jobs):
                            break
                    for k, (_, job) in enumerate(jobs):
                        job((never, clock[at[k] if k < len(at) else hi - 1]))

                def next_head_jobs(until):
                    def finished(kind, g):
                        users = range(g, g + 1 if kind == "Q" else nb)
                        return all(("P" if kind == "V" else "S") + str(t) not in ahead for t in users)

                    ready = [(free, kind, g) for (kind, g), free in last_use.items()
                             if free <= until and (kind, g) not in rebuilt and finished(kind, g)
                             and g >= {"Q": qnow, "K": 0, "V": vnow}[kind]]
                    rebuilt.update((kind, g) for _, kind, g in ready)
                    return [(free + delay, job) for free, kind, g in sorted(ready)
                            for job in operand_jobs(kind, jnp.minimum(h + 1, H - 1), g)]

                first_p, first_o, rebuilt, ahead = None, None, set(), prog.replace("+", " ").split()
                for group in prog.split():
                    if first_p is None and "P" in group:
                        first_p = len(clock)
                        fit([(0, job) for g in range(vnow) for job in operand_jobs("V", h, g)], 0, first_p - 2 * tail)
                    if first_o is None and "O" in group:
                        first_o = len(clock) - 2 * tail
                        jobs = [(0, functools.partial(wo_job, r)) for r in range(0, Mh, 16)]
                        jobs += [(0, job) for g in reversed(range(qnow)) for job in operand_jobs("Q", h, g)]
                        fit(jobs + next_head_jobs(first_o - 64), first_p, first_o)
                    assert first_o is not None or not any(f"S{g}" in group for g in range(qnow))
                    running = [begin(step) for step in group.split("+")]
                    while running:
                        step = min(running, key=lambda s: s[2] / s[1])
                        try:
                            step[2] += next(step[0])
                        except StopIteration:
                            running.remove(step)
                    ahead = [step for step in ahead if step not in group.split("+")]
                fit(next_head_jobs(len(clock)), first_o, len(clock) - tail)
                return carry

            lax.fori_loop(0, H, head, 0)
            for i in range(nb):
                cp_out(i).wait()

        def projections(*shared):
            pl.run_scoped(
                functools.partial(queries, *shared),
                xT=vmem((nb, M, D), BF), wq=vmem((P, M, D), U32), wr=vmem((M,), BF), gw=vmem((M,), BF),
                wg=vmem((M, F), BF), wu=vmem((M, F), BF), wdT=vmem((M, F), BF),
                x7=vmem((7, S // 2, D), BF), wq7=vmem((3, 7, D, T), BF),
                vec_cols=vmem((2, M, T), F32), score=vmem((nb, 1, D), F32))
            pl.run_scoped(
                functools.partial(keys_values, *shared),
                b_sum=vmem((4, nb, T, T), F32), common=vmem((4, 2 * nb, D, T), F32),
                a32=vmem((nb, D, T), F32), v32=vmem((nb, 4, T, T), F32), lhs=vmem((nb, nb, D, T), BF),
                a_fix=vmem((nb, D, T), BF), v_fix=vmem((nb, 4, T, T), BF),
                u_fix=vmem((nb, D, T), BF), b_fix=vmem((nb, 4, T, T), BF))

        if not head_only:
            pl.run_scoped(projections, vmem((S, Dc), BF), vmem((4, P, Dc, T), U32), vmem((nb, D, T), F32))
        pl.run_scoped(attention, vmem((7, S // 2, T), BF), vmem((7, Mh, T), BF), vmem((nb, M, D), BF),
                      *[vmem((D, T), F32)] * nb)

    def fn(A_x, A_c_kv, A_w_q, A_w_uk, A_w_uv, A_w_o, B_x, B_w_r, B_w_gate, B_w_up, B_w_down, gate_w):
        del B_x
        _, S, M = A_x.shape
        _, H, D = A_w_q.shape
        nb = S // D
        assert (D, nb, H) == (2 * T, 8, 16) and A_c_kv.shape == (1, S, nb * T)
        vmem = pltpu.VMEM
        outT = pl.pallas_call(
            kernel,
            name=name,
            in_specs=[pl.BlockSpec(memory_space=pl.ANY)] * 11,
            out_specs=pl.BlockSpec(memory_space=pl.ANY),
            out_shape=jax.ShapeDtypeStruct((M, S), BF),
            scratch_shapes=[
                vmem((H, M, D), BF),
                vmem((H, 4, S // 2, T), BF),
                vmem((H, 4, S, T), BF),
                *[vmem((9, S // 2, T), BF)] * 3,
                vmem((nb, 1, D), F32),
                vmem((nb, M, D), F32),
                pltpu.SemaphoreType.DMA((4,)),
                pltpu.SemaphoreType.DMA((len(_FIRST_PASS),)),
                pltpu.SemaphoreType.DMA((H // 2,)),
                pltpu.SemaphoreType.DMA((nb // 2,)),
            ],
            compiler_params=pltpu.CompilerParams(vmem_limit_bytes=124 * 2**20),
        )(A_x[0].T, A_c_kv[0], A_w_q, A_w_uk, A_w_uv, jnp.swapaxes(A_w_o, 1, 2), B_w_r, gate_w,
          B_w_gate, B_w_up, B_w_down.T)
        return outT.T[None]

    return fn


_impl = make()


@jax.jit
def pallas_gated_mix__compressed_kv_cla__moe_arch_mod__prompt_kernel(
    A_x, A_c_kv, A_w_q, A_w_uk, A_w_uv, A_w_o, B_x, B_w_r, B_w_gate, B_w_up, B_w_down, gate_w,
):
    return _impl(A_x, A_c_kv, A_w_q, A_w_uk, A_w_uv, A_w_o, B_x, B_w_r, B_w_gate, B_w_up, B_w_down, gate_w)
```

```python
import functools
import math

import jax
import jax.numpy as jnp
from jax import lax
import jax.experimental.pallas as pl
import jax.experimental.pallas.tpu as pltpu

BF = jnp.bfloat16
F32 = jnp.float32
U32 = jnp.uint32
T = 128
_cat = jnp.concatenate

_HEAD_PROGRAM = "S7 S6 P7 S4 P6 S5 O6-7 S3 P4+P5 S1 P3 O4 O5 S2 S0+P2 P0+P1 O2-3 O0 O1"
_FIRST_PASS = (((0, 1), ()), ((1, 1), (0, 1)), ((1, 3), (1, 2)), ((3, 6), (2, 3, 5)), ((6, 8), (5, 6, 8)))

_LHS = ((0, 1, 3), (2, 1, 3), (0,), (3,), (0, 1, 1), (2, -1, 0), (1, -1, 3))
_RHS = ((0, 1, 3), (0,), (1, -1, 3), (2, -1, 0), (3,), (0, 1, 1), (2, 1, 3))
_OUT = ({0: 1, 3: 1, 4: -1, 6: 1}, {2: 1, 4: 1}, {1: 1, 3: 1}, {0: 1, 1: -1, 2: 1, 5: 1})


def _operand(rule, quadrant):
    if len(rule) == 1:
        return quadrant(rule[0])
    a, b = quadrant(rule[0]), quadrant(rule[2])
    return a + b if rule[1] > 0 else a - b


def _operands(rules, quads):
    return tuple(_operand(rule, quads.__getitem__) for rule in rules)


def _combine(m, order):
    out = []
    for k, signs in enumerate(_OUT):
        ns = [n for n in order if n in signs]
        if len(ns) == 4:
            ns = ns[::-1] if k == 3 else [ns[2], ns[1], ns[0], ns[3]]
        acc, sign = m[ns[0]], signs[ns[0]]
        for n in ns[1:]:
            if sign > 0:
                acc = acc + m[n] if signs[n] > 0 else acc - m[n]
            else:
                acc, sign = m[n] - acc, 1
        out.append(acc)
    return out


def _dot(a, b):
    return jnp.dot(a, b, preferred_element_type=F32)


def _dot_nt(a, b):
    return lax.dot_general(a, b, (((1,), (1,)), ((), ())), preferred_element_type=F32)


def _sigmoid(z):
    return 1.0 / (1.0 + jnp.exp(-z))


def _inverse_row_sum(partial_sums):
    l = jnp.sum(partial_sums, axis=1, keepdims=True)
    r = pl.reciprocal(l, approx=True)
    return r * (2.0 - l * r)


def _head_of(words, odd):
    if isinstance(odd, int):
        return pltpu.bitcast(words & U32(0xFFFF0000) if odd else words << 16, F32)
    return pltpu.bitcast((words << ((1 - odd) * 16).astype(U32)) & U32(0xFFFF0000), F32)


def _after(x, pin):
    if pin is None:
        return x
    never, late = pin
    bits, late = pltpu.bitcast(x, U32), pltpu.bitcast(late, U32)
    out = _cat([_cat([jnp.where(never, late, bits[r:r + 8, u:u + T]) for u in range(0, bits.shape[1], T)], axis=1)
                for r in range(0, bits.shape[0], 8)], axis=0)
    return pltpu.bitcast(out, x.dtype)


def _spread(jobs, never, marks, lo, hi):
    for k, job in enumerate(jobs):
        job((never, marks[int(len(marks) * (lo + (hi - lo) * k / len(jobs)))]))


def make(prog=_HEAD_PROGRAM, qord=(0, 1, 2, 5, 3, 4, 6), sord=(1, 2, 0, 3, 5, 6, 4), pord=(2, 4, 0, 5, 1, 6, 3),
         oord=(0, 1, 2, 4, 3, 5, 6), late_sum=(0, 1, 6, 7), timed_exp=(4, 5), lead=32, vnow=2, qnow=4, delay=32, tail=12,
         room_s=(4, 4, 3, 1, 1, 1, 1, 1), room_p=(1, 1, 2, 4, 8, 7, 6, 3), room_o=(4, 5, 3, 2, 1, 0, 0),
         spl=(0, 0.75), head_only=False, name="kb"):
    def kernel(xT_hbm, c_hbm, wq_hbm, wuk_hbm, wuv_hbm, woT_hbm, wr_hbm, gw_hbm, wg_hbm, wu_hbm, wdT_hbm, outT_hbm,
               woT, q_all, kv_all, q9, k9, v9, gate, acc, sem, sem_x, sem_q):
        nb, M, D = acc.shape
        S, H, Dc, F = nb * D, q_all.shape[0], c_hbm.shape[1], wg_hbm.shape[1]
        P, Mh = H // 2, M // 2
        q_scale = D ** -0.5 * math.log2(math.e)
        vmem = pltpu.VMEM

        def start_of(i, size):
            return i * size if isinstance(i, int) else pl.multiple_of(i * size, size)

        def cp_kv(w_kv, late):
            return [pltpu.make_async_copy((wuk_hbm, wuv_hbm)[t // 2].bitcast(U32).at[:, j, pl.ds(t % 2 * T, T)],
                                          w_kv.at[t, j], sem.at[1 + late])
                    for t in range(4) for j in range(P) if (j > P // 2) == late]

        def cp_wo():
            return pltpu.make_async_copy(woT_hbm, woT, sem.at[3])

        def put_operands(kind, rows, a):
            if kind == "Q":
                ops = _operands(_LHS, a)
            else:
                ops = _operands(_RHS, a if kind == "V" else (a[0], a[2], a[1], a[3]))
            for n, t in enumerate(ops + (a[1], a[2])):
                {"Q": q9, "K": k9, "V": v9}[kind][n, rows, :] = t.astype(BF)

        def operand_jobs(kind, h, g):
            def job(r, pin):
                if kind == "Q":
                    words = [q_all.bitcast(U32)[h, k, pl.ds((g * T + r) // 2, 8), :] for k in range(4)]
                else:
                    words = [kv_all.bitcast(U32)[h, 2 * (kind == "V") + ch, pl.ds((g * D + rh * T + r) // 2, 8), :]
                             for rh in range(2) for ch in range(2)]
                put_operands(kind, pl.ds(g * T + r, 16), [pltpu.bitcast(_after(w, pin), BF).astype(F32) for w in words])

            return [functools.partial(job, r) for r in range(0, T, 16)]

        def queries(c, w_kv, u_sum, xT, wq, wr, gw, wg, wu, wdT, x7, wq7, vec_cols, score):
            def cp_x(i):
                group = [lo <= i < hi for (lo, hi), _ in _FIRST_PASS].index(True)
                return pltpu.make_async_copy(xT_hbm.at[:, pl.ds(i * D, D)], xT.at[i], sem_x.at[group])

            def cp_q(j):
                return pltpu.make_async_copy(wq_hbm.bitcast(U32).at[:, j, :], wq.at[j], sem_q.at[j])

            def cp_vectors():
                return [pltpu.make_async_copy(src, dst, sem_q.at[1]) for src, dst in ((wr_hbm, wr), (gw_hbm, gw))]

            def cp_rest():
                return [pltpu.make_async_copy(src, dst, sem.at[0])
                        for src, dst in ((c_hbm, c), (wg_hbm, wg), (wu_hbm, wu), (wdT_hbm, wdT))]

            def build_x7(i):
                xt = xT[i].astype(F32)
                pad = jnp.zeros((D - Mh, T), F32)
                quads = [_cat([t, pad], axis=0).T for t in (xt[:Mh, :T], xt[Mh:, :T], xt[:Mh, T:], xt[Mh:, T:])]
                for n, t in enumerate(_operands(_LHS, quads)):
                    x7[n, i * T:(i + 1) * T, :] = t.astype(BF)

            def wq_quadrant(h, r, pin, k):
                return _head_of(_after(wq[h >> 1, pl.ds(k // 2 * Mh + r, 16), pl.ds(k % 2 * T, T)], pin), h & 1)

            def wq7_jobs(h, slot):
                def job(r, pin):
                    for n, t in enumerate(_operands(_RHS, [wq_quadrant(h, r, pin, k) for k in range(4)])):
                        wq7[slot, n, r:r + 16, :] = t.astype(BF)

                return [functools.partial(job, r) for r in range(0, Mh, 16)]

            def u_sum_job(k, r, pin):
                blocks = [_after(c[pl.ds(j * D + r, 16), pl.ds(k * T, T)], pin).astype(F32) for j in range(nb)]
                u_sum[k, r:r + 16, :] = functools.reduce(jnp.add, blocks)

            def gate_jobs(i):
                sums = {}

                def job(t, r, pin):
                    cols = slice(t * T, (t + 1) * T)
                    xt = _after(xT[i, r:r + 32, cols], pin).astype(F32)
                    for u in range(2):
                        p = xt * vec_cols[u, r:r + 32, :]
                        p = (p[0:8] + p[8:16]) + (p[16:24] + p[24:32])
                        sums[u] = p if r == 0 else sums[u] + p
                    if r + 32 == M:
                        score[i, :, cols] = jnp.sum(sums[0], axis=0, keepdims=True)
                        gate[i, :, cols] = _sigmoid(jnp.sum(sums[1], axis=0, keepdims=True))

                return [functools.partial(job, t, r) for t in range(2) for r in range(0, M, 32)]

            def residual_jobs(i):
                keep = []

                def job(r, pin):
                    if not keep:
                        keep.append(1.0 - gate[i])
                    acc[i, r:r + 16, :] = keep[0] * _after(xT[i, r:r + 16, :], pin).astype(F32)

                return [functools.partial(job, r) for r in range(0, M, 16)]

            def route():
                def whole(op, t):
                    return op(op(t, axis=0, keepdims=True), axis=1, keepdims=True)

                r = _cat([score[i] for i in range(nb)], axis=0).astype(BF).astype(F32)
                tok = lax.broadcasted_iota(jnp.int32, (nb, D), 0) * D + lax.broadcasted_iota(jnp.int32, (nb, D), 1)
                bits = pltpu.bitcast(jnp.where(r == 0.0, 0.0, r), jnp.int32) >> 16
                rank = jnp.where(r != r, 0, jnp.where(bits < 0, bits ^ 0x7FFF, bits) + 0x8000)
                key = pltpu.bitcast(0x20000000 + rank * S + (S - 1 - tok), F32)
                lane = lax.broadcasted_iota(jnp.int32, (1, D), 1)
                picks = []
                for _ in range(2):
                    best = whole(jnp.max, key)
                    idx = S - 1 - (pltpu.bitcast(best, jnp.int32)[0, 0] & (S - 1))
                    weight = _sigmoid(whole(jnp.sum, jnp.where(key == best, r, 0.0)))
                    picks.append((idx >> (D.bit_length() - 1), lane == (idx & (D - 1)), weight))
                    key = jnp.where(key == best, 0.0, key)
                return picks

            def gather(picks):
                row = lax.broadcasted_iota(jnp.int32, (16, D), 0)
                return sum(_dot_nt(jnp.where((row == u) & hot, 1.0, 0.0).astype(BF), xT[b])
                           for u, (b, hot, _) in enumerate(picks)).astype(BF)

            def scatter_jobs(y, picks):
                def job(b, hot, col, keep, r, pin):
                    yr = _after(col[r:r + 32], pin)
                    acc[b, r:r + 32, :] += jnp.where(hot, keep * _cat([yr, yr], axis=1), 0.0)

                jobs = []
                for u, (b, hot, weight) in enumerate(picks):
                    col = jnp.broadcast_to(y[u:u + 1] * weight, (T, M)).T
                    keep = 1.0 - gate[b]
                    jobs += [functools.partial(job, b, hot, col, keep, r) for r in range(0, M, 32)]
                return jobs

            def q_proj(h, slots, lo, hi, before=None):
                m = [None] * 7
                for k, n in enumerate(qord):
                    if before is not None:
                        before(k)
                    m[n] = _dot(x7[n, lo * T:hi * T, :], _cat([wq7[slot, n] for slot in slots], axis=1))
                for e in range(len(slots)):
                    for k, t in enumerate(_combine([t[:, e * T:(e + 1) * T] for t in m], qord)):
                        q_all[h + e, k, lo * T:hi * T, :] = (t * q_scale).astype(BF)
                return [m[n][r:r + 8, :T] for n in qord for r in range(0, (hi - lo) * T, 16)]

            def never_set():
                t = xT[0, :16, :T].astype(F32)[:8]
                return t * t < 0.0

            def first_pair():
                wq7[:, :, Mh:, :] = jnp.zeros((3, 7, D - Mh, T), BF)
                for s, (arrived, projected) in enumerate(_FIRST_PASS):
                    for i in range(*arrived):
                        cp_x(i).wait()
                    if s == 1:
                        cp_q(0).wait()
                        for both in zip(wq7_jobs(0, 1), wq7_jobs(1, 2)):
                            for job in both:
                                job(None)
                    if s == len(_FIRST_PASS) - 1:
                        for cp in [cp_q(1)] + cp_vectors():
                            cp.wait()
                    for i in range(*arrived):
                        build_x7(i)
                    marks = [t for lo, hi in zip(projected, projected[1:]) for t in q_proj(0, (1, 2), lo, hi)]
                for u, ref in enumerate((wr, gw)):
                    vec_cols[u] = jnp.broadcast_to(ref[...].astype(F32).reshape(1, M), (T, M)).T
                _spread(wq7_jobs(2, 0), never_set(), marks, 0.35, 0.7)

            def middle_head(h, carry):
                @pl.when((h & 1) == 1)
                def _():
                    cp_q((h + 1) >> 1).wait()

                never = h >= H
                marks, rest = q_proj(h, (0,), 0, nb // 2), q_proj(h, (0,), nb // 2, nb)
                i = jnp.minimum(h - 2, nb - 1)
                _spread(gate_jobs(i) + residual_jobs(i), never, marks + rest, 0, 0.75)

                def next_weights(n, r, pin):
                    wq7[0, n, r:r + 16, :] = _operand(_RHS[n], functools.partial(wq_quadrant, h + 1, r, pin)).astype(BF)

                for k, n in enumerate(qord):
                    jobs = [functools.partial(next_weights, n, r) for r in range(0, Mh, 16)]
                    _spread(jobs, never, rest, k / 7 + 0.005, k / 7 + 0.1)
                return carry

            def last_pair():
                for cp in cp_rest():
                    cp.wait()
                for job in wq7_jobs(H - 1, 1):
                    job(None)
                picks, never = route(), never_set()
                xs, hidden, y = [], [], []

                def take(k):
                    if k == 1:
                        xs.append(gather(picks))

                def up(step, k):
                    for t in range((step + k) * 2 * (F // T) // 21, (step + k + 1) * 2 * (F // T) // 21):
                        hidden.append(_dot(xs[0], (wg, wu)[t % 2][:, t // 2 * T:(t // 2 + 1) * T]))

                def down(step, k):
                    for t in range((step + k) * (F // T) // 14, (step + k + 1) * (F // T) // 14):
                        g, u = hidden[2 * t], hidden[2 * t + 1]
                        y.append(_dot_nt((g * _sigmoid(g) * u).astype(BF), wdT[:, t * T:(t + 1) * T]))

                extras = ([None, take] + [functools.partial(up, 7 * s) for s in range(3)]
                          + [functools.partial(down, 7 * s) for s in range(2)])
                marks = [t for i, extra in enumerate(extras) for t in q_proj(H - 2, (0, 1), i, i + 1, extra)]
                y = functools.reduce(jnp.add, y)
                rest = q_proj(H - 2, (0, 1), nb - 1, nb)
                jobs = [functools.partial(u_sum_job, k, r) for k in range(nb) for r in range(0, D, 16)]
                jobs += [job for g in range(qnow, nb) for job in operand_jobs("Q", 0, g)]
                _spread(jobs, never, marks, 0, 0.97)
                _spread(scatter_jobs(y, picks), never, rest, 0.3, 0.9)

            copies = [cp_x(0), cp_q(0)] + [cp_x(i) for i in range(1, nb)] + [cp_q(1)] + cp_vectors()
            copies += [cp_q(j) for j in range(2, P)]
            for cp in copies + cp_rest() + cp_kv(w_kv, False) + cp_kv(w_kv, True) + [cp_wo()]:
                cp.start()
            first_pair()
            lax.fori_loop(2, H - 2, middle_head, 0)
            last_pair()

        def keys_values(c, w_kv, u_sum, b_sum, common, a32, v32, lhs, a_fix, v_fix, u_fix, b_fix):
            groups = [(j, k) for j in range(0, nb, 2) for k in range(0, nb, 2)]

            def u_block(j, k):
                return c[j * D:(j + 1) * D, k * T:(k + 1) * T]

            def stage_jobs(i, tiles):
                def a_job(j, r, pin):
                    a32[j, r:r + 32, :] = _after(c[pl.ds(start_of(i, D) + r, 32), j * T:(j + 1) * T], pin).astype(F32)

                def v_job(k, t, r, pin):
                    words = w_kv[t, P // 2 + (i >> 1), pl.ds(k * T + r, 32), :]
                    v32[k, t, r:r + 32, :] = _head_of(_after(words, pin), i & 1)

                return ([functools.partial(a_job, j, r) for j in range(nb) for r in range(0, D, 32)]
                        + [functools.partial(v_job, k, t, r)
                           for k in range(nb) for t in tiles for r in range(0, T, 32)])

            def lhs_jobs(j, k):
                def job(dj, r, pin):
                    a = a32[j + dj, r:r + 32, :]
                    for dk in range(2):
                        u = _after(c[pl.ds((j + dj) * D + r, 32), pl.ds((k + dk) * T, T)], pin).astype(F32)
                        lhs[j + dj, k + dk, r:r + 32, :] = (a + u).astype(BF)

                return [functools.partial(job, dj, r) for r in range(0, D, 32) for dj in range(2)]

            def common_terms(t, carry):
                first, second, sums, marks = {}, {}, {}, []
                for j, k in groups:
                    m = [[None, None], [None, None]]
                    for dj in range(2):
                        words = w_kv[t, k // 2, pl.ds((j + dj) * T, T), :]
                        b = _head_of(words, 0), _head_of(words, 1)
                        sums[j + dj] = sums[j + dj] + (b[0] + b[1]) if k else b[0] + b[1]
                        for dk in range(2):
                            m[dj][dk] = _dot(u_block(j + dj, k + dk), b[dk].astype(BF))
                    for e in range(2):
                        over_j, over_k = m[0][e] + m[1][e], m[e][0] + m[e][1]
                        first[k + e] = first[k + e] - over_j if j else -over_j
                        second[j + e] = second[j + e] - over_k if k else -over_k
                    marks += [m[0][0][r:r + 8] for r in range(0, D, 16)]
                for n in range(nb):
                    common[t, n], common[t, nb + n], b_sum[t, n] = first[n], second[n], sums[n]
                _spread(stage_jobs(0, [t]) + lhs_jobs(0, 0), t >= 4, marks, 0, 0.7)
                return carry

            def plane(i, carry):
                never = i >= nb
                first = {(k, t): common[t, k] for k in range(nb) for t in range(4)}
                second = {(j, t): common[t, nb + j] for j in range(nb) for t in range(4)}
                marks = []
                for j, k in groups:
                    if marks:
                        _spread(lhs_jobs(j, k), never, marks[-64:], *spl)
                    for t in range(4):
                        m = [[None, None], [None, None]]
                        for dj in range(2):
                            words = w_kv[t, k // 2, pl.ds((j + dj) * T, T), :]
                            b = _head_of(words, 0), _head_of(words, 1)
                            for dk in range(2):
                                m[dj][dk] = _dot(lhs[j + dj, k + dk], (b[dk] + v32[k + dk, t]).astype(BF))
                        for e in range(2):
                            first[k + e, t] = first[k + e, t] + (m[0][e] + m[1][e])
                            second[j + e, t] = second[j + e, t] + (m[e][0] + m[e][1])
                        marks += [m[0][0][r:r + 8] for r in range(0, D, 16)]

                def a_job(r, pin):
                    a = [_after(a32[j, r:r + 16, :], pin) for j in range(nb)]
                    total = functools.reduce(jnp.add, a)
                    for n in range(nb):
                        a_fix[n, r:r + 16, :] = a[n].astype(BF)
                        u_fix[n, r:r + 16, :] = (total + u_sum[n, r:r + 16, :]).astype(BF)

                def v_job(t, r, pin):
                    v = [_after(v32[k, t, r:r + 16, :], pin) for k in range(nb)]
                    total = functools.reduce(jnp.add, v)
                    for n in range(nb):
                        v_fix[n, t, r:r + 16, :] = v[n].astype(BF)
                        b_fix[n, t, r:r + 16, :] = (total + b_sum[t, n, r:r + 16, :]).astype(BF)

                jobs = [functools.partial(a_job, r) for r in range(0, D, 16)]
                jobs += [functools.partial(v_job, t, r) for t in range(4) for r in range(0, T, 16)]
                _spread(jobs, never, marks, 0.1, 0.7)
                marks = []
                for n in range(nb):
                    x = _dot(u_fix[n], _cat([v_fix[n, t] for t in range(4)], axis=1))
                    done = [first[n, t] - x[:, t * T:(t + 1) * T] for t in range(4)]
                    for t in range(4):
                        kv_all[n, t, pl.ds(start_of(i, D), D), :] = done[t].astype(BF)
                    if n == 0:
                        for kind, (lo, hi) in (("K", done[:2]), ("V", done[2:])):
                            put_operands(kind, pl.ds(start_of(i, T), T), (lo[:T], hi[:T], lo[T:], hi[T:]))
                    y = _dot(a_fix[n], _cat([b_fix[n, t] for t in range(4)], axis=1))
                    for t in range(4):
                        kv_all[nb + i, t, n * D:(n + 1) * D, :] = (second[n, t] - y[:, t * T:(t + 1) * T]).astype(BF)
                    marks += [z[r:r + 8, :T] for z in (x, y) for r in range(0, D, 16)]
                _spread(stage_jobs(jnp.minimum(i + 1, nb - 1), range(4)) + lhs_jobs(0, 0), never, marks, 0, 0.95)
                return carry

            for cp in cp_kv(w_kv, False):
                cp.wait()
            lax.fori_loop(0, 4, common_terms, 0)
            for cp in cp_kv(w_kv, True) + [cp_wo()]:
                cp.wait()
            lax.fori_loop(0, nb, plane, 0)

        def attention(ctx7, wo7, outT, *inv_sums):
            def cp_out(i):
                return pltpu.make_async_copy(outT.at[i], outT_hbm.at[:, pl.ds(i * D, D)], sem.at[0])

            def head(h, carry):
                never = h >= H
                clock, room, scores_of, last_use = [], [], {}, {}

                def tick(x, tiles, free):
                    n = max(1, x.shape[0] * tiles // 64)
                    clock.extend(x[(k * (x.shape[0] // 8) // n) * 8:][:8, -T:] for k in range(n))
                    room.extend([free] * n)
                    return x

                def wo_job(r, pin):
                    quads = [_after(woT[h, pl.ds(rh * Mh + r, 16), pl.ds(ch * T, T)], pin).astype(F32)
                             for rh in range(2) for ch in range(2)]
                    for n, t in enumerate(_operands(_LHS, quads)):
                        wo7[n, r:r + 16, :] = t.astype(BF)

                def scores(i):
                    r = slice(i * T, (i + 1) * T)
                    q_top, q_bot = _cat([q9[2, r, :], q9[7, r, :]], axis=1), _cat([q9[8, r, :], q9[3, r, :]], axis=1)
                    past = [[], [], [], []]
                    if i:
                        m = [None] * 7
                        for n, free in zip(sord, room_s):
                            m[n] = tick(_dot_nt(q9[n, r, :], k9[n, :i * T, :]), i, free)
                            yield i
                        past = [[s[:, t * T:(t + 1) * T] for t in range(i)] for s in _combine(m, sord)]
                    d1 = _dot_nt(_cat([q_top, q_bot], axis=0), _cat([k9[1, r, :], k9[7, r, :]], axis=1))
                    d2 = _dot_nt(q_bot, _cat([k9[8, r, :], k9[4, r, :]], axis=1))
                    tick(d1, 3, room_s[7])
                    yield 6
                    causal = lax.broadcasted_iota(jnp.int32, (T, T), 1) <= lax.broadcasted_iota(jnp.int32, (T, T), 0)
                    diagonal = [jnp.where(causal, d1[:T], -1e9)], [d1[T:], jnp.where(causal, d2, -1e9)]
                    rows = []
                    for u in range(2):
                        first, second = sorted((2 * u, 2 * u + 1), key=lambda k: max(sord.index(n) for n in _OUT[k]))
                        row_max = functools.reduce(jnp.maximum, past[first] + past[second] + diagonal[u])
                        rows.append((past[2 * u] + past[2 * u + 1] + diagonal[u],
                                     jnp.max(row_max, axis=1, keepdims=True)))
                    scores_of[i] = rows, len(clock)
                    last_use.update({("K", g): len(clock) for g in range(i + 1)})
                    last_use["Q", i] = len(clock)

                def attend(i):
                    rows, since = scores_of.pop(i)
                    r = slice(i * T, (i + 1) * T)
                    exps, sums = {}, {}

                    def timed(k):
                        if k not in exps:
                            exps[k] = []
                            where = [(0, -1), (1, -2), (1, -1)] if k == 4 else [(k // 2, k % 2 * i + t) for t in range(i)]
                            for t, (u, idx) in enumerate(where):
                                tiles, row_max = rows[u]
                                parts = []
                                for r0 in range(0, T, 16):
                                    at = min(len(clock) - 1, max(since - 1, len(clock) - lead + t // 4 * 8 + r0 // 16))
                                    parts.append(jnp.exp2(tiles[idx][r0:r0 + 16] - _after(
                                        jnp.broadcast_to(row_max[r0:r0 + 16], (16, T)), (never, clock[at]))))
                                exps[k].append(_cat(parts, axis=0))
                                sums[u] = sums[u] + exps[k][-1] if u in sums else exps[k][-1]
                        return exps[k]

                    if i in timed_exp:
                        def p7(n, t):
                            return _operand(_LHS[n], lambda k: timed(k)[t])
                    else:
                        top, bot = ([jnp.exp2(t - row_max) for t in tiles] for tiles, row_max in rows)
                        ops = [_operands(_LHS, (top[t], top[i + t], bot[t], bot[i + t])) for t in range(i)]

                        def p7(n, t):
                            return ops[t][n]

                    m = [None] * 7
                    for n, free in zip(pord, room_p) if i else ():
                        p = _cat([p7(n, t) for t in range(i)], axis=1).astype(BF)
                        m[n] = tick(_dot(p, v9[n, :i * T, :]), i, free)
                        yield i
                    if i in timed_exp:
                        diagonal = timed(4)
                        for u in range(2):
                            inv_sums[i][u * T:(u + 1) * T, :] = jnp.broadcast_to(_inverse_row_sum(sums[u]), (T, T))
                    else:
                        diagonal = [top[-1], bot[-2], bot[-1]]
                    d1 = _dot(_cat(diagonal[:2], axis=0).astype(BF), _cat([v9[1, r, :], v9[7, r, :]], axis=1))
                    d2 = _dot(diagonal[2].astype(BF), _cat([v9[8, r, :], v9[4, r, :]], axis=1))
                    tick(d1, 3, room_p[7])
                    yield 6
                    last_use.update({("V", g): len(clock) for g in range(i + 1)})
                    o = [d1[:T, :T], d1[:T, T:], d1[T:, :T] + d2[:, :T], d1[T:, T:] + d2[:, T:]]
                    if i:
                        o = [a + b for a, b in zip(o, _combine(m, pord))]
                    if i in timed_exp:
                        zero = pl.multiple_of((h >> H.bit_length() - 1) * T, T)
                        inv = inv_sums[i][pl.ds(zero, T), :], inv_sums[i][pl.ds(zero + T, T), :]
                    else:
                        inv = []
                        for e, late in ((top, o[0]), (bot, o[3])):
                            partial_sums = functools.reduce(jnp.add, e)
                            if i in late_sum:
                                partial_sums = jnp.where(never, late, partial_sums)
                            inv.append(_inverse_row_sum(partial_sums))
                    ctx = (o[0] * inv[0], o[2] * inv[1], o[1] * inv[0], o[3] * inv[1])
                    for n, t in enumerate(_operands(_RHS, ctx)):
                        ctx7[n, r, :] = t.astype(BF)

                def out_proj(lo, hi):
                    m = [None] * 7
                    for n, free in zip(oord, room_o):
                        m[n] = tick(_dot_nt(wo7[n], ctx7[n, lo * T:hi * T, :]), hi - lo, free)
                        yield 1.75 * (hi - lo)
                    for k, a in enumerate(_combine(m, oord)):
                        rows, cols = slice(k // 2 * Mh, (k // 2 + 1) * Mh), slice(k % 2 * T, (k % 2 + 1) * T)
                        for i in range(lo, hi):
                            total = acc[i, rows, cols] + gate[i, :, cols] * a[:, (i - lo) * T:(i - lo + 1) * T]
                            acc[i, rows, cols] = total
                            outT[i, rows, cols] = total.astype(BF)

                    @pl.when(h == H - 1)
                    def _():
                        for i in range(lo, hi):
                            cp_out(i).start()

                def begin(step):
                    kind, (lo, _, hi) = step[0], step[1:].partition("-")
                    lo, hi = int(lo), int(hi or lo) + 1
                    if kind == "O":
                        return [out_proj(lo, hi), 12.25 * (hi - lo), 0]
                    return [(scores if kind == "S" else attend)(lo), 7 * lo + 6, 0]

                def fit(jobs, lo, hi):
                    for cost in range(256, 0, -1):
                        at, saved = [], 0
                        for t in range(lo, hi):
                            if len(at) < len(jobs) and min(jobs[len(at)][0], hi - 1) <= t:
                                saved += room[t]
                                if saved >= cost:
                                    saved = 0
                                    at.append(t)
                        if len(at) == len(jobs):
                            break
                    for k, (_, job) in enumerate(jobs):
                        job((never, clock[at[k] if k < len(at) else hi - 1]))

                def next_head_jobs(until):
                    def finished(kind, g):
                        users = range(g, g + 1 if kind == "Q" else nb)
                        return all(("P" if kind == "V" else "S") + str(t) not in ahead for t in users)

                    ready = [(free, kind, g) for (kind, g), free in last_use.items()
                             if free <= until and (kind, g) not in rebuilt and finished(kind, g)
                             and g >= {"Q": qnow, "K": 0, "V": vnow}[kind]]
                    rebuilt.update((kind, g) for _, kind, g in ready)
                    return [(free + delay, job) for free, kind, g in sorted(ready)
                            for job in operand_jobs(kind, jnp.minimum(h + 1, H - 1), g)]

                first_p, first_o, rebuilt, ahead = None, None, set(), prog.replace("+", " ").split()
                for group in prog.split():
                    if first_p is None and "P" in group:
                        first_p = len(clock)
                        fit([(0, job) for g in range(vnow) for job in operand_jobs("V", h, g)], 0, first_p - 2 * tail)
                    if first_o is None and "O" in group:
                        first_o = len(clock) - 2 * tail
                        jobs = [(0, functools.partial(wo_job, r)) for r in range(0, Mh, 16)]
                        jobs += [(0, job) for g in reversed(range(qnow)) for job in operand_jobs("Q", h, g)]
                        fit(jobs + next_head_jobs(first_o - 64), first_p, first_o)
                    assert first_o is not None or not any(f"S{g}" in group for g in range(qnow))
                    running = [begin(step) for step in group.split("+")]
                    while running:
                        step = min(running, key=lambda s: s[2] / s[1])
                        try:
                            step[2] += next(step[0])
                        except StopIteration:
                            running.remove(step)
                    ahead = [step for step in ahead if step not in group.split("+")]
                fit(next_head_jobs(len(clock)), first_o, len(clock) - tail)
                return carry

            lax.fori_loop(0, H, head, 0)
            for i in range(nb):
                cp_out(i).wait()

        def projections(*shared):
            pl.run_scoped(
                functools.partial(queries, *shared),
                xT=vmem((nb, M, D), BF), wq=vmem((P, M, D), U32), wr=vmem((M,), BF), gw=vmem((M,), BF),
                wg=vmem((M, F), BF), wu=vmem((M, F), BF), wdT=vmem((M, F), BF),
                x7=vmem((7, S // 2, D), BF), wq7=vmem((3, 7, D, T), BF),
                vec_cols=vmem((2, M, T), F32), score=vmem((nb, 1, D), F32))
            pl.run_scoped(
                functools.partial(keys_values, *shared),
                b_sum=vmem((4, nb, T, T), F32), common=vmem((4, 2 * nb, D, T), F32),
                a32=vmem((nb, D, T), F32), v32=vmem((nb, 4, T, T), F32), lhs=vmem((nb, nb, D, T), BF),
                a_fix=vmem((nb, D, T), BF), v_fix=vmem((nb, 4, T, T), BF),
                u_fix=vmem((nb, D, T), BF), b_fix=vmem((nb, 4, T, T), BF))

        if not head_only:
            pl.run_scoped(projections, vmem((S, Dc), BF), vmem((4, P, Dc, T), U32), vmem((nb, D, T), F32))
        pl.run_scoped(attention, vmem((7, S // 2, T), BF), vmem((7, Mh, T), BF), vmem((nb, M, D), BF),
                      *[vmem((D, T), F32)] * nb)

    def fn(A_x, A_c_kv, A_w_q, A_w_uk, A_w_uv, A_w_o, B_x, B_w_r, B_w_gate, B_w_up, B_w_down, gate_w):
        del B_x
        _, S, M = A_x.shape
        _, H, D = A_w_q.shape
        nb = S // D
        assert (D, nb, H) == (2 * T, 8, 16) and A_c_kv.shape == (1, S, nb * T)
        vmem = pltpu.VMEM
        outT = pl.pallas_call(
            kernel,
            name=name,
            in_specs=[pl.BlockSpec(memory_space=pl.ANY)] * 11,
            out_specs=pl.BlockSpec(memory_space=pl.ANY),
            out_shape=jax.ShapeDtypeStruct((M, S), BF),
            scratch_shapes=[
                vmem((H, M, D), BF),
                vmem((H, 4, S // 2, T), BF),
                vmem((H, 4, S, T), BF),
                *[vmem((9, S // 2, T), BF)] * 3,
                vmem((nb, 1, D), F32),
                vmem((nb, M, D), F32),
                pltpu.SemaphoreType.DMA((4,)),
                pltpu.SemaphoreType.DMA((len(_FIRST_PASS),)),
                pltpu.SemaphoreType.DMA((H // 2,)),
            ],
            compiler_params=pltpu.CompilerParams(vmem_limit_bytes=124 * 2**20),
        )(A_x[0].T, A_c_kv[0], A_w_q, A_w_uk, A_w_uv, jnp.swapaxes(A_w_o, 1, 2), B_w_r, gate_w,
          B_w_gate, B_w_up, B_w_down.T)
        return outT.T[None]

    return fn


_impl = make()


@jax.jit
def pallas_gated_mix__compressed_kv_cla__moe_arch_mod__prompt_kernel(
    A_x, A_c_kv, A_w_q, A_w_uk, A_w_uv, A_w_o, B_x, B_w_r, B_w_gate, B_w_up, B_w_down, gate_w,
):
    return _impl(A_x, A_c_kv, A_w_q, A_w_uk, A_w_uv, A_w_o, B_x, B_w_r, B_w_gate, B_w_up, B_w_down, gate_w)
```

```python
import functools
import math

import jax
import jax.numpy as jnp
from jax import lax
import jax.experimental.pallas as pl
import jax.experimental.pallas.tpu as pltpu

BF = jnp.bfloat16
F32 = jnp.float32
U32 = jnp.uint32
T = 128
_cat = jnp.concatenate

_HEAD_PROGRAM = "S7 S6 P7 S4 P6 S5 O6-7 S3 P4+P5 S1 S2 P3 O4 O5 S0+P2 P0+P1 O2-3 O0 O1"
_Q_ORDER, _S_ORDER = (0, 1, 2, 5, 3, 4, 6), (1, 2, 0, 3, 5, 6, 4)
_P_ORDER, _O_ORDER = (2, 4, 0, 5, 1, 6, 3), (0, 1, 2, 4, 3, 6, 5)
_S_ROOM, _P_ROOM, _O_ROOM = (4, 4, 3, 1, 1, 1, 1, 1), (1, 1, 2, 4, 8, 7, 6, 3), (4, 5, 3, 2, 1, 0, 0)
_LATE_SUM, _TIMED_EXP, _LEAD = (0, 3, 6, 7), (4, 5), 32
_Q_NOW, _V_NOW, _DELAY, _MARGIN = 4, 2, 32, 12
_FIRST_PASS = (((0, 1), ()), ((1, 1), (0, 1)), ((1, 3), (1, 2)), ((3, 6), (2, 3, 5)), ((6, 8), (5, 6, 8)))

_LHS = ((0, 1, 3), (2, 1, 3), (0,), (3,), (0, 1, 1), (2, -1, 0), (1, -1, 3))
_RHS = ((0, 1, 3), (0,), (1, -1, 3), (2, -1, 0), (3,), (0, 1, 1), (2, 1, 3))
_OUT = ({0: 1, 3: 1, 4: -1, 6: 1}, {2: 1, 4: 1}, {1: 1, 3: 1}, {0: 1, 1: -1, 2: 1, 5: 1})


def _operand(rule, quadrant):
    if len(rule) == 1:
        return quadrant(rule[0])
    a, b = quadrant(rule[0]), quadrant(rule[2])
    return a + b if rule[1] > 0 else a - b


def _operands(rules, quads):
    return tuple(_operand(rule, quads.__getitem__) for rule in rules)


def _combine(m, order):
    out = []
    for k, signs in enumerate(_OUT):
        ns = [n for n in order if n in signs]
        if len(ns) == 4:
            ns = ns[::-1] if k == 3 else [ns[2], ns[1], ns[0], ns[3]]
        acc, sign = m[ns[0]], signs[ns[0]]
        for n in ns[1:]:
            if sign > 0:
                acc = acc + m[n] if signs[n] > 0 else acc - m[n]
            else:
                acc, sign = m[n] - acc, 1
        out.append(acc)
    return out


def _dot(a, b):
    return jnp.dot(a, b, preferred_element_type=F32)


def _dot_nt(a, b):
    return lax.dot_general(a, b, (((1,), (1,)), ((), ())), preferred_element_type=F32)


def _sigmoid(z):
    return 1.0 / (1.0 + jnp.exp(-z))


def _inverse_row_sum(partial_sums):
    l = jnp.sum(partial_sums, axis=1, keepdims=True)
    r = pl.reciprocal(l, approx=True)
    return r * (2.0 - l * r)


def _head_of(words, odd):
    if isinstance(odd, int):
        return pltpu.bitcast(words & U32(0xFFFF0000) if odd else words << 16, F32)
    return pltpu.bitcast((words << ((1 - odd) * 16).astype(U32)) & U32(0xFFFF0000), F32)


def _after(x, pin):
    if pin is None:
        return x
    never, late = pin
    bits, late = pltpu.bitcast(x, U32), pltpu.bitcast(late, U32)
    out = _cat([_cat([jnp.where(never, late, bits[r:r + 8, u:u + T]) for u in range(0, bits.shape[1], T)], axis=1)
                for r in range(0, bits.shape[0], 8)], axis=0)
    return pltpu.bitcast(out, x.dtype)


def _spread(jobs, never, marks, lo, hi):
    for k, job in enumerate(jobs):
        job((never, marks[int(len(marks) * (lo + (hi - lo) * k / len(jobs)))]))


def _kernel(xT_hbm, c_hbm, wq_hbm, wuk_hbm, wuv_hbm, woT_hbm, wr_hbm, gw_hbm, wg_hbm, wu_hbm, wdT_hbm, outT_hbm,
            woT, q_all, kv_all, q9, k9, v9, gate, acc, sem, sem_x, sem_q):
    nb, M, D = acc.shape
    S, H, Dc, F = nb * D, q_all.shape[0], c_hbm.shape[1], wg_hbm.shape[1]
    P, Mh = H // 2, M // 2
    q_scale = D ** -0.5 * math.log2(math.e)
    vmem = pltpu.VMEM

    def start_of(i, size):
        return i * size if isinstance(i, int) else pl.multiple_of(i * size, size)

    def cp_kv(w_kv, late):
        return [pltpu.make_async_copy((wuk_hbm, wuv_hbm)[t // 2].bitcast(U32).at[:, j, pl.ds(t % 2 * T, T)],
                                      w_kv.at[t, j], sem.at[1 + late])
                for t in range(4) for j in range(P) if (j > P // 2) == late]

    def cp_wo():
        return pltpu.make_async_copy(woT_hbm, woT, sem.at[3])

    def put_operands(kind, rows, a):
        if kind == "Q":
            ops = _operands(_LHS, a)
        else:
            ops = _operands(_RHS, a if kind == "V" else (a[0], a[2], a[1], a[3]))
        for n, t in enumerate(ops + (a[1], a[2])):
            {"Q": q9, "K": k9, "V": v9}[kind][n, rows, :] = t.astype(BF)

    def operand_jobs(kind, h, g):
        def job(r, pin):
            if kind == "Q":
                words = [q_all.bitcast(U32)[h, k, pl.ds((g * T + r) // 2, 8), :] for k in range(4)]
            else:
                words = [kv_all.bitcast(U32)[h, 2 * (kind == "V") + ch, pl.ds((g * D + rh * T + r) // 2, 8), :]
                         for rh in range(2) for ch in range(2)]
            put_operands(kind, pl.ds(g * T + r, 16), [pltpu.bitcast(_after(w, pin), BF).astype(F32) for w in words])

        return [functools.partial(job, r) for r in range(0, T, 16)]

    def queries(c, w_kv, u_sum, xT, wq, wr, gw, wg, wu, wdT, x7, wq7, vec_cols, score):
        def cp_x(i):
            group = [lo <= i < hi for (lo, hi), _ in _FIRST_PASS].index(True)
            return pltpu.make_async_copy(xT_hbm.at[:, pl.ds(i * D, D)], xT.at[i], sem_x.at[group])

        def cp_q(j):
            return pltpu.make_async_copy(wq_hbm.bitcast(U32).at[:, j, :], wq.at[j], sem_q.at[j])

        def cp_vectors():
            return [pltpu.make_async_copy(src, dst, sem_q.at[1]) for src, dst in ((wr_hbm, wr), (gw_hbm, gw))]

        def cp_rest():
            return [pltpu.make_async_copy(src, dst, sem.at[0])
                    for src, dst in ((c_hbm, c), (wg_hbm, wg), (wu_hbm, wu), (wdT_hbm, wdT))]

        def build_x7(i):
            xt = xT[i].astype(F32)
            pad = jnp.zeros((D - Mh, T), F32)
            quads = [_cat([t, pad], axis=0).T for t in (xt[:Mh, :T], xt[Mh:, :T], xt[:Mh, T:], xt[Mh:, T:])]
            for n, t in enumerate(_operands(_LHS, quads)):
                x7[n, i * T:(i + 1) * T, :] = t.astype(BF)

        def wq_quadrant(h, r, pin, k):
            return _head_of(_after(wq[h >> 1, pl.ds(k // 2 * Mh + r, 16), pl.ds(k % 2 * T, T)], pin), h & 1)

        def wq7_jobs(h, slot):
            def job(r, pin):
                for n, t in enumerate(_operands(_RHS, [wq_quadrant(h, r, pin, k) for k in range(4)])):
                    wq7[slot, n, r:r + 16, :] = t.astype(BF)

            return [functools.partial(job, r) for r in range(0, Mh, 16)]

        def u_sum_job(k, r, pin):
            blocks = [_after(c[pl.ds(j * D + r, 16), pl.ds(k * T, T)], pin).astype(F32) for j in range(nb)]
            u_sum[k, r:r + 16, :] = functools.reduce(jnp.add, blocks)

        def gate_jobs(i):
            sums = {}

            def job(t, r, pin):
                cols = slice(t * T, (t + 1) * T)
                xt = _after(xT[i, r:r + 32, cols], pin).astype(F32)
                for u in range(2):
                    p = xt * vec_cols[u, r:r + 32, :]
                    p = (p[0:8] + p[8:16]) + (p[16:24] + p[24:32])
                    sums[u] = p if r == 0 else sums[u] + p
                if r + 32 == M:
                    score[i, :, cols] = jnp.sum(sums[0], axis=0, keepdims=True)
                    gate[i, :, cols] = _sigmoid(jnp.sum(sums[1], axis=0, keepdims=True))

            return [functools.partial(job, t, r) for t in range(2) for r in range(0, M, 32)]

        def residual_jobs(i):
            keep = []

            def job(r, pin):
                if not keep:
                    keep.append(1.0 - gate[i])
                acc[i, r:r + 16, :] = keep[0] * _after(xT[i, r:r + 16, :], pin).astype(F32)

            return [functools.partial(job, r) for r in range(0, M, 16)]

        def route():
            def whole(op, t):
                return op(op(t, axis=0, keepdims=True), axis=1, keepdims=True)

            r = _cat([score[i] for i in range(nb)], axis=0).astype(BF).astype(F32)
            tok = lax.broadcasted_iota(jnp.int32, (nb, D), 0) * D + lax.broadcasted_iota(jnp.int32, (nb, D), 1)
            bits = pltpu.bitcast(jnp.where(r == 0.0, 0.0, r), jnp.int32) >> 16
            rank = jnp.where(r != r, 0, jnp.where(bits < 0, bits ^ 0x7FFF, bits) + 0x8000)
            key = pltpu.bitcast(0x20000000 + rank * S + (S - 1 - tok), F32)
            lane = lax.broadcasted_iota(jnp.int32, (1, D), 1)
            picks = []
            for _ in range(2):
                best = whole(jnp.max, key)
                idx = S - 1 - (pltpu.bitcast(best, jnp.int32)[0, 0] & (S - 1))
                weight = _sigmoid(whole(jnp.sum, jnp.where(key == best, r, 0.0)))
                picks.append((idx >> (D.bit_length() - 1), lane == (idx & (D - 1)), weight))
                key = jnp.where(key == best, 0.0, key)
            return picks

        def gather(picks):
            row = lax.broadcasted_iota(jnp.int32, (16, D), 0)
            return sum(_dot_nt(jnp.where((row == u) & hot, 1.0, 0.0).astype(BF), xT[b])
                       for u, (b, hot, _) in enumerate(picks)).astype(BF)

        def scatter_jobs(y, picks):
            def job(b, hot, col, keep, r, pin):
                yr = _after(col[r:r + 32], pin)
                acc[b, r:r + 32, :] += jnp.where(hot, keep * _cat([yr, yr], axis=1), 0.0)

            jobs = []
            for u, (b, hot, weight) in enumerate(picks):
                col = jnp.broadcast_to(y[u:u + 1] * weight, (T, M)).T
                keep = 1.0 - gate[b]
                jobs += [functools.partial(job, b, hot, col, keep, r) for r in range(0, M, 32)]
            return jobs

        def q_proj(h, slots, lo, hi, before=None):
            m = [None] * 7
            for k, n in enumerate(_Q_ORDER):
                if before is not None:
                    before(k)
                m[n] = _dot(x7[n, lo * T:hi * T, :], _cat([wq7[slot, n] for slot in slots], axis=1))
            for e in range(len(slots)):
                for k, t in enumerate(_combine([t[:, e * T:(e + 1) * T] for t in m], _Q_ORDER)):
                    q_all[h + e, k, lo * T:hi * T, :] = (t * q_scale).astype(BF)
            return [m[n][r:r + 8, :T] for n in _Q_ORDER for r in range(0, (hi - lo) * T, 16)]

        def never_set():
            t = xT[0, :16, :T].astype(F32)[:8]
            return t * t < 0.0

        def first_pair():
            wq7[:, :, Mh:, :] = jnp.zeros((3, 7, D - Mh, T), BF)
            for s, (arrived, projected) in enumerate(_FIRST_PASS):
                for i in range(*arrived):
                    cp_x(i).wait()
                if s == 1:
                    cp_q(0).wait()
                    for both in zip(wq7_jobs(0, 1), wq7_jobs(1, 2)):
                        for job in both:
                            job(None)
                if s == len(_FIRST_PASS) - 1:
                    for cp in [cp_q(1)] + cp_vectors():
                        cp.wait()
                for i in range(*arrived):
                    build_x7(i)
                marks = [t for lo, hi in zip(projected, projected[1:]) for t in q_proj(0, (1, 2), lo, hi)]
            for u, ref in enumerate((wr, gw)):
                vec_cols[u] = jnp.broadcast_to(ref[...].astype(F32).reshape(1, M), (T, M)).T
            _spread(wq7_jobs(2, 0), never_set(), marks, 0.35, 0.7)

        def middle_head(h, carry):
            @pl.when((h & 1) == 1)
            def _():
                cp_q((h + 1) >> 1).wait()

            never = h >= H
            marks, rest = q_proj(h, (0,), 0, nb // 2), q_proj(h, (0,), nb // 2, nb)
            i = jnp.minimum(h - 2, nb - 1)
            _spread(gate_jobs(i) + residual_jobs(i), never, marks + rest, 0, 0.75)

            def next_weights(n, r, pin):
                wq7[0, n, r:r + 16, :] = _operand(_RHS[n], functools.partial(wq_quadrant, h + 1, r, pin)).astype(BF)

            for k, n in enumerate(_Q_ORDER):
                jobs = [functools.partial(next_weights, n, r) for r in range(0, Mh, 16)]
                _spread(jobs, never, rest, k / 7 + 0.005, k / 7 + 0.1)
            return carry

        def last_pair():
            for cp in cp_rest():
                cp.wait()
            for job in wq7_jobs(H - 1, 1):
                job(None)
            picks, never = route(), never_set()
            xs, hidden, y = [], [], []

            def take(k):
                if k == 1:
                    xs.append(gather(picks))

            def up(step, k):
                for t in range((step + k) * 2 * (F // T) // 21, (step + k + 1) * 2 * (F // T) // 21):
                    hidden.append(_dot(xs[0], (wg, wu)[t % 2][:, t // 2 * T:(t // 2 + 1) * T]))

            def down(step, k):
                for t in range((step + k) * (F // T) // 14, (step + k + 1) * (F // T) // 14):
                    g, u = hidden[2 * t], hidden[2 * t + 1]
                    y.append(_dot_nt((g * _sigmoid(g) * u).astype(BF), wdT[:, t * T:(t + 1) * T]))

            extras = ([None, take] + [functools.partial(up, 7 * s) for s in range(3)]
                      + [functools.partial(down, 7 * s) for s in range(2)])
            marks = [t for i, extra in enumerate(extras) for t in q_proj(H - 2, (0, 1), i, i + 1, extra)]
            y = functools.reduce(jnp.add, y)
            rest = q_proj(H - 2, (0, 1), nb - 1, nb)
            jobs = [functools.partial(u_sum_job, k, r) for k in range(nb) for r in range(0, D, 16)]
            jobs += [job for g in range(_Q_NOW, nb) for job in operand_jobs("Q", 0, g)]
            _spread(jobs, never, marks, 0, 0.97)
            _spread(scatter_jobs(y, picks), never, rest, 0.3, 0.9)

        copies = [cp_x(0), cp_q(0)] + [cp_x(i) for i in range(1, nb)] + [cp_q(1)] + cp_vectors()
        copies += [cp_q(j) for j in range(2, P)]
        for cp in copies + cp_rest() + cp_kv(w_kv, False) + cp_kv(w_kv, True) + [cp_wo()]:
            cp.start()
        first_pair()
        lax.fori_loop(2, H - 2, middle_head, 0)
        last_pair()

    def keys_values(c, w_kv, u_sum, b_sum, common, a32, v32, lhs, a_fix, v_fix, u_fix, b_fix):
        groups = [(j, k) for j in range(0, nb, 2) for k in range(0, nb, 2)]

        def u_block(j, k):
            return c[j * D:(j + 1) * D, k * T:(k + 1) * T]

        def stage_jobs(i, tiles):
            def a_job(j, r, pin):
                a32[j, r:r + 32, :] = _after(c[pl.ds(start_of(i, D) + r, 32), j * T:(j + 1) * T], pin).astype(F32)

            def v_job(k, t, r, pin):
                words = w_kv[t, P // 2 + (i >> 1), pl.ds(k * T + r, 32), :]
                v32[k, t, r:r + 32, :] = _head_of(_after(words, pin), i & 1)

            return ([functools.partial(a_job, j, r) for j in range(nb) for r in range(0, D, 32)]
                    + [functools.partial(v_job, k, t, r)
                       for k in range(nb) for t in tiles for r in range(0, T, 32)])

        def lhs_jobs(j, k):
            def job(dj, r, pin):
                a = a32[j + dj, r:r + 32, :]
                for dk in range(2):
                    u = _after(c[pl.ds((j + dj) * D + r, 32), pl.ds((k + dk) * T, T)], pin).astype(F32)
                    lhs[j + dj, k + dk, r:r + 32, :] = (a + u).astype(BF)

            return [functools.partial(job, dj, r) for r in range(0, D, 32) for dj in range(2)]

        def common_terms(t, carry):
            first, second, sums, marks = {}, {}, {}, []
            for j, k in groups:
                m = [[None, None], [None, None]]
                for dj in range(2):
                    words = w_kv[t, k // 2, pl.ds((j + dj) * T, T), :]
                    b = _head_of(words, 0), _head_of(words, 1)
                    sums[j + dj] = sums[j + dj] + (b[0] + b[1]) if k else b[0] + b[1]
                    for dk in range(2):
                        m[dj][dk] = _dot(u_block(j + dj, k + dk), b[dk].astype(BF))
                for e in range(2):
                    over_j, over_k = m[0][e] + m[1][e], m[e][0] + m[e][1]
                    first[k + e] = first[k + e] - over_j if j else -over_j
                    second[j + e] = second[j + e] - over_k if k else -over_k
                marks += [m[0][0][r:r + 8] for r in range(0, D, 16)]
            for n in range(nb):
                common[t, n], common[t, nb + n], b_sum[t, n] = first[n], second[n], sums[n]
            _spread(stage_jobs(0, [t]) + lhs_jobs(0, 0), t >= 4, marks, 0, 0.7)
            return carry

        def plane(i, carry):
            never = i >= nb
            first = {(k, t): common[t, k] for k in range(nb) for t in range(4)}
            second = {(j, t): common[t, nb + j] for j in range(nb) for t in range(4)}
            marks = []
            for j, k in groups:
                if marks:
                    _spread(lhs_jobs(j, k), never, marks[-64:], 0, 0.75)
                for t in range(4):
                    m = [[None, None], [None, None]]
                    for dj in range(2):
                        words = w_kv[t, k // 2, pl.ds((j + dj) * T, T), :]
                        b = _head_of(words, 0), _head_of(words, 1)
                        for dk in range(2):
                            m[dj][dk] = _dot(lhs[j + dj, k + dk], (b[dk] + v32[k + dk, t]).astype(BF))
                    for e in range(2):
                        first[k + e, t] = first[k + e, t] + (m[0][e] + m[1][e])
                        second[j + e, t] = second[j + e, t] + (m[e][0] + m[e][1])
                    marks += [m[0][0][r:r + 8] for r in range(0, D, 16)]

            def a_job(r, pin):
                a = [_after(a32[j, r:r + 16, :], pin) for j in range(nb)]
                total = functools.reduce(jnp.add, a)
                for n in range(nb):
                    a_fix[n, r:r + 16, :] = a[n].astype(BF)
                    u_fix[n, r:r + 16, :] = (total + u_sum[n, r:r + 16, :]).astype(BF)

            def v_job(t, r, pin):
                v = [_after(v32[k, t, r:r + 16, :], pin) for k in range(nb)]
                total = functools.reduce(jnp.add, v)
                for n in range(nb):
                    v_fix[n, t, r:r + 16, :] = v[n].astype(BF)
                    b_fix[n, t, r:r + 16, :] = (total + b_sum[t, n, r:r + 16, :]).astype(BF)

            jobs = [functools.partial(a_job, r) for r in range(0, D, 16)]
            jobs += [functools.partial(v_job, t, r) for t in range(4) for r in range(0, T, 16)]
            _spread(jobs, never, marks, 0.1, 0.7)
            marks = []
            for n in range(nb):
                x = _dot(u_fix[n], _cat([v_fix[n, t] for t in range(4)], axis=1))
                done = [first[n, t] - x[:, t * T:(t + 1) * T] for t in range(4)]
                for t in range(4):
                    kv_all[n, t, pl.ds(start_of(i, D), D), :] = done[t].astype(BF)
                if n == 0:
                    for kind, (lo, hi) in (("K", done[:2]), ("V", done[2:])):
                        put_operands(kind, pl.ds(start_of(i, T), T), (lo[:T], hi[:T], lo[T:], hi[T:]))
                y = _dot(a_fix[n], _cat([b_fix[n, t] for t in range(4)], axis=1))
                for t in range(4):
                    kv_all[nb + i, t, n * D:(n + 1) * D, :] = (second[n, t] - y[:, t * T:(t + 1) * T]).astype(BF)
                marks += [z[r:r + 8, :T] for z in (x, y) for r in range(0, D, 16)]
            _spread(stage_jobs(jnp.minimum(i + 1, nb - 1), range(4)) + lhs_jobs(0, 0), never, marks, 0, 0.95)
            return carry

        for cp in cp_kv(w_kv, False):
            cp.wait()
        lax.fori_loop(0, 4, common_terms, 0)
        for cp in cp_kv(w_kv, True) + [cp_wo()]:
            cp.wait()
        lax.fori_loop(0, nb, plane, 0)

    def attention(ctx7, wo7, outT, *inv_sums):
        def cp_out(i):
            return pltpu.make_async_copy(outT.at[i], outT_hbm.at[:, pl.ds(i * D, D)], sem.at[0])

        def head(h, carry):
            never = h >= H
            clock, room, scores_of, last_use = [], [], {}, {}

            def tick(x, tiles, free):
                n = max(1, x.shape[0] * tiles // 64)
                clock.extend(x[(k * (x.shape[0] // 8) // n) * 8:][:8, -T:] for k in range(n))
                room.extend([free] * n)
                return x

            def wo_job(r, pin):
                quads = [_after(woT[h, pl.ds(rh * Mh + r, 16), pl.ds(ch * T, T)], pin).astype(F32)
                         for rh in range(2) for ch in range(2)]
                for n, t in enumerate(_operands(_LHS, quads)):
                    wo7[n, r:r + 16, :] = t.astype(BF)

            def scores(i):
                r = slice(i * T, (i + 1) * T)
                q_top, q_bot = _cat([q9[2, r, :], q9[7, r, :]], axis=1), _cat([q9[8, r, :], q9[3, r, :]], axis=1)
                past = [[], [], [], []]
                if i:
                    m = [None] * 7
                    for n, free in zip(_S_ORDER, _S_ROOM):
                        m[n] = tick(_dot_nt(q9[n, r, :], k9[n, :i * T, :]), i, free)
                        yield i
                    past = [[s[:, t * T:(t + 1) * T] for t in range(i)] for s in _combine(m, _S_ORDER)]
                d1 = _dot_nt(_cat([q_top, q_bot], axis=0), _cat([k9[1, r, :], k9[7, r, :]], axis=1))
                d2 = _dot_nt(q_bot, _cat([k9[8, r, :], k9[4, r, :]], axis=1))
                tick(d1, 3, _S_ROOM[7])
                yield 6
                causal = lax.broadcasted_iota(jnp.int32, (T, T), 1) <= lax.broadcasted_iota(jnp.int32, (T, T), 0)
                diagonal = [jnp.where(causal, d1[:T], -1e9)], [d1[T:], jnp.where(causal, d2, -1e9)]
                rows = []
                for u in range(2):
                    first, second = sorted((2 * u, 2 * u + 1), key=lambda k: max(_S_ORDER.index(n) for n in _OUT[k]))
                    row_max = functools.reduce(jnp.maximum, past[first] + past[second] + diagonal[u])
                    rows.append((past[2 * u] + past[2 * u + 1] + diagonal[u],
                                 jnp.max(row_max, axis=1, keepdims=True)))
                scores_of[i] = rows, len(clock)
                last_use.update({("K", g): len(clock) for g in range(i + 1)})
                last_use["Q", i] = len(clock)

            def attend(i):
                rows, since = scores_of.pop(i)
                r = slice(i * T, (i + 1) * T)
                exps, sums = {}, {}

                def timed(k):
                    if k not in exps:
                        exps[k] = []
                        where = [(0, -1), (1, -2), (1, -1)] if k == 4 else [(k // 2, k % 2 * i + t) for t in range(i)]
                        for t, (u, idx) in enumerate(where):
                            tiles, row_max = rows[u]
                            parts = []
                            for r0 in range(0, T, 16):
                                at = min(len(clock) - 1, max(since - 1, len(clock) - _LEAD + t // 4 * 8 + r0 // 16))
                                parts.append(jnp.exp2(tiles[idx][r0:r0 + 16] - _after(
                                    jnp.broadcast_to(row_max[r0:r0 + 16], (16, T)), (never, clock[at]))))
                            exps[k].append(_cat(parts, axis=0))
                            sums[u] = sums[u] + exps[k][-1] if u in sums else exps[k][-1]
                    return exps[k]

                if i in _TIMED_EXP:
                    def p7(n, t):
                        return _operand(_LHS[n], lambda k: timed(k)[t])
                else:
                    top, bot = ([jnp.exp2(t - row_max) for t in tiles] for tiles, row_max in rows)
                    ops = [_operands(_LHS, (top[t], top[i + t], bot[t], bot[i + t])) for t in range(i)]

                    def p7(n, t):
                        return ops[t][n]

                m = [None] * 7
                for n, free in zip(_P_ORDER, _P_ROOM) if i else ():
                    p = _cat([p7(n, t) for t in range(i)], axis=1).astype(BF)
                    m[n] = tick(_dot(p, v9[n, :i * T, :]), i, free)
                    yield i
                if i in _TIMED_EXP:
                    diagonal = timed(4)
                    for u in range(2):
                        inv_sums[i][u * T:(u + 1) * T, :] = jnp.broadcast_to(_inverse_row_sum(sums[u]), (T, T))
                else:
                    diagonal = [top[-1], bot[-2], bot[-1]]
                d1 = _dot(_cat(diagonal[:2], axis=0).astype(BF), _cat([v9[1, r, :], v9[7, r, :]], axis=1))
                d2 = _dot(diagonal[2].astype(BF), _cat([v9[8, r, :], v9[4, r, :]], axis=1))
                tick(d1, 3, _P_ROOM[7])
                yield 6
                last_use.update({("V", g): len(clock) for g in range(i + 1)})
                o = [d1[:T, :T], d1[:T, T:], d1[T:, :T] + d2[:, :T], d1[T:, T:] + d2[:, T:]]
                if i:
                    o = [a + b for a, b in zip(o, _combine(m, _P_ORDER))]
                if i in _TIMED_EXP:
                    zero = pl.multiple_of((h >> H.bit_length() - 1) * T, T)
                    inv = inv_sums[i][pl.ds(zero, T), :], inv_sums[i][pl.ds(zero + T, T), :]
                else:
                    inv = []
                    for e, late in ((top, o[0]), (bot, o[3])):
                        partial_sums = functools.reduce(jnp.add, e)
                        if i in _LATE_SUM:
                            partial_sums = jnp.where(never, late, partial_sums)
                        inv.append(_inverse_row_sum(partial_sums))
                ctx = (o[0] * inv[0], o[2] * inv[1], o[1] * inv[0], o[3] * inv[1])
                for n, t in enumerate(_operands(_RHS, ctx)):
                    ctx7[n, r, :] = t.astype(BF)

            def out_proj(lo, hi):
                m = [None] * 7
                for n, free in zip(_O_ORDER, _O_ROOM):
                    m[n] = tick(_dot_nt(wo7[n], ctx7[n, lo * T:hi * T, :]), hi - lo, free)
                    yield 1.75 * (hi - lo)
                for k, a in enumerate(_combine(m, _O_ORDER)):
                    rows, cols = slice(k // 2 * Mh, (k // 2 + 1) * Mh), slice(k % 2 * T, (k % 2 + 1) * T)
                    for i in range(lo, hi):
                        total = acc[i, rows, cols] + gate[i, :, cols] * a[:, (i - lo) * T:(i - lo + 1) * T]
                        acc[i, rows, cols] = total
                        outT[i, rows, cols] = total.astype(BF)

                @pl.when(h == H - 1)
                def _():
                    for i in range(lo, hi):
                        cp_out(i).start()

            def begin(step):
                kind, (lo, _, hi) = step[0], step[1:].partition("-")
                lo, hi = int(lo), int(hi or lo) + 1
                if kind == "O":
                    return [out_proj(lo, hi), 12.25 * (hi - lo), 0]
                return [(scores if kind == "S" else attend)(lo), 7 * lo + 6, 0]

            def fit(jobs, lo, hi):
                for cost in range(256, 0, -1):
                    at, saved = [], 0
                    for t in range(lo, hi):
                        if len(at) < len(jobs) and min(jobs[len(at)][0], hi - 1) <= t:
                            saved += room[t]
                            if saved >= cost:
                                saved = 0
                                at.append(t)
                    if len(at) == len(jobs):
                        break
                for k, (_, job) in enumerate(jobs):
                    job((never, clock[at[k] if k < len(at) else hi - 1]))

            def next_head_jobs(until):
                def finished(kind, g):
                    users = range(g, g + 1 if kind == "Q" else nb)
                    return all(("P" if kind == "V" else "S") + str(t) not in ahead for t in users)

                ready = [(free, kind, g) for (kind, g), free in last_use.items()
                         if free <= until and (kind, g) not in rebuilt and finished(kind, g)
                         and g >= {"Q": _Q_NOW, "K": 0, "V": _V_NOW}[kind]]
                rebuilt.update((kind, g) for _, kind, g in ready)
                return [(free + _DELAY, job) for free, kind, g in sorted(ready)
                        for job in operand_jobs(kind, jnp.minimum(h + 1, H - 1), g)]

            first_p, first_o, rebuilt, ahead = None, None, set(), _HEAD_PROGRAM.replace("+", " ").split()
            for group in _HEAD_PROGRAM.split():
                if first_p is None and "P" in group:
                    first_p = len(clock)
                    fit([(0, job) for g in range(_V_NOW) for job in operand_jobs("V", h, g)], 0, first_p - 2 * _MARGIN)
                if first_o is None and "O" in group:
                    first_o = len(clock) - 2 * _MARGIN
                    jobs = [(0, functools.partial(wo_job, r)) for r in range(0, Mh, 16)]
                    jobs += [(0, job) for g in reversed(range(_Q_NOW)) for job in operand_jobs("Q", h, g)]
                    fit(jobs + next_head_jobs(first_o - 64), first_p, first_o)
                assert first_o is not None or not any(f"S{g}" in group for g in range(_Q_NOW))
                running = [begin(step) for step in group.split("+")]
                while running:
                    step = min(running, key=lambda s: s[2] / s[1])
                    try:
                        step[2] += next(step[0])
                    except StopIteration:
                        running.remove(step)
                ahead = [step for step in ahead if step not in group.split("+")]
            fit(next_head_jobs(len(clock)), first_o, len(clock) - _MARGIN)
            return carry

        lax.fori_loop(0, H, head, 0)
        for i in range(nb):
            cp_out(i).wait()

    def projections(*shared):
        pl.run_scoped(
            functools.partial(queries, *shared),
            xT=vmem((nb, M, D), BF), wq=vmem((P, M, D), U32), wr=vmem((M,), BF), gw=vmem((M,), BF),
            wg=vmem((M, F), BF), wu=vmem((M, F), BF), wdT=vmem((M, F), BF),
            x7=vmem((7, S // 2, D), BF), wq7=vmem((3, 7, D, T), BF),
            vec_cols=vmem((2, M, T), F32), score=vmem((nb, 1, D), F32))
        pl.run_scoped(
            functools.partial(keys_values, *shared),
            b_sum=vmem((4, nb, T, T), F32), common=vmem((4, 2 * nb, D, T), F32),
            a32=vmem((nb, D, T), F32), v32=vmem((nb, 4, T, T), F32), lhs=vmem((nb, nb, D, T), BF),
            a_fix=vmem((nb, D, T), BF), v_fix=vmem((nb, 4, T, T), BF),
            u_fix=vmem((nb, D, T), BF), b_fix=vmem((nb, 4, T, T), BF))

    pl.run_scoped(projections, vmem((S, Dc), BF), vmem((4, P, Dc, T), U32), vmem((nb, D, T), F32))
    pl.run_scoped(attention, vmem((7, S // 2, T), BF), vmem((7, Mh, T), BF), vmem((nb, M, D), BF),
                  *[vmem((D, T), F32)] * nb)


@jax.jit
def pallas_gated_mix__compressed_kv_cla__moe_arch_mod__prompt_kernel(
    A_x, A_c_kv, A_w_q, A_w_uk, A_w_uv, A_w_o, B_x, B_w_r, B_w_gate, B_w_up, B_w_down, gate_w,
):
    del B_x
    _, S, M = A_x.shape
    _, H, D = A_w_q.shape
    nb = S // D
    assert (D, nb, H) == (2 * T, 8, 16) and A_c_kv.shape == (1, S, nb * T)
    vmem = pltpu.VMEM
    outT = pl.pallas_call(
        _kernel,
        in_specs=[pl.BlockSpec(memory_space=pl.ANY)] * 11,
        out_specs=pl.BlockSpec(memory_space=pl.ANY),
        out_shape=jax.ShapeDtypeStruct((M, S), BF),
        scratch_shapes=[
            vmem((H, M, D), BF),
            vmem((H, 4, S // 2, T), BF),
            vmem((H, 4, S, T), BF),
            *[vmem((9, S // 2, T), BF)] * 3,
            vmem((nb, 1, D), F32),
            vmem((nb, M, D), F32),
            pltpu.SemaphoreType.DMA((4,)),
            pltpu.SemaphoreType.DMA((len(_FIRST_PASS),)),
            pltpu.SemaphoreType.DMA((H // 2,)),
        ],
        compiler_params=pltpu.CompilerParams(vmem_limit_bytes=124 * 2**20),
    )(A_x[0].T, A_c_kv[0], A_w_q, A_w_uk, A_w_uv, jnp.swapaxes(A_w_o, 1, 2), B_w_r, gate_w,
      B_w_gate, B_w_up, B_w_down.T)
    return outT.T[None]
```
